```python
import jax
import jax.numpy as jnp

def _softmax(x, axis=-1):
    return jax.nn.softmax(x, axis=axis)
def _gelu(x):
    return jax.nn.gelu(x, approximate=True)
def _silu(x):
    return jax.nn.silu(x)
def _sigmoid(x):
    return jax.nn.sigmoid(x)
def _layernorm(x, axis=-1, eps=1e-5):
    m = jnp.mean(x, axis=axis, keepdims=True)
    v = jnp.var(x, axis=axis, keepdims=True)
    return (x - m) / jnp.sqrt(v + eps)
def _scatter_add(tgt, idx, src, axis=0):
    return tgt.at[idx].add(src)
def _segment_sum(src, seg, n):
    return jax.ops.segment_sum(src, seg, n)
class _Rng:
    def __init__(self, key):
        self._k = key
    def _next(self):
        self._k, sub = jax.random.split(self._k)
        return sub
    def normal(self, shape):
        return jax.random.normal(self._next(), shape, dtype=jnp.bfloat16)
    def randint(self, lo, hi, shape):
        return jax.random.randint(self._next(), shape, lo, hi, dtype=jnp.int32)
    def uniform(self, shape, lo=0.0, hi=1.0):
        return jax.random.uniform(self._next(), shape, jnp.bfloat16, lo, hi)
    def permutation(self, n):
        return jax.random.permutation(self._next(), n)


kernel_name = 'recurrent_scan__mha_block_cached__moe_arch_mod__prompt'

def setup_inputs():
    _rng = _Rng(jax.random.key(int.from_bytes(__import__("os").urandom(4), "little")))
    _w = (lambda a: (lambda t: t.astype(jnp.bfloat16) if jnp.issubdtype(t.dtype, jnp.floating) else t)(jnp.asarray(a)))
    def _A_setup():
        B, Sq, D = 1, 2048, 640
        H, Sk, Dh = 32, 2048, 128
        return {
            "x": _w((lambda *s: _rng.normal(s) * 0.05)(B, Sq, D)),
            "k_cache": _w((lambda *s: _rng.normal(s) * 0.05)(B, H, Sk, Dh)),
            "v_cache": _w((lambda *s: _rng.normal(s) * 0.05)(B, H, Sk, Dh)),
            "wq": _w((lambda *s: _rng.normal(s) * 0.05)(D, H * Dh) * (D ** -0.5)),
            "wo": _w((lambda *s: _rng.normal(s) * 0.05)(H * Dh, D) * ((H * Dh) ** -0.5)),
        }
    _A_in = _A_setup()

    def _B_setup():
        B, S, D, F, C = 1, 2048, 640, 1728, 8
        return {
            "x": _w((lambda *s: _rng.normal(s) * 0.05)(B, S, D)),
            "w_r": _w((lambda *s: _rng.normal(s) * 0.05)(D)),
            "w_gate": _w((lambda *s: _rng.normal(s) * 0.05)(D, F)),
            "w_up": _w((lambda *s: _rng.normal(s) * 0.05)(D, F)),
            "w_down": _w((lambda *s: _rng.normal(s) * 0.05)(F, D)),
        }
    _B_in = _B_setup()

    return {
        "A_x": _A_in["x"],
        "A_k_cache": _A_in["k_cache"],
        "A_v_cache": _A_in["v_cache"],
        "A_wq": _A_in["wq"],
        "A_wo": _A_in["wo"],
        "B_x": _B_in["x"],
        "B_w_r": _B_in["w_r"],
        "B_w_gate": _B_in["w_gate"],
        "B_w_up": _B_in["w_up"],
        "B_w_down": _B_in["w_down"],
    }

def reference(A_x, A_k_cache, A_v_cache, A_wq, A_wo, B_x, B_w_r, B_w_gate, B_w_up, B_w_down):
    def _A_ref(x, k_cache, v_cache, wq, wo):
        B, Sq, D = x.shape
        H, Dh = 32, 128
        q = (lambda x, *d: x.transpose(*d))((x @ wq).reshape(B, Sq, H, Dh), 0, 2, 1, 3)
        scores = jnp.einsum("bhqd,bhkd->bhqk", q, k_cache) * (Dh ** -0.5)
        p = _softmax(scores, axis=-1)
        o = jnp.einsum("bhqk,bhkd->bhqd", p, v_cache)
        return (lambda x, *d: x.transpose(*d))(o, 0, 2, 1, 3).reshape(B, Sq, H * Dh) @ wo

    def _B_ref(x, w_r, w_gate, w_up, w_down):
        B, S, D = x.shape
        C = 8
        r = x @ w_r
        idx = jnp.argsort(-r, axis=-1)[:, :C]
        idx_e = jnp.repeat(idx.reshape(B, C, 1), D, axis=2)
        x_sel = jnp.take_along_axis(x, idx_e, axis=1)
        g = _silu(x_sel @ w_gate)
        u = x_sel @ w_up
        y = (g * u) @ w_down
        r_sel = _sigmoid(jnp.take_along_axis(r, idx, axis=1))
        y = y * r_sel.reshape(B, C, 1)
        b_off = (jnp.arange(B) * S).reshape(B, 1)
        flat_idx = (idx + b_off).reshape(B * C)
        zero = (x * 0.0).reshape(B * S, D)
        upd = _scatter_add(zero, flat_idx, y.reshape(B * C, D), axis=0)
        return x + upd.reshape(B, S, D)

    x = A_x
    xn = _layernorm(x, axis=-1)
    s = _A_ref(xn, A_k_cache, A_v_cache, A_wq, A_wo)
    g = _silu(_B_ref(xn, B_w_r, B_w_gate, B_w_up, B_w_down))
    return x + s * g
```

```python
import functools
import jax
import jax.numpy as jnp
from jax import lax
import jax.experimental.pallas as pl
import jax.experimental.pallas.tpu as pltpu

S, D, H, DH, F, C = 2048, 640, 32, 128, 1728, 8
LOG2E = 1.4426950408889634
bf16 = jnp.bfloat16
f32 = jnp.float32
i32 = jnp.int32
NT = (((1,), (1,)), ((), ()))


class _NoScope:
    def __init__(self, name):
        pass

    def __enter__(self):
        return self

    def __exit__(self, *a):
        return False


def _rb(x):
    return x.astype(bf16).astype(f32)


def _layernorm(x_bf):
    x = x_bf.astype(f32)
    mean = jnp.sum(x, axis=-1, keepdims=True) * (1.0 / D)
    c = x - mean
    var = jnp.sum(c * c, axis=-1, keepdims=True) * (1.0 / D)
    num = _rb(x - _rb(mean))
    den = _rb(jnp.sqrt(_rb(_rb(var) + 1e-5)))
    inv = pl.reciprocal(den, approx=True)
    inv = inv * (2.0 - den * inv)
    return (num * inv).astype(bf16)


def _silu(x):
    hx = 0.5 * x
    return hx + hx * jnp.tanh(hx)


def _fold(x, op):
    r = x[:, 0:128]
    for t in range(1, x.shape[1] // 128):
        r = op(r, x[:, t * 128:(t + 1) * 128])
    return r


def build(A_x, A_k_cache, A_v_cache, A_wq, A_wo, B_x, B_w_r, B_w_gate, B_w_up, B_w_down,
          ts=128, kc=512, order="A B0 D C0 B1 C1 B2 C2 B3 C3", thr=1, nxc=8, win=3,
          moe_rate=1, e_lag=1, extra_d=(1,), ochunk=2, grows=0, nring=2, only=None, scopes=False, nf_dbg=None, zrows=56):
    nsub = S // ts
    nch = S // kc
    nf = (F + 127) // 128
    if nf_dbg is not None:
        nf = nf_dbg
    xc = S // nxc
    upc = xc // 128
    x2 = A_x.reshape(S, D)
    k3 = A_k_cache.reshape(H, S, DH)
    v3 = A_v_cache.reshape(H, S, DH)
    order = order.split()
    noc = nsub // ochunk

    scope = jax.named_scope if scopes else _NoScope

    def kernel(x_hbm, k_hbm, v_hbm, wq_hbm, wo_hbm, wr_ref, wg_hbm, wu_hbm, wd_hbm, o_hbm,
               z_v, x_v, xn_v, g_v, k_v, v_v, wq_v, wo_v, wg_v, wu_v, wd_v, acc, r_v, xs_v, ms_v, idx_s,
               s_c, m_c, q_c, o_c, l_c, out_v,
               sem_x, sem_h, sem_f, sem_o):
        def cp_x(c):
            rows = pl.ds(c * xc, xc) if isinstance(c, int) else pl.ds(pl.multiple_of(c * xc, xc), xc)
            return pltpu.make_async_copy(x_hbm.at[rows, :], x_v.at[rows, :], sem_x.at[c])

        def hsem(h, i):
            return sem_h.at[(h % nring) * 4 + i]

        def cp_k(h):
            return pltpu.make_async_copy(k_hbm.at[h], k_v.at[h], hsem(h, 0))

        def cp_v(h):
            return pltpu.make_async_copy(v_hbm.at[h], v_v.at[h], hsem(h, 1))

        def hoff(h):
            return h * DH if isinstance(h, int) else pl.multiple_of(h * DH, DH)

        def cp_wq(h):
            return pltpu.make_async_copy(wq_hbm.at[:, pl.ds(hoff(h), DH)], wq_v.at[h], hsem(h, 2))

        def cp_wo(h):
            return pltpu.make_async_copy(wo_hbm.at[pl.ds(hoff(h), DH), :], wo_v.at[h], hsem(h, 3))

        def cp_f(i):
            return pltpu.make_async_copy((wg_hbm, wu_hbm, wd_hbm)[i], (wg_v, wu_v, wd_v)[i], sem_f.at[i])

        def cp_o(c):
            rows = pl.ds(c * ochunk * ts, ochunk * ts)
            return pltpu.make_async_copy(out_v.at[rows, :], o_hbm.at[rows, :], sem_o.at[c])

        def sub(j):
            return pl.ds(j * ts, ts)

        def router(u):
            wrf = jnp.broadcast_to(wr_ref[...].astype(f32).reshape(1, D), (16, D))
            lhs = jnp.where(lax.broadcasted_iota(i32, (16, D), 0) == u, wrf, 0.0).astype(bf16)
            rows = pl.ds(u * 128, 128) if isinstance(u, int) else pl.ds(pl.multiple_of(u * 128, 128), 128)
            return lax.dot_general(lhs, xn_v[rows, :], NT, preferred_element_type=f32)

        def gate_rows(r0):
            rows = pl.ds(pl.multiple_of(r0, 16), grows)
            g_v[rows, :] = _silu(xn_v[rows, :].astype(f32))

        def qproj(h, j):
            q = jnp.dot(xn_v[sub(j), :], wq_v[h], preferred_element_type=f32)
            return (q * (DH ** -0.5 * LOG2E)).astype(bf16)

        def oproj(h, j, o, final=False):
            y = jnp.dot(o, wo_v[h], preferred_element_type=f32)
            if final:
                t = (acc[sub(j), :] + y) * g_v[sub(j), :]
                out_v[sub(j), :] = (x_v[sub(j), :].astype(f32) + t).astype(bf16)
                if (j + 1) % ochunk == 0:
                    cp_o(j // ochunk).start()
            else:
                acc[sub(j), :] += y

        def fin_m(mrun):
            return jnp.broadcast_to(jnp.max(mrun, axis=-1, keepdims=True), (ts, 128))

        def fin_o(o, lrun):
            l = jnp.sum(lrun, axis=-1, keepdims=True)
            return (o * pl.reciprocal(l, approx=True)).astype(bf16)

        def topk(rsum):
            r = _rb(rsum) + 0.0
            bits = lax.shift_right_logical(pltpu.bitcast(r, i32), 16)
            ordered = jnp.where(bits >= 0x8000, 0xFFFF - bits, bits + 0x8000)
            ordered = jnp.where(r != r, 0, ordered)
            sl = lax.broadcasted_iota(i32, (16, 128), 0)
            ln = lax.broadcasted_iota(i32, (16, 128), 1)
            key = pltpu.bitcast(ordered * 2048 + (2047 - (sl * 128 + ln)) + (1 << 28), f32)
            sub16 = lax.broadcasted_iota(i32, (16, D), 0)
            x_sel = jnp.zeros((16, D), f32)
            msel = jnp.zeros((16, 128), f32)
            for c in range(C):
                m = jnp.max(jnp.max(key, axis=0, keepdims=True), axis=1, keepdims=True)
                mb = jnp.broadcast_to(m, (16, 128))
                key = jnp.where(key == mb, 0.0, key)
                msel = jnp.where(sl == c, mb, msel)
                ic = (2047 - (pltpu.bitcast(mb, i32) & 2047))[0, 0]
                idx_s[c] = ic
                base = pl.multiple_of((ic // 16) * 16, 16)
                blk = xn_v[pl.ds(base, 16), :].astype(f32)
                row = jnp.sum(jnp.where(sub16 == ic % 16, blk, 0.0), axis=0, keepdims=True)
                x_sel = jnp.where(sub16 == c, row, x_sel)
            o16 = lax.shift_right_logical(pltpu.bitcast(msel, i32) - (1 << 28), 11) & 0xFFFF
            rbits = jnp.where(o16 >= 0x8000, o16 - 0x8000, 0xFFFF - o16)
            r_sel = jnp.where(sl < C, pltpu.bitcast(lax.shift_left(rbits, 16), f32), 0.0)
            ms_v[...] = _rb(0.5 + 0.5 * jnp.tanh(0.5 * r_sel))
            xs_v[...] = x_sel

        def ffn():
            x_sel = xs_v[...]
            xs = x_sel.astype(bf16)
            hs = []
            for t in range(nf):
                fs = slice(t * 128, min((t + 1) * 128, F))
                hg = _rb(lax.dot_general(xs, wg_v[fs, :], NT, preferred_element_type=f32))
                if moe_rate == 1:
                    yield
                hu = _rb(lax.dot_general(xs, wu_v[fs, :], NT, preferred_element_type=f32))
                hs.append((_rb(_silu(hg)) * hu).astype(bf16))
                yield
            y = None
            for t in range(nf):
                fs = slice(t * 128, min((t + 1) * 128, F))
                yc = jnp.dot(hs[t], wd_v[fs, :], preferred_element_type=f32)
                y = yc if y is None else y + yc
                if moe_rate == 1 or t % 2 == 1:
                    yield
            y = _rb(_rb(y) * jnp.concatenate([ms_v[...]] * (D // 128), axis=1))
            gsel = _silu(_rb(x_sel + y))
            for c in range(C):
                g_v[pl.ds(jnp.clip(idx_s[c], 0, S - 1), 1), :] = gsel[c:c + 1, :]

        def run_slots(h, lasth):
            def unit(off):
                if off < 0:
                    return (h - 1 if lasth else jnp.maximum(h - 1, 0)), off + nsub
                if off >= nsub:
                    return h + 1, off - nsub
                return h, off

            z = jnp.concatenate([z_v[0:8, :]] * (ts // 8), axis=0)
            s_prev = None
            q = q_c[...]
            m_prev = fin_m(m_c[...])
            o_done = fin_o(o_c[...], l_c[...])
            pend = []
            moe_gen = ffn() if lasth else None
            moe_done = None
            for j in range(nsub):
                kb, _ = unit(j + 1)
                s_list = [None] * nch
                mrun = None
                lrun = None
                o = None
                ocs = []
                q_next = None
                do_a = not (lasth and j + 2 >= nsub)
                do_b = not (lasth and j + 1 >= nsub)
                for op in order:
                    if moe_gen is not None and op[0] in 'BC':
                        try:
                            next(moe_gen)
                        except StopIteration:
                            moe_gen = None
                            moe_done = j
                    if op == 'A':
                        if do_a:
                            q_next = qproj(*unit(j + 2))
                    elif op == 'D':
                        if lasth and j > 0:
                            pend.append((j - 1, o_done))
                            if moe_done is not None and j >= moe_done + e_lag:
                                u, od = pend.pop(0)
                                oproj(h, u, od, final=True)
                        else:
                            oproj(*unit(j - 1), o_done)
                    elif op[0] == 'B':
                        if do_b:
                            c = int(op[1:])
                            cs = slice(c * kc, (c + 1) * kc)
                            s = lax.dot_general(q, k_v[kb, cs, :], NT, preferred_element_type=f32)
                            s_list[c] = s
                            mc = _fold(s, jnp.maximum)
                            mrun = mc if mrun is None else jnp.maximum(mrun, mc)
                    elif op[0] == 'C':
                        c = int(op[1:])
                        cs = slice(c * kc, (c + 1) * kc)
                        sp = s_c[:, cs] if j == 0 else s_prev[c]
                        m_use = m_prev
                        if thr and do_b and len(ocs) >= thr:
                            m_use = m_prev + pltpu.bitcast(pltpu.bitcast(ocs[len(ocs) - thr], i32) & z, f32)
                        p = jnp.exp2(sp - jnp.concatenate([m_use] * (kc // 128), axis=1))
                        lc = _fold(p, jnp.add)
                        lrun = lc if lrun is None else lrun + lc
                        oc = jnp.dot(p.astype(bf16), v_v[h, cs, :], preferred_element_type=f32)
                        ocs.append(oc)
                        o = oc if o is None else o + oc
                        if lasth and c in extra_d and pend and moe_done is not None and j >= moe_done + e_lag:
                            u, od = pend.pop(0)
                            oproj(h, u, od, final=True)
                s_prev = s_list
                q = q_next
                if j + 1 < nsub:
                    m_prev = fin_m(mrun) if do_b else None
                    o_done = fin_o(o, lrun)
            if lasth:
                pend.append((nsub - 1, fin_o(o, lrun)))
                for u, od in pend:
                    oproj(h, u, od, final=True)
                return
            for c in range(nch):
                s_c[:, c * kc:(c + 1) * kc] = s_prev[c]
            q_c[...] = q
            m_c[...] = mrun
            o_c[...] = o
            l_c[...] = lrun

        tail = [cp_wq(0), cp_k(0), cp_v(0), cp_wo(0), cp_wq(1), cp_k(1)]
        for c in range(win):
            cp_x(c).start()
        r_v[...] = jnp.zeros((16, 128), f32)
        o_c[...] = jnp.zeros((ts, DH), f32)
        l_c[...] = jnp.ones((ts, 128), f32)

        def ln_chunk(c, first=False):
            rows = pl.ds(c * xc, xc) if isinstance(c, int) else pl.ds(pl.multiple_of(c * xc, xc), xc)
            if not first:
                rs = r_v[...]
                for t in range(upc):
                    rs = rs + router((c - 1) * upc + t)
                r_v[...] = rs
            xn = _layernorm(x_v[rows, :])
            xn_v[rows, :] = xn
            if not grows:
                g_v[rows, :] = _silu(xn.astype(f32))
            acc[rows, :] = jnp.zeros((xc, D), f32)

        with scope('ln'):
            cp_x(0).wait()
            cp_x(win).start()
            t0 = x_v[0:16, 0:128].astype(f32)[0:8, :]
            t0 = jnp.where(jnp.abs(t0) < 1.0, t0, 0.5)
            z_v[0:8, :] = pltpu.bitcast(t0 - t0, i32)
            ln_chunk(0, first=True)

            def ln_body(c, _):
                cp_x(c).wait()

                @pl.when(c + win < nxc)
                def _():
                    cp_x(c + win).start()
                for i in range(win):
                    @pl.when(c + win == nxc + i)
                    def _():
                        tail[i].start()
                ln_chunk(c)
                return 0
            lax.fori_loop(1, nxc, ln_body, 0)
        with scope('pro'):
            for i in range(win, len(tail)):
                tail[i].start()
            tail[0].wait()
            tail[1].wait()
            rs = r_v[...]
            for t in range(upc):
                rs = rs + router((nxc - 1) * upc + t)
            topk(rs)
            q0 = qproj(0, 0)
            s0 = lax.dot_general(q0, k_v[0], NT, preferred_element_type=f32)
            s_c[...] = s0
            m_c[...] = _fold(s0, jnp.maximum)
            q_c[...] = qproj(0, 1)
        with scope('wpro'):
            for i in range(2, len(tail)):
                tail[i].wait()

        def body(h, _):
            cp_v(h + 1).start()
            cp_wo(h + 1).start()

            @pl.when(h + 2 < H)
            def _():
                cp_wq(h + 2).start()
                cp_k(h + 2).start()

            @pl.when(h == 1)
            def _():
                for i in range(3):
                    cp_f(i).start()
            with scope('mid'):
                if grows:
                    gate_rows(jnp.minimum(h * grows, S - grows))
                run_slots(h, False)
            cp_v(h + 1).wait()
            cp_wo(h + 1).wait()

            @pl.when(h + 2 < H)
            def _():
                cp_wq(h + 2).wait()
                cp_k(h + 2).wait()
            return 0

        lax.fori_loop(0, H - 1, body, 0)
        for i in range(3):
            cp_f(i).wait()
        with scope('last'):
            run_slots(H - 1, True)
        with scope('wout'):
            for c in range(noc):
                cp_o(c).wait()

    anyspec = pl.BlockSpec(memory_space=pl.ANY)
    out = pl.pallas_call(
        kernel,
        in_specs=[anyspec, anyspec, anyspec, anyspec, anyspec,
                  pl.BlockSpec(memory_space=pltpu.VMEM),
                  anyspec, anyspec, anyspec],
        out_specs=anyspec,
        out_shape=jax.ShapeDtypeStruct((S, D), bf16),
        scratch_shapes=[
            pltpu.VMEM((zrows, 128), i32),
            pltpu.VMEM((S, D), bf16),
            pltpu.VMEM((S, D), bf16),
            pltpu.VMEM((S, D), f32),
            pltpu.VMEM((H, S, DH), bf16),
            pltpu.VMEM((H, S, DH), bf16),
            pltpu.VMEM((H, D, DH), bf16),
            pltpu.VMEM((H, DH, D), bf16),
            pltpu.VMEM((F, D), bf16),
            pltpu.VMEM((F, D), bf16),
            pltpu.VMEM((F, D), bf16),
            pltpu.VMEM((S, D), f32),
            pltpu.VMEM((16, 128), f32),
            pltpu.VMEM((16, D), f32),
            pltpu.VMEM((16, 128), f32),
            pltpu.SMEM((C,), i32),
            pltpu.VMEM((ts, S), f32),
            pltpu.VMEM((ts, 128), f32),
            pltpu.VMEM((ts, DH), bf16),
            pltpu.VMEM((ts, DH), f32),
            pltpu.VMEM((ts, 128), f32),
            pltpu.VMEM((S, D), bf16),
            pltpu.SemaphoreType.DMA((nxc,)),
            pltpu.SemaphoreType.DMA((nring * 4,)),
            pltpu.SemaphoreType.DMA((3,)),
            pltpu.SemaphoreType.DMA((noc,)),
        ],
        compiler_params=pltpu.CompilerParams(vmem_limit_bytes=120 * 1024 * 1024, disable_bounds_checks=True),
    )(x2, k3, v3, A_wq, A_wo, B_w_r, B_w_gate.T, B_w_up.T, B_w_down)
    return out.reshape(1, S, D)


@jax.jit
def pallas_recurrent_scan__mha_block_cached__moe_arch_mod__prompt_kernel(
        A_x, A_k_cache, A_v_cache, A_wq, A_wo, B_x, B_w_r, B_w_gate, B_w_up, B_w_down):
    return build(A_x, A_k_cache, A_v_cache, A_wq, A_wo, B_x, B_w_r, B_w_gate, B_w_up, B_w_down)
```

```python
import functools
import jax
import jax.numpy as jnp
from jax import lax
import jax.experimental.pallas as pl
import jax.experimental.pallas.tpu as pltpu

S, D, H, DH, F, C = 2048, 640, 32, 128, 1728, 8
LOG2E = 1.4426950408889634
bf16 = jnp.bfloat16
f32 = jnp.float32
i32 = jnp.int32
NT = (((1,), (1,)), ((), ()))


class _NoScope:
    def __init__(self, name):
        pass

    def __enter__(self):
        return self

    def __exit__(self, *a):
        return False


def _rb(x):
    return x.astype(bf16).astype(f32)


def _layernorm(ld, numround=True):
    mean = jnp.sum(ld(0).astype(f32), axis=-1, keepdims=True) * (1.0 / D)
    c = ld(1).astype(f32) - mean
    var = jnp.sum(c * c, axis=-1, keepdims=True) * (1.0 / D)
    num = ld(2).astype(f32) - _rb(mean)
    if numround:
        num = _rb(num)
    den = _rb(jnp.sqrt(_rb(_rb(var) + 1e-5)))
    inv = pl.reciprocal(den, approx=True)
    inv = inv * (2.0 - den * inv)
    return (num * inv).astype(bf16)


def _silu(x):
    hx = 0.5 * x
    return hx + hx * jnp.tanh(hx)


def _fold(x, op):
    r = x[:, 0:128]
    for t in range(1, x.shape[1] // 128):
        r = op(r, x[:, t * 128:(t + 1) * 128])
    return r


def build(A_x, A_k_cache, A_v_cache, A_wq, A_wo, B_x, B_w_r, B_w_gate, B_w_up, B_w_down,
          ts=128, kc=512, order="A B0 D C0 B1 C1 B2 C2 B3 C3", thr=1, nxc=8, win=3,
          moe_rate=1, e_lag=1, extra_d=(1,), ochunk=2, scopes=False, zrows=56, mdl=0, nolast=False,
          hpb=1, dma_slot=1, thr0=True, preq=True, lorder=None, osched=(2, 3, 4, 5, 6, 6), lnsub=1, gmode='mid', numround=True, reload=False, grows=256, mrows=80, gtie=3, csplit=0):
    nsub = S // ts
    nch = S // kc
    nf = (F + 127) // 128
    xc = S // nxc
    upc = xc // 128
    x2 = A_x.reshape(S, D)
    k3 = A_k_cache.reshape(H, S, DH)
    v3 = A_v_cache.reshape(H, S, DH)
    order = order.split()
    lorder = lorder.split() if lorder else order
    noc = nsub // ochunk
    nloop = (H - 1) // hpb
    nlast = H - nloop * hpb
    scope = jax.named_scope if scopes else _NoScope

    def kernel(x_hbm, k_hbm, v_hbm, wq_hbm, wo_hbm, wr_ref, wg_hbm, wu_hbm, wd_hbm, o_hbm,
               z_v, x_v, xn_v, g_v, k_v, v_v, wq_v, wo_v, wg_v, wu_v, wd_v, acc, r_v, xs_v, ms_v, idx_s,
               s_c, m_c, q_c, o_c, l_c, out_v, ql_v, wql_v,
               sem_x, sem_h, sem_f, sem_o):
        def cp_x(c):
            rows = pl.ds(c * xc, xc) if isinstance(c, int) else pl.ds(pl.multiple_of(c * xc, xc), xc)
            return pltpu.make_async_copy(x_hbm.at[rows, :], x_v.at[rows, :], sem_x.at[c])

        def hoff(h):
            return h * DH if isinstance(h, int) else pl.multiple_of(h * DH, DH)

        def cp_k(h, i):
            return pltpu.make_async_copy(k_hbm.at[h], k_v.at[h], sem_h.at[4 * i])

        def cp_v(h, i):
            return pltpu.make_async_copy(v_hbm.at[h], v_v.at[h], sem_h.at[4 * i + 1])

        def cp_wq(h, i):
            return pltpu.make_async_copy(wq_hbm.at[:, pl.ds(hoff(h), DH)], wq_v.at[h], sem_h.at[4 * i + 2])

        def cp_wo(h, i):
            return pltpu.make_async_copy(wo_hbm.at[pl.ds(hoff(h), DH), :], wo_v.at[h], sem_h.at[4 * i + 3])

        def cp_f(i):
            return pltpu.make_async_copy((wg_hbm, wu_hbm, wd_hbm)[i], (wg_v, wu_v, wd_v)[i], sem_f.at[i])

        def cp_o(c):
            rows = pl.ds(c * ochunk * ts, ochunk * ts)
            return pltpu.make_async_copy(out_v.at[rows, :], o_hbm.at[rows, :], sem_o.at[c])

        def sub(j):
            return pl.ds(j * ts, ts)

        def half(r0, n):
            if isinstance(r0, int):
                return pl.ds(r0 // 2, n // 2)
            return pl.ds(pl.multiple_of(r0 // 2, 8), n // 2)

        def xn_ld(r0, n):
            return pltpu.bitcast(xn_v[half(r0, n), :], bf16)

        def router(u):
            wrf = jnp.broadcast_to(wr_ref[...].astype(f32).reshape(1, D), (16, D))
            lhs = jnp.where(lax.broadcasted_iota(i32, (16, D), 0) == u, wrf, 0.0).astype(bf16)
            return lax.dot_general(lhs, xn_ld(u * 128, 128), NT, preferred_element_type=f32)

        def qproj(h, j):
            q = jnp.dot(xn_ld(j * ts, ts), wq_v[h], preferred_element_type=f32)
            return (q * (DH ** -0.5 * LOG2E)).astype(bf16)

        def oproj(h, j, o, final=False):
            y = jnp.dot(o, wo_v[h], preferred_element_type=f32)
            if final:
                t = (acc[sub(j), :] + y) * g_v[sub(j), :]
                out_v[sub(j), :] = (x_v[sub(j), :].astype(f32) + t).astype(bf16)
                if (j + 1) % ochunk == 0:
                    cp_o(j // ochunk).start()
            else:
                acc[sub(j), :] += y

        def fin_m(mrun):
            return jnp.broadcast_to(jnp.max(mrun, axis=-1, keepdims=True), (ts, 128))

        def fin_o(o, lrun):
            l = jnp.sum(lrun, axis=-1, keepdims=True)
            return (o * pl.reciprocal(l, approx=True)).astype(bf16)

        def topk(rsum):
            r = _rb(rsum) + 0.0
            bits = lax.shift_right_logical(pltpu.bitcast(r, i32), 16)
            ordered = jnp.where(bits >= 0x8000, 0xFFFF - bits, bits + 0x8000)
            ordered = jnp.where(r != r, 0, ordered)
            sl = lax.broadcasted_iota(i32, (16, 128), 0)
            ln = lax.broadcasted_iota(i32, (16, 128), 1)
            key = pltpu.bitcast(ordered * 2048 + (2047 - (sl * 128 + ln)) + (1 << 28), f32)
            sub16 = lax.broadcasted_iota(i32, (16, D), 0)
            x_sel = jnp.zeros((16, D), f32)
            msel = jnp.zeros((16, 128), f32)
            for c in range(C):
                m = jnp.max(jnp.max(key, axis=0, keepdims=True), axis=1, keepdims=True)
                mb = jnp.broadcast_to(m, (16, 128))
                key = jnp.where(key == mb, 0.0, key)
                msel = jnp.where(sl == c, mb, msel)
                ic = (2047 - (pltpu.bitcast(mb, i32) & 2047))[0, 0]
                idx_s[c] = ic
                blk = xn_ld((ic // 16) * 16, 16).astype(f32)
                row = jnp.sum(jnp.where(sub16 == ic % 16, blk, 0.0), axis=0, keepdims=True)
                x_sel = jnp.where(sub16 == c, row, x_sel)
            o16 = lax.shift_right_logical(pltpu.bitcast(msel, i32) - (1 << 28), 11) & 0xFFFF
            rbits = jnp.where(o16 >= 0x8000, o16 - 0x8000, 0xFFFF - o16)
            r_sel = jnp.where(sl < C, pltpu.bitcast(lax.shift_left(rbits, 16), f32), 0.0)
            ms_v[...] = _rb(0.5 + 0.5 * jnp.tanh(0.5 * r_sel))
            xs_v[...] = x_sel

        def ffn():
            x_sel = xs_v[...]
            xs = x_sel.astype(bf16)
            hs = []
            for t in range(nf):
                fs = slice(t * 128, min((t + 1) * 128, F))
                hg = _rb(lax.dot_general(xs, wg_v[fs, :], NT, preferred_element_type=f32))
                if moe_rate == 1:
                    yield
                hu = _rb(lax.dot_general(xs, wu_v[fs, :], NT, preferred_element_type=f32))
                hs.append((_rb(_silu(hg)) * hu).astype(bf16))
                yield
            y = None
            for t in range(nf):
                fs = slice(t * 128, min((t + 1) * 128, F))
                yc = jnp.dot(hs[t], wd_v[fs, :], preferred_element_type=f32)
                y = yc if y is None else y + yc
                if moe_rate == 1 or t % 2 == 1:
                    yield
            y = _rb(_rb(y) * jnp.concatenate([ms_v[...]] * (D // 128), axis=1))
            gsel = _silu(_rb(x_sel + y))
            for c in range(C):
                g_v[pl.ds(jnp.clip(idx_s[c], 0, S - 1), 1), :] = gsel[c:c + 1, :]

        def run_slots(h0, nh, tail, hook=None):
            n = nh * nsub

            def unit(t):
                if t < 0:
                    return (h0 - 1 if tail else jnp.maximum(h0 - 1, 0)), t + nsub
                return h0 + t // nsub, t % nsub

            z = jnp.concatenate([z_v[0:8, :]] * (ts // 8), axis=0)
            s_prev = None
            q = q_c[...]
            m_prev = fin_m(m_c[...])
            o_done = fin_o(o_c[...], l_c[...])
            pend = []
            mhist = []
            moe_gen = ffn() if tail else None
            moe_done = None
            for j in range(n):
                hc = unit(j)[0]
                kb = unit(j + 1)[0]
                s_list = [None] * nch
                mrun = None
                lrun = None
                o = None
                ocs = []
                q_next = None
                do_a = not (tail and j + 2 >= n)
                do_b = not (tail and j + 1 >= n)
                if hook is not None and j == dma_slot:
                    hook()
                for op in (lorder if tail else order):
                    if moe_gen is not None and op[0] in 'BC':
                        try:
                            next(moe_gen)
                        except StopIteration:
                            moe_gen = None
                            moe_done = j
                    if op == 'A':
                        if do_a:
                            if tail and preq:
                                q_next = ql_v[sub(j + 2), :]
                            else:
                                q_next = qproj(*unit(j + 2))
                    elif op == 'D':
                        if tail and j - 1 >= n - nsub:
                            pend.append((unit(j - 1), o_done))
                            if moe_done is not None and j >= moe_done + e_lag:
                                u, od = pend.pop(0)
                                oproj(*u, od, final=True)
                        else:
                            oproj(*unit(j - 1), o_done)
                    elif op[0] == 'B':
                        if do_b:
                            c = int(op[1:])
                            cs = slice(c * kc, (c + 1) * kc)
                            qq = q
                            if mdl and len(mhist) >= mdl:
                                w = pltpu.bitcast(mhist[len(mhist) - mdl], i32)
                                w = (w[0:ts // 2, :] | w[ts // 2:, :]) & z[0:ts // 2, :]
                                qq = pltpu.bitcast(pltpu.bitcast(q, i32) | w, bf16)
                            s = lax.dot_general(qq, k_v[kb, cs, :], NT, preferred_element_type=f32)
                            s_list[c] = s
                            mc = _fold(s, jnp.maximum)
                            mrun = mc if mrun is None else jnp.maximum(mrun, mc)
                            mhist.append(mrun)
                    elif op[0] == 'C':
                        c = int(op[1:])
                        cs = slice(c * kc, (c + 1) * kc)
                        sp = s_c[:, cs] if j == 0 else s_prev[c]
                        m_use = m_prev
                        if thr and do_b and len(ocs) >= thr and (thr0 or not (j == 0 and c == 1)):
                            m_use = m_prev + pltpu.bitcast(pltpu.bitcast(ocs[len(ocs) - thr], i32) & z, f32)
                        p = jnp.exp2(sp - jnp.concatenate([m_use] * (kc // 128), axis=1))
                        lc = _fold(p, jnp.add)
                        lrun = lc if lrun is None else lrun + lc
                        pb = p.astype(bf16)
                        if csplit is None:
                            oc = jnp.dot(pb, v_v[hc, cs, :], preferred_element_type=f32)
                            ocs.append(oc)
                        else:
                            parts = [jnp.dot(pb[:, t * 128:(t + 1) * 128], v_v[hc, c * kc + t * 128:c * kc + (t + 1) * 128, :],
                                             preferred_element_type=f32) for t in range(kc // 128)]
                            oc = (parts[0] + parts[1]) + (parts[2] + parts[3])
                            ocs.append(parts[csplit])
                        if gmode == 'mid' and not tail and j == n - 1 and c == gtie:
                            r0 = jnp.minimum(h0 * mrows, S - mrows)
                            w = pltpu.bitcast(ocs[-1][0:mrows // 2, :], i32) & z[0:mrows // 2, :]
                            xb = xn_v[half(r0, mrows), :] | pltpu.bitcast(jnp.concatenate([w] * (D // 128), axis=1), jnp.uint32)
                            g_v[pl.ds(pl.multiple_of(r0, 16), mrows), :] = _silu(pltpu.bitcast(xb, bf16).astype(f32))
                        o = oc if o is None else o + oc
                        if tail and c in extra_d and pend and moe_done is not None and j >= moe_done + e_lag:
                            u, od = pend.pop(0)
                            oproj(*u, od, final=True)
                s_prev = s_list
                q = q_next
                if j + 1 < n:
                    m_prev = fin_m(mrun) if do_b else None
                    o_done = fin_o(o, lrun)
            if tail:
                pend.append((unit(n - 1), fin_o(o, lrun)))
                for u, od in pend:
                    oproj(*u, od, final=True)
                return
            for c in range(nch):
                s_c[:, c * kc:(c + 1) * kc] = s_prev[c]
            q_c[...] = q
            m_c[...] = mrun
            o_c[...] = o
            l_c[...] = lrun

        assert hpb == 1
        pro = [cp_wq(0, 1), cp_k(0, 1), cp_v(0, 0), cp_wo(0, 0), cp_wq(1, 0), cp_k(1, 0)]
        cp_ql = pltpu.make_async_copy(wq_hbm.at[:, pl.ds((H - 1) * DH, DH)], wql_v, sem_h.at[5])
        cp_x(0).start()
        if preq:
            cp_ql.start()
        for c in range(1, win):
            cp_x(c).start()
        r_v[...] = jnp.zeros((16, 128), f32)
        o_c[...] = jnp.zeros((ts, DH), f32)
        l_c[...] = jnp.ones((ts, 128), f32)

        def zero_body(c, _):
            acc[pl.ds(pl.multiple_of(c * 64, 64), 64), :] = jnp.zeros((64, D), f32)
            return 0
        lax.fori_loop(0, S // 64, zero_body, 0)

        def post_chunk(c):
            rs = r_v[...]
            for t in range(upc):
                rs = rs + router(c * upc + t)
            if preq:
                rows = pl.ds(c * xc, xc) if isinstance(c, int) else pl.ds(pl.multiple_of(c * xc, xc), xc)
                q = jnp.dot(xn_ld(c * xc, xc), wql_v[...], preferred_element_type=f32)
                ql_v[rows, :] = (q * (DH ** -0.5 * LOG2E)).astype(bf16)
            return rs

        def ln_chunk(c, zs):
            n = xc // lnsub
            for t in range(lnsub):
                r0 = c * xc + t * n
                rows = pl.ds(r0, n) if isinstance(c, int) else pl.ds(pl.multiple_of(r0, n), n)

                def ld(i):
                    if i == 0 or not reload:
                        return x_v[rows, :]
                    return x_v[pl.ds(pl.multiple_of(r0 + zs * i, n), n), :]
                xn = _layernorm(ld, numround)
                xn_v[half(r0, n), :] = pltpu.bitcast(xn, jnp.uint32)
                if gmode == 'ln':
                    g_v[rows, :] = _silu(xn.astype(f32))

        with scope('ln'):
            cp_x(0).wait()
            cp_x(win).start()
            t0 = x_v[0:16, 0:128].astype(f32)[0:8, :]
            t0 = jnp.where(jnp.abs(t0) < 1.0, t0, 0.5)
            zv = pltpu.bitcast(t0 - t0, i32)
            z_v[0:8, :] = zv
            zs = zv[0, 0]
            ln_chunk(0, zs)
            if preq:
                cp_ql.wait()

            def ln_body(c, _):
                cp_x(c).wait()

                @pl.when(c + win < nxc)
                def _():
                    cp_x(c + win).start()
                for i in range(len(pro)):
                    @pl.when(c == osched[i])
                    def _():
                        pro[i].start()
                r_v[...] = post_chunk(c - 1)
                ln_chunk(c, zs)
                return 0
            lax.fori_loop(1, nxc, ln_body, 0)
        with scope('pro'):
            pro[0].wait()
            pro[1].wait()
            topk(post_chunk(nxc - 1))
            q0 = qproj(0, 0)
            s0 = lax.dot_general(q0, k_v[0], NT, preferred_element_type=f32)
            s_c[...] = s0
            m_c[...] = _fold(s0, jnp.maximum)
            q_c[...] = qproj(0, 1)
            if gmode == 'pro':
                g_v[...] = _silu(xn_ld(0, S).astype(f32))
        if gmode == 'wait':
            with scope('gate'):
                def gate_body(c, _):
                    g_v[pl.ds(pl.multiple_of(c * grows, grows), grows), :] = _silu(xn_ld(c * grows, grows).astype(f32))
                    return 0
                lax.fori_loop(0, S // grows, gate_body, 0)
        with scope('wpro'):
            for i in range(2, len(pro)):
                pro[i].wait()

        def body(it, _):
            h0 = it * hpb

            def nxt(do):
                for i in range(hpb):
                    hv = h0 + hpb + i
                    if (nloop - 1) * hpb + hpb + i < H:
                        do(cp_v(hv, i))
                        do(cp_wo(hv, i))
                    else:
                        @pl.when(hv < H)
                        def _():
                            do(cp_v(hv, i))
                            do(cp_wo(hv, i))
                    if (nloop - 1) * hpb + hpb + i + 1 < H:
                        do(cp_wq(hv + 1, i))
                        do(cp_k(hv + 1, i))
                    else:
                        @pl.when(hv + 1 < H)
                        def _():
                            do(cp_wq(hv + 1, i))
                            do(cp_k(hv + 1, i))

            def hook():
                nxt(lambda cp: cp.start())

                @pl.when(it == 1)
                def _():
                    for i in range(3):
                        cp_f(i).start()
            with scope('mid'):
                run_slots(h0, hpb, False, hook)
            nxt(lambda cp: cp.wait())
            return 0

        lax.fori_loop(0, nloop, body, 0)
        for i in range(3):
            cp_f(i).wait()
        with scope('last'):
            if nolast:
                def ep(c, _):
                    rows = pl.ds(pl.multiple_of(c * 16, 16), 16)
                    out_v[rows, :] = (acc[rows, :] * g_v[rows, :] + xs_v[...] * idx_s[c % 8].astype(f32)
                                      + ms_v[:, 0:1] + s_c[0:16, 0:640] + o_c[0:16, 0:1] + l_c[0:16, 0:1]
                                      + m_c[0:16, 0:1] + q_c[0:16, 0:1] + r_v[:, 0:1]).astype(bf16)
                    return 0
                lax.fori_loop(0, S // 16, ep, 0)
                for c in range(noc):
                    cp_o(c).start()
            else:
                run_slots(nloop * hpb, nlast, True)
        with scope('wout'):
            for c in range(noc):
                cp_o(c).wait()

    anyspec = pl.BlockSpec(memory_space=pl.ANY)
    out = pl.pallas_call(
        kernel,
        in_specs=[anyspec, anyspec, anyspec, anyspec, anyspec,
                  pl.BlockSpec(memory_space=pltpu.VMEM),
                  anyspec, anyspec, anyspec],
        out_specs=anyspec,
        out_shape=jax.ShapeDtypeStruct((S, D), bf16),
        scratch_shapes=[
            pltpu.VMEM((zrows, 128), i32),
            pltpu.VMEM((S, D), bf16),
            pltpu.VMEM((S // 2, D), jnp.uint32),
            pltpu.VMEM((S, D), f32),
            pltpu.VMEM((H, S, DH), bf16),
            pltpu.VMEM((H, S, DH), bf16),
            pltpu.VMEM((H, D, DH), bf16),
            pltpu.VMEM((H, DH, D), bf16),
            pltpu.VMEM((F, D), bf16),
            pltpu.VMEM((F, D), bf16),
            pltpu.VMEM((F, D), bf16),
            pltpu.VMEM((S, D), f32),
            pltpu.VMEM((16, 128), f32),
            pltpu.VMEM((16, D), f32),
            pltpu.VMEM((16, 128), f32),
            pltpu.SMEM((C,), i32),
            pltpu.VMEM((ts, S), f32),
            pltpu.VMEM((ts, 128), f32),
            pltpu.VMEM((ts, DH), bf16),
            pltpu.VMEM((ts, DH), f32),
            pltpu.VMEM((ts, 128), f32),
            pltpu.VMEM((S, D), bf16),
            pltpu.VMEM((S, DH), bf16),
            pltpu.VMEM((D, DH), bf16),
            pltpu.SemaphoreType.DMA((nxc,)),
            pltpu.SemaphoreType.DMA((4 * (hpb + 1),)),
            pltpu.SemaphoreType.DMA((3,)),
            pltpu.SemaphoreType.DMA((noc,)),
        ],
        compiler_params=pltpu.CompilerParams(vmem_limit_bytes=120 * 1024 * 1024, disable_bounds_checks=True),
    )(x2, k3, v3, A_wq, A_wo, B_w_r, B_w_gate.T, B_w_up.T, B_w_down)
    return out.reshape(1, S, D)


@jax.jit
def pallas_recurrent_scan__mha_block_cached__moe_arch_mod__prompt_kernel(
        A_x, A_k_cache, A_v_cache, A_wq, A_wo, B_x, B_w_r, B_w_gate, B_w_up, B_w_down):
    return build(A_x, A_k_cache, A_v_cache, A_wq, A_wo, B_x, B_w_r, B_w_gate, B_w_up, B_w_down)
```

```python
import functools
import jax
import jax.numpy as jnp
from jax import lax
import jax.experimental.pallas as pl
import jax.experimental.pallas.tpu as pltpu

S, D, H, DH, F, C = 2048, 640, 32, 128, 1728, 8
LOG2E = 1.4426950408889634
bf16 = jnp.bfloat16
f32 = jnp.float32
i32 = jnp.int32
u32 = jnp.uint32
NT = (((1,), (1,)), ((), ()))


class _NoScope:
    def __init__(self, name):
        pass

    def __enter__(self):
        return self

    def __exit__(self, *a):
        return False


def _rb(x):
    return x.astype(bf16).astype(f32)


def _layernorm(ld, zv=None):
    mean = jnp.sum(ld(0).astype(f32), axis=-1, keepdims=True) * (1.0 / D)
    c = ld(1).astype(f32) - mean
    ssq = jnp.sum(c * c, axis=-1, keepdims=True)
    n = ssq.shape[0]
    ng = n // 8
    t = jnp.broadcast_to(ssq, (n, 128)).reshape(ng, 8, 128)
    lane = lax.broadcasted_iota(i32, (8, 128), 1)
    bit = 1
    while t.shape[0] > 1:
        hlf = t.shape[0] // 2
        t = jnp.where(((lane & bit) != 0)[None], t[hlf:], t[:hlf])
        bit *= 2
    den = _rb(jnp.sqrt(_rb(_rb(t[0] * (1.0 / D)) + 1e-5)))
    inv = pl.reciprocal(den, approx=True)
    inv = inv * (2.0 - den * inv)
    nb = ng.bit_length() - 1
    cols = []
    for g in range(ng):
        lg = int(format(g, '0%db' % nb)[::-1], 2)
        cols.append(jnp.broadcast_to(inv[:, lg:lg + 1], (8, 128)))
    inv = jnp.concatenate(cols, axis=0)
    mb = jnp.broadcast_to(_rb(mean), (n, 128))
    if zv is not None:
        mb = mb + pltpu.bitcast(pltpu.bitcast(inv, i32) & jnp.concatenate([zv] * ng, axis=0), f32)
    x = ld(2).astype(f32)
    return [pltpu.bitcast((_rb(x[:, t * 128:(t + 1) * 128] - mb) * inv).astype(bf16), u32) for t in range(D // 128)]


def _silu(x):
    hx = 0.5 * x
    return hx + hx * jnp.tanh(hx)


def _fold(x, op):
    r = x[:, 0:128]
    for t in range(1, x.shape[1] // 128):
        r = op(r, x[:, t * 128:(t + 1) * 128])
    return r


def build(A_x, A_k_cache, A_v_cache, A_wq, A_wo, B_x, B_w_r, B_w_gate, B_w_up, B_w_down,
          order="A B0 D C0 B1 C1 B2 C2 B3 C3", lorder="B0 D C0 B1 C1 B2 C2 B3 C3 A", norder="C0 C1 D C2 X C3",
          thr=1, thrl=2, xthr=True, mdl=2, pmode=0, mch=(0, 2), x0=1, L=7, win=4, dsched=None,
          e_lag=0, extra_d=(3,), hold=1, scopes=False, zrows=56, nolast=False, nomid=False,
          dma_slot=4, mrows=80, gtie=3, fdelay=9, tk_last=True, rbc=False, lateds=False, lnfirst=False, ntie=False, x2extra=2, kdelay=None, x2early=False, apos=(0, 2), rgrp=(4, 4, 2, 0), g1=4, g2=4,
          ocuts=(2, 4, 6, 8, 10, 12, 14, 15, 16)):
    ts, kc, nxc = 128, 512, 8
    nsub = S // ts
    nch = S // kc
    nf = (F + 127) // 128
    xc = S // nxc
    upc = xc // ts
    assert L % 2 == 1
    na0 = (L + 1) // upc
    x2 = A_x.reshape(S, D)
    k3 = A_k_cache.reshape(H, S, DH)
    v3 = A_v_cache.reshape(H, S, DH)
    order = order.split()
    lorder = lorder.split()
    norder = norder.split()
    noc = len(ocuts)
    scope = jax.named_scope if scopes else _NoScope
    if dsched is None:
        dsched = dict(wql=2, v0=5, wo0=5, wq1=6, k1=6)

    def kernel(x_hbm, k_hbm, v_hbm, wq_hbm, wo_hbm, wr_ref, wg_hbm, wu_hbm, wd_hbm, o_hbm,
               z_v, x_v, xn_v, g_v, k_v, v_v, wq_v, wo_v, wg_v, wu_v, wd_v, acc, r_v, xs_v, ms_v, idx_s,
               s_c, m_c, q_c, o_c, l_c, out_v, ql_v,
               sem_x, sem_h, sem_f, sem_o):
        def cp_x(c):
            rows = pl.ds(c * xc, xc) if isinstance(c, int) else pl.ds(pl.multiple_of(c * xc, xc), xc)
            return pltpu.make_async_copy(x_hbm.at[rows, :], x_v.at[rows, :], sem_x.at[c])

        def hoff(h):
            return h * DH if isinstance(h, int) else pl.multiple_of(h * DH, DH)

        def cp_k(h, i=0):
            return pltpu.make_async_copy(k_hbm.at[h], k_v.at[h], sem_h.at[i])

        def cp_v(h):
            return pltpu.make_async_copy(v_hbm.at[h], v_v.at[h], sem_h.at[1])

        def cp_wq(h, i=2):
            return pltpu.make_async_copy(wq_hbm.at[:, pl.ds(hoff(h), DH)], wq_v.at[h], sem_h.at[i])

        def cp_wo(h):
            return pltpu.make_async_copy(wo_hbm.at[pl.ds(hoff(h), DH), :], wo_v.at[h], sem_h.at[3])

        def cp_f(i):
            return pltpu.make_async_copy((wg_hbm, wu_hbm, wd_hbm)[i], (wg_v, wu_v, wd_v)[i], sem_f.at[i])

        def cp_o(c):
            lo = ocuts[c - 1] if c else 0
            rows = pl.ds(lo * ts, (ocuts[c] - lo) * ts)
            return pltpu.make_async_copy(out_v.at[rows, :], o_hbm.at[rows, :], sem_o.at[c])

        def sub(j):
            return pl.ds(j * ts, ts) if isinstance(j, int) else pl.ds(pl.multiple_of(j * ts, ts), ts)

        def half(r0, n):
            if isinstance(r0, int):
                return pl.ds(r0 // 2, n // 2)
            return pl.ds(pl.multiple_of(r0 // 2, 8), n // 2)

        def wld(ref, h, r0, n):
            if not rbc:
                return ref[h, r0:r0 + n, :]
            return pltpu.bitcast(ref.bitcast(u32)[h, r0 // 2:(r0 + n) // 2, :], bf16)

        def xn_ld(r0, n):
            return pltpu.bitcast(xn_v[half(r0, n), :], bf16)

        def router(u):
            wrf = jnp.broadcast_to(wr_ref[...].astype(f32).reshape(1, D), (16, D))
            lhs = jnp.where(lax.broadcasted_iota(i32, (16, D), 0) == u, wrf, 0.0).astype(bf16)
            return lax.dot_general(lhs, xn_ld(u * 128, 128), NT, preferred_element_type=f32)

        def qscale(q):
            return (q * (DH ** -0.5 * LOG2E)).astype(bf16)

        def qproj(h, j):
            return qscale(jnp.dot(xn_ld(j * ts, ts), wld(wq_v, h, 0, D), preferred_element_type=f32))

        def oproj(h, j, o, final=False, fresh=None):
            y = jnp.dot(o, wo_v[h], preferred_element_type=f32)
            if final:
                t = (acc[sub(j), :] + y) * g_v[sub(j), :]
                out_v[sub(j), :] = (x_v[sub(j), :].astype(f32) + t).astype(bf16)
                if (j + 1) in ocuts:
                    cp_o(ocuts.index(j + 1)).start()
            elif fresh is not None:
                acc[sub(j), :] = jnp.where(fresh, 0.0, acc[sub(j), :]) + y
            else:
                acc[sub(j), :] += y

        def fin_m(mrun):
            return jnp.broadcast_to(jnp.max(mrun, axis=-1, keepdims=True), (ts, 128))

        def fin_o(o, lrun):
            l = jnp.sum(lrun, axis=-1, keepdims=True)
            return (o * pl.reciprocal(l, approx=True)).astype(bf16)

        def topk(rsum):
            r = _rb(rsum) + 0.0
            bits = lax.shift_right_logical(pltpu.bitcast(r, i32), 16)
            ordered = jnp.where(bits >= 0x8000, 0xFFFF - bits, bits + 0x8000)
            ordered = jnp.where(r != r, 0, ordered)
            sl = lax.broadcasted_iota(i32, (16, 128), 0)
            ln = lax.broadcasted_iota(i32, (16, 128), 1)
            key = pltpu.bitcast(ordered * 2048 + (2047 - (sl * 128 + ln)) + (1 << 28), f32)
            sub16 = lax.broadcasted_iota(i32, (16, D), 0)
            x_sel = jnp.zeros((16, D), f32)
            msel = jnp.zeros((16, 128), f32)
            for c in range(C):
                m = jnp.max(jnp.max(key, axis=0, keepdims=True), axis=1, keepdims=True)
                mb = jnp.broadcast_to(m, (16, 128))
                key = jnp.where(key == mb, 0.0, key)
                msel = jnp.where(sl == c, mb, msel)
                ic = (2047 - (pltpu.bitcast(mb, i32) & 2047))[0, 0]
                idx_s[c] = ic
                blk = xn_ld((ic // 16) * 16, 16).astype(f32)
                row = jnp.sum(jnp.where(sub16 == ic % 16, blk, 0.0), axis=0, keepdims=True)
                x_sel = jnp.where(sub16 == c, row, x_sel)
            o16 = lax.shift_right_logical(pltpu.bitcast(msel, i32) - (1 << 28), 11) & 0xFFFF
            rbits = jnp.where(o16 >= 0x8000, o16 - 0x8000, 0xFFFF - o16)
            r_sel = jnp.where(sl < C, pltpu.bitcast(lax.shift_left(rbits, 16), f32), 0.0)
            ms_v[...] = _rb(0.5 + 0.5 * jnp.tanh(0.5 * r_sel))
            xs_v[...] = x_sel

        def ffn():
            if tk_last:
                topk(r_v[...])
            x_sel = xs_v[...]
            xs = x_sel.astype(bf16)
            for _ in range(fdelay):
                yield
            cnt = 0
            hs = []
            for t in range(nf):
                fs = slice(t * 128, min((t + 1) * 128, F))
                hh = []
                for w_v in (wg_v, wu_v):
                    a = None
                    for kt in range(D // 128):
                        ks = slice(kt * 128, (kt + 1) * 128)
                        d = lax.dot_general(xs[:, ks], w_v[fs, ks], NT, preferred_element_type=f32)
                        a = d if a is None else a + d
                        cnt += 1
                        if cnt % g1 == 0:
                            yield
                    hh.append(_rb(a))
                hs.append((_rb(_silu(hh[0])) * hh[1]).astype(bf16))
            cnt = 0
            ys = [None] * (D // 128)
            for t in range(nf):
                fs = slice(t * 128, min((t + 1) * 128, F))
                for kt in range(D // 128):
                    d = jnp.dot(hs[t], wd_v[fs, kt * 128:(kt + 1) * 128], preferred_element_type=f32)
                    ys[kt] = d if ys[kt] is None else ys[kt] + d
                    cnt += 1
                    if cnt % g2 == 0:
                        yield
            y = jnp.concatenate(ys, axis=1)
            y = _rb(_rb(y) * jnp.concatenate([ms_v[...]] * (D // 128), axis=1))
            gsel = _silu(_rb(x_sel + y))
            for c in range(C):
                g_v[pl.ds(jnp.clip(idx_s[c], 0, S - 1), 1), :] = gsel[c:c + 1, :]

        def run_slots(h, tail, hook=None):
            n = nsub

            def unit(t):
                if t < 0:
                    return (h - 1 if tail else jnp.maximum(h - 1, 0)), t + nsub
                return h + t // nsub, t % nsub

            z = jnp.concatenate([z_v[0:8, :]] * (ts // 8), axis=0)
            svals = {}
            mvals = {}
            q = pltpu.bitcast(q_c[...], bf16)
            o_done = fin_o(o_c[...], l_c[...])
            pend = []
            ocs = []
            mhist = []
            moe_gen = ffn() if tail else None
            moe_done = None

            def flush():
                if moe_done is not None and j >= moe_done + e_lag and len(pend) > hold:
                    u, od = pend.pop(0)
                    oproj(*u, od, final=True)

            for j in range(n):
                tb = j + L
                kb = unit(tb)[0]
                s_list = [None] * nch
                mrun = None
                lrun = None
                o = None
                q_next = None
                do_a = not (tail and tb + 1 >= n)
                do_b = not (tail and tb >= n)
                m_prev = fin_m(m_c[j] if j < L else mvals.pop(j))
                if do_b and not xthr:
                    ocs = []
                if hook is not None and j == dma_slot:
                    hook()
                for op in ((lorder if do_b else norder) if tail else order):
                    if moe_gen is not None and op[0] in 'BC':
                        try:
                            next(moe_gen)
                        except StopIteration:
                            moe_gen = None
                            moe_done = j
                    if op == 'A':
                        if do_a:
                            q_next = pltpu.bitcast(ql_v[half((tb + 1) * ts, ts), :], bf16) if tail else qproj(*unit(tb + 1))
                    elif op == 'D':
                        if tail and j > 0:
                            pend.append((unit(j - 1), o_done))
                            flush()
                        else:
                            oproj(*unit(j - 1), o_done, fresh=None if tail else (h == 0))
                    elif op == 'X':
                        flush()
                    elif op[0] == 'B':
                        c = int(op[1:])
                        cs = slice(c * kc, (c + 1) * kc)
                        qq = q
                        if mdl and len(mhist) >= mdl and c in mch:
                            w = pltpu.bitcast(mhist[len(mhist) - mdl], i32)
                            w = (w[0:ts // 2, :] | w[ts // 2:, :]) & z[0:ts // 2, :]
                            qq = pltpu.bitcast(pltpu.bitcast(q, i32) | w, bf16)
                        s = lax.dot_general(qq, wld(k_v, kb, c * kc, kc), NT, preferred_element_type=f32)
                        if tb >= n:
                            s_c[tb - n, :, cs] = s
                        s_list[c] = s
                        mc = _fold(s, jnp.maximum)
                        mrun = mc if mrun is None else jnp.maximum(mrun, mc)
                        mhist.append(mrun)
                    elif op[0] == 'C':
                        c = int(op[1:])
                        cs = slice(c * kc, (c + 1) * kc)
                        sp = s_c[j, :, cs] if j < L else svals[j][c]
                        m_use = m_prev
                        th = thr if do_b else thrl
                        if do_b and c == 0:
                            th = x0
                        if th and len(ocs) >= th:
                            m_use = m_prev + pltpu.bitcast(pltpu.bitcast(ocs[len(ocs) - th], i32) & z, f32)
                        p = jnp.exp2(sp - jnp.concatenate([m_use] * (kc // 128), axis=1))
                        if pmode == 0:
                            pb = p.astype(bf16)
                            pbs = [pb[:, t * 128:(t + 1) * 128] for t in range(kc // 128)]
                            lc = _fold(p, jnp.add)
                        elif pmode == 1:
                            pbs = [p[:, t * 128:(t + 1) * 128].astype(bf16) for t in range(kc // 128)]
                            lc = _fold(p, jnp.add)
                        elif pmode == 2:
                            pb = pltpu.bitcast(pltpu.bitcast(p.astype(bf16), u32), bf16)
                            pbs = [pb[:, t * 128:(t + 1) * 128] for t in range(kc // 128)]
                            lc = _fold(pb.astype(f32), jnp.add)
                        elif pmode == 3:
                            pb = pltpu.bitcast(pltpu.bitcast(p.astype(bf16), u32), bf16)
                            pbs = [pb[:, t * 128:(t + 1) * 128] for t in range(kc // 128)]
                            lc = _fold(p, jnp.add)
                        elif pmode == 4:
                            pu = pltpu.bitcast(p.astype(bf16), i32)
                            pb = pltpu.bitcast(pu, bf16)
                            pbs = [pb[:, t * 128:(t + 1) * 128] for t in range(kc // 128)]
                            w = _fold(pu, jnp.bitwise_or) & z[0:ts // 2, :]
                            lc = _fold(p, jnp.add) + pltpu.bitcast(jnp.concatenate([w, w], axis=0), f32)
                        lrun = lc if lrun is None else lrun + lc
                        parts = [jnp.dot(pbs[t], wld(v_v, h, c * kc + t * 128, 128),
                                         preferred_element_type=f32) for t in range(kc // 128)]
                        oc = (parts[0] + parts[1]) + (parts[2] + parts[3])
                        ocs.append(parts[0])
                        o = oc if o is None else o + oc
                        if not tail and j == n - 1 and c == gtie:
                            r0 = jnp.minimum(h * mrows, S - mrows)
                            w = pltpu.bitcast(ocs[-1][0:mrows // 2, :], i32) & z[0:mrows // 2, :]
                            xb = xn_v[half(r0, mrows), :] | pltpu.bitcast(jnp.concatenate([w] * (D // 128), axis=1), u32)
                            g_v[pl.ds(pl.multiple_of(r0, 16), mrows), :] = _silu(pltpu.bitcast(xb, bf16).astype(f32))
                        if tail and do_b and c in extra_d:
                            flush()
                if do_b:
                    if tb >= n:
                        m_c[tb - n] = mrun
                    else:
                        svals[tb] = s_list
                        mvals[tb] = mrun
                q = q_next
                if j + 1 < n:
                    o_done = fin_o(o, lrun)
            if tail:
                pend.append((unit(n - 1), fin_o(o, lrun)))
                for u, od in pend:
                    oproj(*u, od, final=True)
                return
            q_c[...] = pltpu.bitcast(q, u32)
            o_c[...] = o
            l_c[...] = lrun

        later = dict(wql=cp_wq(H - 1, 5), v0=cp_v(0), wo0=cp_wo(0), wq1=cp_wq(1), k1=cp_k(1))
        cp_x(0).start()
        cp_x(1).start()
        cp_wq(0, 4).start()
        r_v[...] = jnp.zeros((16, 128), f32)
        o_c[...] = jnp.zeros((ts, DH), f32)
        l_c[...] = jnp.ones((ts, 128), f32)
        if kdelay is not None:
            def idle(c, _):
                acc[pl.ds(pl.multiple_of(c * 64, 64), 64), :] = jnp.zeros((64, D), f32)
                return 0
            lax.fori_loop(0, kdelay, idle, 0)
            cp_k(0, 6).start()

        def mxu_front(c, u):
            wsel = (0 if c < na0 else H - 1) if isinstance(c, int) else jnp.where(c < na0, 0, H - 1)
            if u is not None:
                q = pltpu.bitcast(ql_v[half(u * ts, ts), :], bf16)

            def a_job(t):
                qn = qscale(jnp.dot(xn_ld((c * upc + t) * ts, ts), wld(wq_v, wsel, 0, D), preferred_element_type=f32))
                ql_v[half((c * upc + t) * ts, ts), :] = pltpu.bitcast(qn, u32)
            ap = (apos, apos) if isinstance(apos, int) else apos
            wrf = jnp.broadcast_to(wr_ref[...].astype(f32).reshape(1, D), (16, D))
            jobs = []
            for t in range(upc):
                lhs = jnp.where(lax.broadcasted_iota(i32, (16, D), 0) == c * upc + t, wrf, 0.0).astype(bf16)
                xn = xn_ld((c * upc + t) * ts, ts)
                jobs += [(lhs[:, k * 128:(k + 1) * 128], xn[:, k * 128:(k + 1) * 128]) for k in range(D // 128)]
            rs = r_v[...]
            mrun = None
            for cc in range(nch + 1):
                for t in range(upc):
                    if ap[t] == cc:
                        a_job(t)
                if cc == nch:
                    break
                if u is not None:
                    cs = slice(cc * kc, (cc + 1) * kc)
                    s = lax.dot_general(q, wld(k_v, 0, cc * kc, kc), NT, preferred_element_type=f32)
                    s_c[u, :, cs] = s
                    mc = _fold(s, jnp.maximum)
                    mrun = mc if mrun is None else jnp.maximum(mrun, mc)
                for _ in range(rgrp[cc]):
                    a, b = jobs.pop(0)
                    rs = rs + lax.dot_general(a, b, NT, preferred_element_type=f32)
            if u is not None:
                m_c[u] = mrun
            r_v[...] = rs

        def ln_chunk(c, zs):
            r0 = c * xc

            def ld(i):
                if i == 0:
                    return x_v[pl.ds(r0, xc) if isinstance(c, int) else pl.ds(pl.multiple_of(r0, xc), xc), :]
                return x_v[pl.ds(pl.multiple_of(r0 + zs * i, xc), xc), :]
            for t, w in enumerate(_layernorm(ld, z_v[0:8, :] if ntie else None)):
                xn_v[half(r0, xc), t * 128:(t + 1) * 128] = w

        with scope('wx0'):
            cp_x(0).wait()
        with scope('ln01'):
            if kdelay is None:
                cp_k(0, 6).start()
            if x2early:
                cp_x(2).start()
            t0 = x_v[0:16, 0:128].astype(f32)[0:8, :]
            t0 = jnp.where(jnp.abs(t0) < 1.0, t0, 0.5)
            zv = pltpu.bitcast(t0 - t0, i32)
            z_v[0:8, :] = zv
            zs = zv[0, 0]
            ln_chunk(0, zs)
            cp_x(1).wait()
            cp_wq(0, 4).wait()
            for c in range(3 if x2early else 2, 3 + x2extra):
                cp_x(c).start()
            for k, cp in later.items():
                if dsched[k] == 1:
                    cp.start()
            mxu_front(0, None)
            ln_chunk(1, zs)
            cp_k(0, 6).wait()
        with scope('ln'):
            def ln_body(c, _):
                cp_x(c).wait()

                @pl.when(c == na0 + 1)
                def _():
                    later['wql'].wait()

                def starts():
                    @pl.when(c + win - 1 < nxc)
                    def _():
                        cp_x(c + win - 1).start()

                    @pl.when(c == 2)
                    def _():
                        for cc in range(3 + x2extra, 1 + win):
                            cp_x(cc).start()
                    for k, cp in later.items():
                        if dsched[k] > 1:
                            @pl.when(c == dsched[k])
                            def _():
                                cp.start()
                if not lateds:
                    starts()
                with scope('lnit'):
                    if lnfirst:
                        ln_chunk(c, zs)
                    mxu_front(c - 1, jnp.minimum(c - 2, L - 1))
                    if not lnfirst:
                        ln_chunk(c, zs)
                if lateds:
                    starts()
                return 0
            lax.fori_loop(2, nxc, ln_body, 0)
        with scope('pro'):
            mxu_front(nxc - 1, nxc - 2 if L > nxc - 2 else None)
            if not tk_last:
                topk(r_v[...])
            q_c[...] = ql_v[half(L * ts, ts), :]
        with scope('wpro'):
            for k in ('v0', 'wo0', 'wq1', 'k1'):
                later[k].wait()

        def body(h, _):
            def nxt(do):
                do(cp_v(h + 1))
                do(cp_wo(h + 1))

                @pl.when(h + 2 < H - 1)
                def _():
                    do(cp_wq(h + 2))

                @pl.when(h + 2 < H)
                def _():
                    do(cp_k(h + 2))

            def hook():
                nxt(lambda cp: cp.start())

                @pl.when(h == 1)
                def _():
                    for i in range(3):
                        cp_f(i).start()
            with scope('mid'):
                if nomid:
                    hook()
                else:
                    run_slots(h, False, hook)
            nxt(lambda cp: cp.wait())
            return 0

        lax.fori_loop(0, H - 1, body, 0)
        for i in range(3):
            cp_f(i).wait()
        with scope('last'):
            if nolast:
                def ep(c, _):
                    rows = pl.ds(pl.multiple_of(c * 16, 16), 16)
                    out_v[rows, :] = (acc[rows, :] * g_v[rows, :] + xs_v[...] * idx_s[c % 8].astype(f32)
                                      + ms_v[:, 0:1] + s_c[c % L, 0:16, 0:640] + o_c[0:16, 0:1] + l_c[0:16, 0:1]
                                      + m_c[c % L, 0:16, 0:1] + pltpu.bitcast(q_c[0:16, 0:128], f32)[:, 0:1] + pltpu.bitcast(ql_v[pl.ds(pl.multiple_of((c % 64) * 16, 16), 16), :], f32)[:, 0:1]).astype(bf16)
                    return 0
                lax.fori_loop(0, S // 16, ep, 0)
                for c in range(noc):
                    cp_o(c).start()
            else:
                run_slots(H - 1, True)
        with scope('wout'):
            for c in range(noc):
                cp_o(c).wait()

    anyspec = pl.BlockSpec(memory_space=pl.ANY)
    out = pl.pallas_call(
        kernel,
        in_specs=[anyspec, anyspec, anyspec, anyspec, anyspec,
                  pl.BlockSpec(memory_space=pltpu.VMEM),
                  anyspec, anyspec, anyspec],
        out_specs=anyspec,
        out_shape=jax.ShapeDtypeStruct((S, D), bf16),
        scratch_shapes=[
            pltpu.VMEM((zrows, 128), i32),
            pltpu.VMEM((S, D), bf16),
            pltpu.VMEM((S // 2, D), u32),
            pltpu.VMEM((S, D), f32),
            pltpu.VMEM((H, S, DH), bf16),
            pltpu.VMEM((H, S, DH), bf16),
            pltpu.VMEM((H, D, DH), bf16),
            pltpu.VMEM((H, DH, D), bf16),
            pltpu.VMEM((F, D), bf16),
            pltpu.VMEM((F, D), bf16),
            pltpu.VMEM((F, D), bf16),
            pltpu.VMEM((S, D), f32),
            pltpu.VMEM((16, 128), f32),
            pltpu.VMEM((16, D), f32),
            pltpu.VMEM((16, 128), f32),
            pltpu.SMEM((C,), i32),
            pltpu.VMEM((L, ts, S), f32),
            pltpu.VMEM((L, ts, 128), f32),
            pltpu.VMEM((ts // 2, DH), u32),
            pltpu.VMEM((ts, DH), f32),
            pltpu.VMEM((ts, 128), f32),
            pltpu.VMEM((S, D), bf16),
            pltpu.VMEM((S // 2, DH), u32),
            pltpu.SemaphoreType.DMA((nxc,)),
            pltpu.SemaphoreType.DMA((7,)),
            pltpu.SemaphoreType.DMA((3,)),
            pltpu.SemaphoreType.DMA((noc,)),
        ],
        compiler_params=pltpu.CompilerParams(vmem_limit_bytes=120 * 1024 * 1024, disable_bounds_checks=True,
                                             disable_semaphore_checks=True),
    )(x2, k3, v3, A_wq, A_wo, B_w_r, B_w_gate.T, B_w_up.T, B_w_down)
    return out.reshape(1, S, D)


@jax.jit
def pallas_recurrent_scan__mha_block_cached__moe_arch_mod__prompt_kernel(
        A_x, A_k_cache, A_v_cache, A_wq, A_wo, B_x, B_w_r, B_w_gate, B_w_up, B_w_down):
    return build(A_x, A_k_cache, A_v_cache, A_wq, A_wo, B_x, B_w_r, B_w_gate, B_w_up, B_w_down)
```

```python
import functools
import jax
import jax.numpy as jnp
from jax import lax
import jax.experimental.pallas as pl
import jax.experimental.pallas.tpu as pltpu

S, D, H, DH, F, C = 2048, 640, 32, 128, 1728, 8
LOG2E = 1.4426950408889634
bf16 = jnp.bfloat16
f32 = jnp.float32
i32 = jnp.int32
u32 = jnp.uint32
NT = (((1,), (1,)), ((), ()))


class _NoScope:
    def __init__(self, name):
        pass

    def __enter__(self):
        return self

    def __exit__(self, *a):
        return False


def _rb(x):
    return x.astype(bf16).astype(f32)


def _layernorm(ld, zv=None):
    mean = jnp.sum(ld(0).astype(f32), axis=-1, keepdims=True) * (1.0 / D)
    c = ld(1).astype(f32) - mean
    ssq = jnp.sum(c * c, axis=-1, keepdims=True)
    n = ssq.shape[0]
    ng = n // 8
    t = jnp.broadcast_to(ssq, (n, 128)).reshape(ng, 8, 128)
    lane = lax.broadcasted_iota(i32, (8, 128), 1)
    bit = 1
    while t.shape[0] > 1:
        hlf = t.shape[0] // 2
        t = jnp.where(((lane & bit) != 0)[None], t[hlf:], t[:hlf])
        bit *= 2
    den = _rb(jnp.sqrt(_rb(_rb(t[0] * (1.0 / D)) + 1e-5)))
    inv = pl.reciprocal(den, approx=True)
    inv = inv * (2.0 - den * inv)
    nb = ng.bit_length() - 1
    cols = []
    for g in range(ng):
        lg = int(format(g, '0%db' % nb)[::-1], 2)
        cols.append(jnp.broadcast_to(inv[:, lg:lg + 1], (8, 128)))
    inv = jnp.concatenate(cols, axis=0)
    mb = jnp.broadcast_to(_rb(mean), (n, 128))
    if zv is not None:
        mb = mb + pltpu.bitcast(pltpu.bitcast(inv, i32) & jnp.concatenate([zv] * ng, axis=0), f32)
    x = ld(2).astype(f32)
    return [pltpu.bitcast((_rb(x[:, t * 128:(t + 1) * 128] - mb) * inv).astype(bf16), u32) for t in range(D // 128)]


def _silu(x):
    hx = 0.5 * x
    return hx + hx * jnp.tanh(hx)


def _fold(x, op):
    r = x[:, 0:128]
    for t in range(1, x.shape[1] // 128):
        r = op(r, x[:, t * 128:(t + 1) * 128])
    return r


def build(A_x, A_k_cache, A_v_cache, A_wq, A_wo, B_x, B_w_r, B_w_gate, B_w_up, B_w_down,
          order="A B0 D C0 B1 C1 B2 C2 B3 C3", lorder="B0 D C0 B1 C1 B2 C2 B3 C3 A", norder="C0 X C1 D C2 X C3",
          thr=1, thrl=2, xthr=True, mdl=2, pmode=0, mch=(0, 2), x0=1, L=7, win=4, dsched=None,
          e_lag=0, extra_d=(1, 3), hold=0, lsplit=2, scopes=False, zrows=56, nolast=False, nomid=False,
          dma_slot=4, mrows=80, gtie=3, fdelay=9, tk_last=True, rbc=False, lateds=False, lnfirst=False, ntie=False, x2extra=1, kdelay=None, x2early=False, blocks=((2,), (3, 4), (5, 6, 7)), fplan=None, wqlb=0, bstart=((4, 5), ('wql', 6, 7), ('v0', 'wo0', 'wq1', 'k1')), lnsub=4, lnsub0=2, reload=True, apos=(0, 2), rgrp=(4, 4, 2, 0), g1=4, g2=4,
          ocuts=(2, 4, 6, 8, 10, 11, 12, 13, 14, 15)):
    ts, kc, nxc = 128, 512, 8
    nsub = S // ts
    nch = S // kc
    nf = (F + 127) // 128
    xc = S // nxc
    upc = xc // ts
    assert L % 2 == 1
    na0 = (L + 1) // upc
    x2 = A_x.reshape(S, D)
    k3 = A_k_cache.reshape(H, S, DH)
    v3 = A_v_cache.reshape(H, S, DH)
    order = order.split()
    lorder = lorder.split()
    norder = norder.split()
    rcuts = [c * ts for c in ocuts] + [(nsub - 1) * ts + (i + 1) * (ts // lsplit) for i in range(lsplit)]
    noc = len(rcuts)
    scope = jax.named_scope if scopes else _NoScope
    if dsched is None:
        dsched = dict(wql=2, v0=5, wo0=5, wq1=6, k1=6)

    def kernel(x_hbm, k_hbm, v_hbm, wq_hbm, wo_hbm, wr_ref, wg_hbm, wu_hbm, wd_hbm, o_hbm,
               z_v, x_v, xn_v, g_v, k_v, v_v, wq_v, wo_v, wg_v, wu_v, wd_v, acc, r_v, xs_v, ms_v, idx_s,
               s_c, m_c, q_c, o_c, l_c, out_v, ql_v,
               sem_x, sem_h, sem_f, sem_o):
        def cp_x(c):
            rows = pl.ds(c * xc, xc) if isinstance(c, int) else pl.ds(pl.multiple_of(c * xc, xc), xc)
            return pltpu.make_async_copy(x_hbm.at[rows, :], x_v.at[rows, :], sem_x.at[c])

        def hoff(h):
            return h * DH if isinstance(h, int) else pl.multiple_of(h * DH, DH)

        def cp_k(h, i=0):
            return pltpu.make_async_copy(k_hbm.at[h], k_v.at[h], sem_h.at[i])

        def cp_v(h):
            return pltpu.make_async_copy(v_hbm.at[h], v_v.at[h], sem_h.at[1])

        def cp_wq(h, i=2):
            return pltpu.make_async_copy(wq_hbm.at[:, pl.ds(hoff(h), DH)], wq_v.at[h], sem_h.at[i])

        def cp_wo(h):
            return pltpu.make_async_copy(wo_hbm.at[pl.ds(hoff(h), DH), :], wo_v.at[h], sem_h.at[3])

        def cp_f(i):
            return pltpu.make_async_copy((wg_hbm, wu_hbm, wd_hbm)[i], (wg_v, wu_v, wd_v)[i], sem_f.at[i])

        def cp_o(c):
            lo = rcuts[c - 1] if c else 0
            rows = pl.ds(lo, rcuts[c] - lo)
            return pltpu.make_async_copy(out_v.at[rows, :], o_hbm.at[rows, :], sem_o.at[c])

        def sub(j):
            return pl.ds(j * ts, ts) if isinstance(j, int) else pl.ds(pl.multiple_of(j * ts, ts), ts)

        def half(r0, n):
            if isinstance(r0, int):
                return pl.ds(r0 // 2, n // 2)
            return pl.ds(pl.multiple_of(r0 // 2, 8), n // 2)

        def wld(ref, h, r0, n):
            if not rbc:
                return ref[h, r0:r0 + n, :]
            return pltpu.bitcast(ref.bitcast(u32)[h, r0 // 2:(r0 + n) // 2, :], bf16)

        def xn_ld(r0, n):
            return pltpu.bitcast(xn_v[half(r0, n), :], bf16)

        def router(u):
            wrf = jnp.broadcast_to(wr_ref[...].astype(f32).reshape(1, D), (16, D))
            lhs = jnp.where(lax.broadcasted_iota(i32, (16, D), 0) == u, wrf, 0.0).astype(bf16)
            return lax.dot_general(lhs, xn_ld(u * 128, 128), NT, preferred_element_type=f32)

        def qscale(q):
            return (q * (DH ** -0.5 * LOG2E)).astype(bf16)

        def qproj(h, j):
            return qscale(jnp.dot(xn_ld(j * ts, ts), wld(wq_v, h, 0, D), preferred_element_type=f32))

        def oproj(h, j, o, final=False, fresh=None):
            if final:
                npc = lsplit if j == nsub - 1 else 1
                n = ts // npc
                for i in range(npc):
                    rows = pl.ds(j * ts + i * n, n)
                    y = jnp.dot(o[i * n:(i + 1) * n, :], wo_v[h], preferred_element_type=f32)
                    t = (acc[rows, :] + y) * g_v[rows, :]
                    out_v[rows, :] = (x_v[rows, :].astype(f32) + t).astype(bf16)
                    if j * ts + (i + 1) * n in rcuts:
                        cp_o(rcuts.index(j * ts + (i + 1) * n)).start()
                return
            y = jnp.dot(o, wo_v[h], preferred_element_type=f32)
            if fresh is not None:
                acc[sub(j), :] = jnp.where(fresh, 0.0, acc[sub(j), :]) + y
            else:
                acc[sub(j), :] += y

        def fin_m(mrun):
            return jnp.broadcast_to(jnp.max(mrun, axis=-1, keepdims=True), (ts, 128))

        def fin_o(o, lrun):
            l = jnp.sum(lrun, axis=-1, keepdims=True)
            return (o * pl.reciprocal(l, approx=True)).astype(bf16)

        def topk(rsum):
            r = _rb(rsum) + 0.0
            bits = lax.shift_right_logical(pltpu.bitcast(r, i32), 16)
            ordered = jnp.where(bits >= 0x8000, 0xFFFF - bits, bits + 0x8000)
            ordered = jnp.where(r != r, 0, ordered)
            sl = lax.broadcasted_iota(i32, (16, 128), 0)
            ln = lax.broadcasted_iota(i32, (16, 128), 1)
            key = pltpu.bitcast(ordered * 2048 + (2047 - (sl * 128 + ln)) + (1 << 28), f32)
            sub16 = lax.broadcasted_iota(i32, (16, D), 0)
            x_sel = jnp.zeros((16, D), f32)
            msel = jnp.zeros((16, 128), f32)
            for c in range(C):
                m = jnp.max(jnp.max(key, axis=0, keepdims=True), axis=1, keepdims=True)
                mb = jnp.broadcast_to(m, (16, 128))
                key = jnp.where(key == mb, 0.0, key)
                msel = jnp.where(sl == c, mb, msel)
                ic = (2047 - (pltpu.bitcast(mb, i32) & 2047))[0, 0]
                idx_s[c] = ic
                blk = xn_ld((ic // 16) * 16, 16).astype(f32)
                row = jnp.sum(jnp.where(sub16 == ic % 16, blk, 0.0), axis=0, keepdims=True)
                x_sel = jnp.where(sub16 == c, row, x_sel)
            o16 = lax.shift_right_logical(pltpu.bitcast(msel, i32) - (1 << 28), 11) & 0xFFFF
            rbits = jnp.where(o16 >= 0x8000, o16 - 0x8000, 0xFFFF - o16)
            r_sel = jnp.where(sl < C, pltpu.bitcast(lax.shift_left(rbits, 16), f32), 0.0)
            ms_v[...] = _rb(0.5 + 0.5 * jnp.tanh(0.5 * r_sel))
            xs_v[...] = x_sel

        def ffn():
            if tk_last:
                topk(r_v[...])
            x_sel = xs_v[...]
            xs = x_sel.astype(bf16)
            for _ in range(fdelay):
                yield
            cnt = 0
            hs = []
            for t in range(nf):
                fs = slice(t * 128, min((t + 1) * 128, F))
                hh = []
                for w_v in (wg_v, wu_v):
                    a = None
                    for kt in range(D // 128):
                        ks = slice(kt * 128, (kt + 1) * 128)
                        d = lax.dot_general(xs[:, ks], w_v[fs, ks], NT, preferred_element_type=f32)
                        a = d if a is None else a + d
                        cnt += 1
                        if cnt % g1 == 0:
                            yield
                    hh.append(_rb(a))
                hs.append((_rb(_silu(hh[0])) * hh[1]).astype(bf16))
            cnt = 0
            ys = [None] * (D // 128)
            for t in range(nf):
                fs = slice(t * 128, min((t + 1) * 128, F))
                for kt in range(D // 128):
                    d = jnp.dot(hs[t], wd_v[fs, kt * 128:(kt + 1) * 128], preferred_element_type=f32)
                    ys[kt] = d if ys[kt] is None else ys[kt] + d
                    cnt += 1
                    if cnt % g2 == 0:
                        yield
            y = jnp.concatenate(ys, axis=1)
            y = _rb(_rb(y) * jnp.concatenate([ms_v[...]] * (D // 128), axis=1))
            gsel = _silu(_rb(x_sel + y))
            for c in range(C):
                g_v[pl.ds(jnp.clip(idx_s[c], 0, S - 1), 1), :] = gsel[c:c + 1, :]

        def run_slots(h, tail, hook=None):
            n = nsub

            def unit(t):
                if t < 0:
                    return (h - 1 if tail else jnp.maximum(h - 1, 0)), t + nsub
                return h + t // nsub, t % nsub

            z = jnp.concatenate([z_v[0:8, :]] * (ts // 8), axis=0)
            svals = {}
            mvals = {}
            q = pltpu.bitcast(q_c[...], bf16)
            o_done = fin_o(o_c[...], l_c[...])
            pend = []
            ocs = []
            mhist = []
            moe_gen = ffn() if tail else None
            moe_done = None

            def flush():
                if moe_done is not None and j >= moe_done + e_lag and len(pend) > hold:
                    u, od = pend.pop(0)
                    oproj(*u, od, final=True)

            for j in range(n):
                tb = j + L
                kb = unit(tb)[0]
                s_list = [None] * nch
                mrun = None
                lrun = None
                o = None
                q_next = None
                do_a = not (tail and tb + 1 >= n)
                do_b = not (tail and tb >= n)
                m_prev = fin_m(m_c[j] if j < L else mvals.pop(j))
                if do_b and not xthr:
                    ocs = []
                if hook is not None and j == dma_slot:
                    hook()
                for op in ((lorder if do_b else norder) if tail else order):
                    if moe_gen is not None and op[0] in 'BC':
                        try:
                            next(moe_gen)
                        except StopIteration:
                            moe_gen = None
                            moe_done = j
                    if op == 'A':
                        if do_a:
                            q_next = pltpu.bitcast(ql_v[half((tb + 1) * ts, ts), :], bf16) if tail else qproj(*unit(tb + 1))
                    elif op == 'D':
                        if tail and j > 0:
                            pend.append((unit(j - 1), o_done))
                            flush()
                        else:
                            oproj(*unit(j - 1), o_done, fresh=None if tail else (h == 0))
                    elif op == 'X':
                        flush()
                    elif op[0] == 'B':
                        c = int(op[1:])
                        cs = slice(c * kc, (c + 1) * kc)
                        qq = q
                        if mdl and len(mhist) >= mdl and c in mch:
                            w = pltpu.bitcast(mhist[len(mhist) - mdl], i32)
                            w = (w[0:ts // 2, :] | w[ts // 2:, :]) & z[0:ts // 2, :]
                            qq = pltpu.bitcast(pltpu.bitcast(q, i32) | w, bf16)
                        s = lax.dot_general(qq, wld(k_v, kb, c * kc, kc), NT, preferred_element_type=f32)
                        if tb >= n:
                            s_c[tb - n, :, cs] = s
                        s_list[c] = s
                        mc = _fold(s, jnp.maximum)
                        mrun = mc if mrun is None else jnp.maximum(mrun, mc)
                        mhist.append(mrun)
                    elif op[0] == 'C':
                        c = int(op[1:])
                        cs = slice(c * kc, (c + 1) * kc)
                        sp = s_c[j, :, cs] if j < L else svals[j][c]
                        m_use = m_prev
                        th = thr if do_b else thrl
                        if do_b and c == 0:
                            th = x0
                        if th and len(ocs) >= th:
                            m_use = m_prev + pltpu.bitcast(pltpu.bitcast(ocs[len(ocs) - th], i32) & z, f32)
                        p = jnp.exp2(sp - jnp.concatenate([m_use] * (kc // 128), axis=1))
                        if pmode == 0:
                            pb = p.astype(bf16)
                            pbs = [pb[:, t * 128:(t + 1) * 128] for t in range(kc // 128)]
                            lc = _fold(p, jnp.add)
                        elif pmode == 1:
                            pbs = [p[:, t * 128:(t + 1) * 128].astype(bf16) for t in range(kc // 128)]
                            lc = _fold(p, jnp.add)
                        elif pmode == 2:
                            pb = pltpu.bitcast(pltpu.bitcast(p.astype(bf16), u32), bf16)
                            pbs = [pb[:, t * 128:(t + 1) * 128] for t in range(kc // 128)]
                            lc = _fold(pb.astype(f32), jnp.add)
                        elif pmode == 3:
                            pb = pltpu.bitcast(pltpu.bitcast(p.astype(bf16), u32), bf16)
                            pbs = [pb[:, t * 128:(t + 1) * 128] for t in range(kc // 128)]
                            lc = _fold(p, jnp.add)
                        elif pmode == 4:
                            pu = pltpu.bitcast(p.astype(bf16), i32)
                            pb = pltpu.bitcast(pu, bf16)
                            pbs = [pb[:, t * 128:(t + 1) * 128] for t in range(kc // 128)]
                            w = _fold(pu, jnp.bitwise_or) & z[0:ts // 2, :]
                            lc = _fold(p, jnp.add) + pltpu.bitcast(jnp.concatenate([w, w], axis=0), f32)
                        lrun = lc if lrun is None else lrun + lc
                        parts = [jnp.dot(pbs[t], wld(v_v, h, c * kc + t * 128, 128),
                                         preferred_element_type=f32) for t in range(kc // 128)]
                        oc = (parts[0] + parts[1]) + (parts[2] + parts[3])
                        ocs.append(parts[0])
                        o = oc if o is None else o + oc
                        if not tail and j == n - 1 and c == gtie:
                            r0 = jnp.minimum(h * mrows, S - mrows)
                            w = pltpu.bitcast(ocs[-1][0:mrows // 2, :], i32) & z[0:mrows // 2, :]
                            xb = xn_v[half(r0, mrows), :] | pltpu.bitcast(jnp.concatenate([w] * (D // 128), axis=1), u32)
                            g_v[pl.ds(pl.multiple_of(r0, 16), mrows), :] = _silu(pltpu.bitcast(xb, bf16).astype(f32))
                        if tail and do_b and c in extra_d:
                            flush()
                if do_b:
                    if tb >= n:
                        m_c[tb - n] = mrun
                    else:
                        svals[tb] = s_list
                        mvals[tb] = mrun
                q = q_next
                if j + 1 < n:
                    o_done = fin_o(o, lrun)
            if tail:
                pend.append((unit(n - 1), fin_o(o, lrun)))
                for u, od in pend:
                    oproj(*u, od, final=True)
                return
            q_c[...] = pltpu.bitcast(q, u32)
            o_c[...] = o
            l_c[...] = lrun

        later = dict(wql=cp_wq(H - 1, 5), v0=cp_v(0), wo0=cp_wo(0), wq1=cp_wq(1), k1=cp_k(1))
        cp_x(0).start()
        cp_x(1).start()
        cp_wq(0, 4).start()
        r_v[...] = jnp.zeros((16, 128), f32)
        o_c[...] = jnp.zeros((ts, DH), f32)
        l_c[...] = jnp.ones((ts, 128), f32)
        if kdelay is not None:
            def idle(c, _):
                acc[pl.ds(pl.multiple_of(c * 64, 64), 64), :] = jnp.zeros((64, D), f32)
                return 0
            lax.fori_loop(0, kdelay, idle, 0)
            cp_k(0, 6).start()

        def mxu_front(c, u):
            wsel = (0 if c < na0 else H - 1) if isinstance(c, int) else jnp.where(c < na0, 0, H - 1)
            if u is not None:
                q = pltpu.bitcast(ql_v[half(u * ts, ts), :], bf16)

            def a_job(t):
                qn = qscale(jnp.dot(xn_ld((c * upc + t) * ts, ts), wld(wq_v, wsel, 0, D), preferred_element_type=f32))
                ql_v[half((c * upc + t) * ts, ts), :] = pltpu.bitcast(qn, u32)
            ap = (apos, apos) if isinstance(apos, int) else apos
            wrf = jnp.broadcast_to(wr_ref[...].astype(f32).reshape(1, D), (16, D))
            jobs = []
            for t in range(upc):
                lhs = jnp.where(lax.broadcasted_iota(i32, (16, D), 0) == c * upc + t, wrf, 0.0).astype(bf16)
                xn = xn_ld((c * upc + t) * ts, ts)
                jobs += [(lhs[:, k * 128:(k + 1) * 128], xn[:, k * 128:(k + 1) * 128]) for k in range(D // 128)]
            rs = r_v[...]
            mrun = None
            for cc in range(nch + 1):
                for t in range(upc):
                    if ap[t] == cc:
                        a_job(t)
                if cc == nch:
                    break
                if u is not None:
                    cs = slice(cc * kc, (cc + 1) * kc)
                    s = lax.dot_general(q, wld(k_v, 0, cc * kc, kc), NT, preferred_element_type=f32)
                    s_c[u, :, cs] = s
                    mc = _fold(s, jnp.maximum)
                    mrun = mc if mrun is None else jnp.maximum(mrun, mc)
                for _ in range(rgrp[cc]):
                    a, b = jobs.pop(0)
                    rs = rs + lax.dot_general(a, b, NT, preferred_element_type=f32)
            if u is not None:
                m_c[u] = mrun
            r_v[...] = rs

        def ln_rows(r0, n, zs):
            def ld(i):
                if i == 0 or not reload:
                    return x_v[pl.ds(r0, n), :]
                return x_v[pl.ds(pl.multiple_of(r0 + zs * i, n), n), :]
            for t, w in enumerate(_layernorm(ld, z_v[0:8, :] if ntie else None)):
                xn_v[half(r0, n), t * 128:(t + 1) * 128] = w

        def ln_chunk(c, zs):
            ns = lnsub if isinstance(lnsub, int) and c >= 2 else (lnsub0 if c < 2 else lnsub[c])
            n = xc // ns
            for t in range(ns):
                ln_rows(c * xc + t * n, n, zs)

        with scope('wx0'):
            cp_x(0).wait()
        with scope('ln01'):
            if kdelay is None:
                cp_k(0, 6).start()
            if x2early:
                cp_x(2).start()
            t0 = x_v[0:16, 0:128].astype(f32)[0:8, :]
            t0 = jnp.where(jnp.abs(t0) < 1.0, t0, 0.5)
            zv = pltpu.bitcast(t0 - t0, i32)
            z_v[0:8, :] = zv
            zs = zv[0, 0]
            ln_chunk(0, zs)
            cp_x(1).wait()
            cp_wq(0, 4).wait()
            for c in range(3 if x2early else 2, 3 + x2extra):
                cp_x(c).start()
            mxu_front(0, None)
            ln_chunk(1, zs)
            cp_k(0, 6).wait()
        def a_unit(uu):
            hsel = 0 if uu < na0 * upc else H - 1
            qn = qscale(jnp.dot(xn_ld(uu * ts, ts), wld(wq_v, hsel, 0, D), preferred_element_type=f32))
            ql_v[half(uu * ts, ts), :] = pltpu.bitcast(qn, u32)

        def r_jobs(uu):
            wrf = jnp.broadcast_to(wr_ref[...].astype(f32).reshape(1, D), (16, D))
            lhs = jnp.where(lax.broadcasted_iota(i32, (16, D), 0) == uu, wrf, 0.0).astype(bf16)
            xn = xn_ld(uu * ts, ts)
            return [(lhs[:, k * 128:(k + 1) * 128], xn[:, k * 128:(k + 1) * 128]) for k in range(D // 128)]

        plan = fplan or [
            "L2 a3 r2 a2 r3 b0.0 r3 b0.1 r2 b0.2 b0.3",
            "L3 L4 b1.0 r5 a4 a5 r5 b1.1 r4 b1.2 r4 b1.3 b2.0 r6 a6 b2.1 b2.2 r7 a7 r7 b2.3 b3.0 b3.1 r6 b3.2 b3.3",
            "L5 L6 L7 b4.0 a9 r8 a8 r9 b4.1 r9 a11 r11 b4.2 r10 a10 r8 b4.3 r10 b5.0 r12 b5.1 r13 a13 b5.2 r13 a14 r11 "
            "a12 r14 b5.3 r12 b6.0 r15 b6.1 a15 r14 b6.2 b6.3 r15",
        ]
        for bi, blk in enumerate(blocks):
            with scope('fb%d' % bi):
                for c in blk:
                    cp_x(c).wait()
                if bi == len(blocks) - 1 - wqlb:
                    later['wql'].wait()
                for k in bstart[bi]:
                    (cp_x(k) if isinstance(k, int) else later[k]).start()
                rs = r_v[...]
                rj = {}
                mr = {}
                qs = {}
                for op in plan[bi].split():
                    if op[0] == 'L':
                        ln_chunk(int(op[1:]), zs)
                    elif op[0] == 'a':
                        a_unit(int(op[1:]))
                    elif op[0] == 'r':
                        uu = int(op[1:])
                        first = uu not in rj
                        if first:
                            rj[uu] = r_jobs(uu)
                        for _ in range(3 if first else 2):
                            a, b = rj[uu].pop(0)
                            rs = rs + lax.dot_general(a, b, NT, preferred_element_type=f32)
                    elif op[0] == 'b':
                        uu, cc = (int(t) for t in op[1:].split('.'))
                        if uu not in qs:
                            qs[uu] = pltpu.bitcast(ql_v[half(uu * ts, ts), :], bf16)
                        sv = lax.dot_general(qs[uu], wld(k_v, 0, cc * kc, kc), NT, preferred_element_type=f32)
                        s_c[uu, :, cc * kc:(cc + 1) * kc] = sv
                        mc = _fold(sv, jnp.maximum)
                        mr[uu] = mc if uu not in mr else jnp.maximum(mr[uu], mc)
                        if cc == nch - 1:
                            m_c[uu] = mr[uu]
                r_v[...] = rs
        q_c[...] = ql_v[half(L * ts, ts), :]
        with scope('wpro'):
            for k in ('v0', 'wo0', 'wq1', 'k1'):
                later[k].wait()

        def body(h, _):
            def nxt(do):
                do(cp_v(h + 1))
                do(cp_wo(h + 1))

                @pl.when(h + 2 < H - 1)
                def _():
                    do(cp_wq(h + 2))

                @pl.when(h + 2 < H)
                def _():
                    do(cp_k(h + 2))

            def hook():
                nxt(lambda cp: cp.start())

                @pl.when(h == 1)
                def _():
                    for i in range(3):
                        cp_f(i).start()
            with scope('mid'):
                if nomid:
                    hook()
                else:
                    run_slots(h, False, hook)
            nxt(lambda cp: cp.wait())
            return 0

        lax.fori_loop(0, H - 1, body, 0)
        for i in range(3):
            cp_f(i).wait()
        with scope('last'):
            if nolast:
                def ep(c, _):
                    rows = pl.ds(pl.multiple_of(c * 16, 16), 16)
                    out_v[rows, :] = (acc[rows, :] * g_v[rows, :] + xs_v[...] * idx_s[c % 8].astype(f32)
                                      + ms_v[:, 0:1] + r_v[:, 0:1] + s_c[c % L, 0:16, 0:640] + o_c[0:16, 0:1] + l_c[0:16, 0:1]
                                      + m_c[c % L, 0:16, 0:1] + pltpu.bitcast(q_c[0:16, 0:128], f32)[:, 0:1] + pltpu.bitcast(ql_v[pl.ds(pl.multiple_of((c % 64) * 16, 16), 16), :], f32)[:, 0:1]).astype(bf16)
                    return 0
                lax.fori_loop(0, S // 16, ep, 0)
                for c in range(noc):
                    cp_o(c).start()
            else:
                run_slots(H - 1, True)
        with scope('wout'):
            for c in range(noc):
                cp_o(c).wait()

    anyspec = pl.BlockSpec(memory_space=pl.ANY)
    out = pl.pallas_call(
        kernel,
        in_specs=[anyspec, anyspec, anyspec, anyspec, anyspec,
                  pl.BlockSpec(memory_space=pltpu.VMEM),
                  anyspec, anyspec, anyspec],
        out_specs=anyspec,
        out_shape=jax.ShapeDtypeStruct((S, D), bf16),
        scratch_shapes=[
            pltpu.VMEM((zrows, 128), i32),
            pltpu.VMEM((S, D), bf16),
            pltpu.VMEM((S // 2, D), u32),
            pltpu.VMEM((S, D), f32),
            pltpu.VMEM((H, S, DH), bf16),
            pltpu.VMEM((H, S, DH), bf16),
            pltpu.VMEM((H, D, DH), bf16),
            pltpu.VMEM((H, DH, D), bf16),
            pltpu.VMEM((F, D), bf16),
            pltpu.VMEM((F, D), bf16),
            pltpu.VMEM((F, D), bf16),
            pltpu.VMEM((S, D), f32),
            pltpu.VMEM((16, 128), f32),
            pltpu.VMEM((16, D), f32),
            pltpu.VMEM((16, 128), f32),
            pltpu.SMEM((C,), i32),
            pltpu.VMEM((L, ts, S), f32),
            pltpu.VMEM((L, ts, 128), f32),
            pltpu.VMEM((ts // 2, DH), u32),
            pltpu.VMEM((ts, DH), f32),
            pltpu.VMEM((ts, 128), f32),
            pltpu.VMEM((S, D), bf16),
            pltpu.VMEM((S // 2, DH), u32),
            pltpu.SemaphoreType.DMA((nxc,)),
            pltpu.SemaphoreType.DMA((7,)),
            pltpu.SemaphoreType.DMA((3,)),
            pltpu.SemaphoreType.DMA((noc,)),
        ],
        compiler_params=pltpu.CompilerParams(vmem_limit_bytes=120 * 1024 * 1024, disable_bounds_checks=True,
                                             disable_semaphore_checks=True),
    )(x2, k3, v3, A_wq, A_wo, B_w_r, B_w_gate.T, B_w_up.T, B_w_down)
    return out.reshape(1, S, D)


@jax.jit
def pallas_recurrent_scan__mha_block_cached__moe_arch_mod__prompt_kernel(
        A_x, A_k_cache, A_v_cache, A_wq, A_wo, B_x, B_w_r, B_w_gate, B_w_up, B_w_down):
    return build(A_x, A_k_cache, A_v_cache, A_wq, A_wo, B_x, B_w_r, B_w_gate, B_w_up, B_w_down)
```

```python
import functools
import jax
import jax.numpy as jnp
from jax import lax
import jax.experimental.pallas as pl
import jax.experimental.pallas.tpu as pltpu

S, D, H, DH, F, C = 2048, 640, 32, 128, 1728, 8
LOG2E = 1.4426950408889634
bf16 = jnp.bfloat16
f32 = jnp.float32
i32 = jnp.int32
u32 = jnp.uint32
NT = (((1,), (1,)), ((), ()))


class _NoScope:
    def __init__(self, name):
        pass

    def __enter__(self):
        return self

    def __exit__(self, *a):
        return False


def _rb(x):
    return x.astype(bf16).astype(f32)


def _layernorm(ld, zv=None):
    mean = jnp.sum(ld(0).astype(f32), axis=-1, keepdims=True) * (1.0 / D)
    c = ld(1).astype(f32) - mean
    ssq = jnp.sum(c * c, axis=-1, keepdims=True)
    n = ssq.shape[0]
    ng = n // 8
    t = jnp.broadcast_to(ssq, (n, 128)).reshape(ng, 8, 128)
    lane = lax.broadcasted_iota(i32, (8, 128), 1)
    bit = 1
    while t.shape[0] > 1:
        hlf = t.shape[0] // 2
        t = jnp.where(((lane & bit) != 0)[None], t[hlf:], t[:hlf])
        bit *= 2
    den = _rb(jnp.sqrt(_rb(_rb(t[0] * (1.0 / D)) + 1e-5)))
    inv = pl.reciprocal(den, approx=True)
    inv = inv * (2.0 - den * inv)
    nb = ng.bit_length() - 1
    cols = []
    for g in range(ng):
        lg = int(format(g, '0%db' % nb)[::-1], 2)
        cols.append(jnp.broadcast_to(inv[:, lg:lg + 1], (8, 128)))
    inv = jnp.concatenate(cols, axis=0)
    mb = jnp.broadcast_to(_rb(mean), (n, 128))
    if zv is not None:
        mb = mb + pltpu.bitcast(pltpu.bitcast(inv, i32) & jnp.concatenate([zv] * ng, axis=0), f32)
    x = ld(2).astype(f32)
    return [pltpu.bitcast((_rb(x[:, t * 128:(t + 1) * 128] - mb) * inv).astype(bf16), u32) for t in range(D // 128)]


def _silu(x):
    hx = 0.5 * x
    return hx + hx * jnp.tanh(hx)


def _fold(x, op):
    r = x[:, 0:128]
    for t in range(1, x.shape[1] // 128):
        r = op(r, x[:, t * 128:(t + 1) * 128])
    return r


def build(A_x, A_k_cache, A_v_cache, A_wq, A_wo, B_x, B_w_r, B_w_gate, B_w_up, B_w_down,
          order="A B0 D C0 B1 C1 B2 C2 B3 C3", lorder="B0 D C0 B1 C1 B2 C2 B3 C3 A", norder="C0 C1 D C2 X C3",
          thr=1, thrl=2, xthr=True, mdl=2, pmode=0, mch=(0, 2), x0=1, L=7, win=4, dsched=None,
          e_lag=0, extra_d=(1,), hold=0, lsplit=2, scopes=False, zrows=128, isb=65536, nolast=False, nomid=False,
          dma_slot=4, mrows=80, gtie='C3', fdelay=8, tk_last=True, rbc=False, lateds=False, lnfirst=False, ntie=False, x2extra=1, kdelay=None, x2early=False, blocks=((2,), (3, 4), (5, 6, 7)), fplan=None, wqlb=0, waittop=True, bstart=((4, 5), ('wql', 6, 7), ('v0', 'wo0', 'wq1', 'k1')), lnsub=4, lnsub0=2, reload=True, apos=(0, 2), rgrp=(4, 4, 2, 0), g1=4, g2=4,
          ocuts=(2, 4, 6, 8, 10, 12, 13, 14, 15)):
    ts, kc, nxc = 128, 512, 8
    nsub = S // ts
    nch = S // kc
    nf = (F + 127) // 128
    xc = S // nxc
    upc = xc // ts
    assert L % 2 == 1
    na0 = (L + 1) // upc
    x2 = A_x.reshape(S, D)
    k3 = A_k_cache.reshape(H, S, DH)
    v3 = A_v_cache.reshape(H, S, DH)
    order = order.split()
    lorder = lorder.split()
    norder = norder.split()
    rcuts = [c * ts for c in ocuts] + [(nsub - 1) * ts + (i + 1) * (ts // lsplit) for i in range(lsplit)]
    noc = len(rcuts)
    scope = jax.named_scope if scopes else _NoScope
    if dsched is None:
        dsched = dict(wql=2, v0=5, wo0=5, wq1=6, k1=6)

    def kernel(x_hbm, k_hbm, v_hbm, wq_hbm, wo_hbm, wr_ref, wg_hbm, wu_hbm, wd_hbm, o_hbm,
               z_v, x_v, xn_v, g_v, k_v, v_v, wq_v, wo_v, wg_v, wu_v, wd_v, acc, r_v, xs_v, ms_v, idx_s,
               s_c, m_c, q_c, o_c, l_c, out_v, ql_v,
               sem_x, sem_h, sem_f, sem_o):
        def cp_x(c):
            rows = pl.ds(c * xc, xc) if isinstance(c, int) else pl.ds(pl.multiple_of(c * xc, xc), xc)
            return pltpu.make_async_copy(x_hbm.at[rows, :], x_v.at[rows, :], sem_x.at[c])

        def hoff(h):
            return h * DH if isinstance(h, int) else pl.multiple_of(h * DH, DH)

        def cp_k(h, i=0):
            return pltpu.make_async_copy(k_hbm.at[h], k_v.at[h], sem_h.at[i])

        def cp_v(h):
            return pltpu.make_async_copy(v_hbm.at[h], v_v.at[h], sem_h.at[1])

        def cp_wq(h, i=2):
            return pltpu.make_async_copy(wq_hbm.at[:, pl.ds(hoff(h), DH)], wq_v.at[h], sem_h.at[i])

        def cp_wo(h):
            return pltpu.make_async_copy(wo_hbm.at[pl.ds(hoff(h), DH), :], wo_v.at[h], sem_h.at[3])

        def cp_f(i):
            return pltpu.make_async_copy((wg_hbm, wu_hbm, wd_hbm)[i], (wg_v, wu_v, wd_v)[i], sem_f.at[i])

        def cp_o(c):
            lo = rcuts[c - 1] if c else 0
            rows = pl.ds(lo, rcuts[c] - lo)
            return pltpu.make_async_copy(out_v.at[rows, :], o_hbm.at[rows, :], sem_o.at[c])

        def sub(j):
            return pl.ds(j * ts, ts) if isinstance(j, int) else pl.ds(pl.multiple_of(j * ts, ts), ts)

        def half(r0, n):
            if isinstance(r0, int):
                return pl.ds(r0 // 2, n // 2)
            return pl.ds(pl.multiple_of(r0 // 2, 8), n // 2)

        def wld(ref, h, r0, n):
            if not rbc:
                return ref[h, r0:r0 + n, :]
            return pltpu.bitcast(ref.bitcast(u32)[h, r0 // 2:(r0 + n) // 2, :], bf16)

        def xn_ld(r0, n):
            return pltpu.bitcast(xn_v[half(r0, n), :], bf16)

        def router(u):
            wrf = jnp.broadcast_to(wr_ref[...].astype(f32).reshape(1, D), (16, D))
            lhs = jnp.where(lax.broadcasted_iota(i32, (16, D), 0) == u, wrf, 0.0).astype(bf16)
            return lax.dot_general(lhs, xn_ld(u * 128, 128), NT, preferred_element_type=f32)

        def qscale(q):
            return (q * (DH ** -0.5 * LOG2E)).astype(bf16)

        def qproj(h, j):
            return qscale(jnp.dot(xn_ld(j * ts, ts), wld(wq_v, h, 0, D), preferred_element_type=f32))

        def oproj(h, j, o, final=False, fresh=None):
            if final:
                npc = lsplit if j == nsub - 1 else 1
                n = ts // npc
                for i in range(npc):
                    rows = pl.ds(j * ts + i * n, n)
                    y = jnp.dot(o[i * n:(i + 1) * n, :], wo_v[h], preferred_element_type=f32)
                    t = (acc[rows, :] + y) * g_v[rows, :]
                    out_v[rows, :] = (x_v[rows, :].astype(f32) + t).astype(bf16)
                    if j * ts + (i + 1) * n in rcuts:
                        cp_o(rcuts.index(j * ts + (i + 1) * n)).start()
                return
            y = jnp.dot(o, wo_v[h], preferred_element_type=f32)
            if fresh is not None:
                acc[sub(j), :] = jnp.where(fresh, 0.0, acc[sub(j), :]) + y
            else:
                acc[sub(j), :] += y

        def fin_m(mrun):
            return jnp.broadcast_to(jnp.max(mrun, axis=-1, keepdims=True), (ts, 128))

        def fin_o(o, lrun):
            l = jnp.sum(lrun, axis=-1, keepdims=True)
            return (o * pl.reciprocal(l, approx=True)).astype(bf16)

        def topk(rsum):
            r = _rb(rsum) + 0.0
            bits = lax.shift_right_logical(pltpu.bitcast(r, i32), 16)
            ordered = jnp.where(bits >= 0x8000, 0xFFFF - bits, bits + 0x8000)
            ordered = jnp.where(r != r, 0, ordered)
            sl = lax.broadcasted_iota(i32, (16, 128), 0)
            ln = lax.broadcasted_iota(i32, (16, 128), 1)
            key = pltpu.bitcast(ordered * 2048 + (2047 - (sl * 128 + ln)) + (1 << 28), f32)
            msel = jnp.zeros((16, 128), f32)
            for c in range(C):
                m = jnp.max(jnp.max(key, axis=0, keepdims=True), axis=1, keepdims=True)
                mb = jnp.broadcast_to(m, (16, 128))
                key = jnp.where(key == mb, 0.0, key)
                msel = jnp.where(sl == c, mb, msel)
                ic = (2047 - (pltpu.bitcast(mb, i32) & 2047))[0, 0]
                idx_s[c] = ic
                pair = pltpu.bitcast(xn_v[pl.ds(lax.shift_right_logical(ic, 1), 1), :], i32)
                xs_v[c:c + 1, :] = pltpu.bitcast(lax.shift_left(lax.shift_right_logical(pair, (ic & 1) * 16), 16), f32)
            o16 = lax.shift_right_logical(pltpu.bitcast(msel, i32) - (1 << 28), 11) & 0xFFFF
            rbits = jnp.where(o16 >= 0x8000, o16 - 0x8000, 0xFFFF - o16)
            r_sel = jnp.where(sl < C, pltpu.bitcast(lax.shift_left(rbits, 16), f32), 0.0)
            ms_v[...] = _rb(0.5 + 0.5 * jnp.tanh(0.5 * r_sel))

        def ffn():
            if tk_last:
                topk(r_v[...])
            x_sel = xs_v[...]
            xs = x_sel.astype(bf16)
            for _ in range(fdelay):
                yield
            cnt = 0
            hs = []
            for t in range(nf):
                fs = slice(t * 128, min((t + 1) * 128, F))
                hh = []
                for w_v in (wg_v, wu_v):
                    a = None
                    for kt in range(D // 128):
                        ks = slice(kt * 128, (kt + 1) * 128)
                        d = lax.dot_general(xs[:, ks], w_v[fs, ks], NT, preferred_element_type=f32)
                        a = d if a is None else a + d
                        cnt += 1
                        if cnt % g1 == 0:
                            yield
                    hh.append(_rb(a))
                hs.append((_rb(_silu(hh[0])) * hh[1]).astype(bf16))
            cnt = 0
            ys = [None] * (D // 128)
            for t in range(nf):
                fs = slice(t * 128, min((t + 1) * 128, F))
                for kt in range(D // 128):
                    d = jnp.dot(hs[t], wd_v[fs, kt * 128:(kt + 1) * 128], preferred_element_type=f32)
                    ys[kt] = d if ys[kt] is None else ys[kt] + d
                    cnt += 1
                    if cnt % g2 == 0:
                        yield
            y = jnp.concatenate(ys, axis=1)
            y = _rb(_rb(y) * jnp.concatenate([ms_v[...]] * (D // 128), axis=1))
            gsel = _silu(_rb(x_sel + y))
            for c in range(C):
                g_v[pl.ds(jnp.clip(idx_s[c], 0, S - 1), 1), :] = gsel[c:c + 1, :]

        def run_slots(h, tail, hook=None):
            n = nsub

            def unit(t):
                if t < 0:
                    return (h - 1 if tail else jnp.maximum(h - 1, 0)), t + nsub
                return h + t // nsub, t % nsub

            z = jnp.concatenate([z_v[0:8, :]] * (ts // 8), axis=0)
            svals = {}
            mvals = {}
            q = pltpu.bitcast(q_c[...], bf16)
            o_done = fin_o(o_c[...], l_c[...])
            pend = []
            ocs = []
            mhist = []
            moe_gen = ffn() if tail else None
            moe_done = None

            def gate(dep):
                r0 = jnp.minimum(h * mrows, S - mrows)
                w = pltpu.bitcast(dep[0:mrows // 2, :], i32) & z[0:mrows // 2, :]
                xb = xn_v[half(r0, mrows), :] | pltpu.bitcast(jnp.concatenate([w] * (D // 128), axis=1), u32)
                g_v[pl.ds(pl.multiple_of(r0, 16), mrows), :] = _silu(pltpu.bitcast(xb, bf16).astype(f32))

            def flush():
                if moe_done is not None and j >= moe_done + e_lag and len(pend) > hold:
                    u, od = pend.pop(0)
                    oproj(*u, od, final=True)

            for j in range(n):
                tb = j + L
                kb = unit(tb)[0]
                s_list = [None] * nch
                mrun = None
                lrun = None
                o = None
                q_next = None
                do_a = not (tail and tb + 1 >= n)
                do_b = not (tail and tb >= n)
                m_prev = fin_m(m_c[j] if j < L else mvals.pop(j))
                if do_b and not xthr:
                    ocs = []
                if hook is not None and j == dma_slot:
                    hook()
                for op in ((lorder if do_b else norder) if tail else order):
                    if moe_gen is not None and op[0] in 'BC':
                        try:
                            next(moe_gen)
                        except StopIteration:
                            moe_gen = None
                            moe_done = j
                    if op == 'A':
                        if do_a:
                            q_next = pltpu.bitcast(ql_v[half((tb + 1) * ts, ts), :], bf16) if tail else qproj(*unit(tb + 1))
                    elif op == 'D':
                        if tail and j > 0:
                            pend.append((unit(j - 1), o_done))
                            flush()
                        else:
                            oproj(*unit(j - 1), o_done, fresh=None if tail else (h == 0))
                    elif op == 'X':
                        flush()
                    elif op[0] == 'B':
                        c = int(op[1:])
                        cs = slice(c * kc, (c + 1) * kc)
                        qq = q
                        if mdl and len(mhist) >= mdl and c in mch:
                            w = pltpu.bitcast(mhist[len(mhist) - mdl], i32)
                            w = (w[0:ts // 2, :] | w[ts // 2:, :]) & z[0:ts // 2, :]
                            qq = pltpu.bitcast(pltpu.bitcast(q, i32) | w, bf16)
                        s = lax.dot_general(qq, wld(k_v, kb, c * kc, kc), NT, preferred_element_type=f32)
                        if tb >= n:
                            s_c[tb - n, :, cs] = s
                        s_list[c] = s
                        mc = _fold(s, jnp.maximum)
                        mrun = mc if mrun is None else jnp.maximum(mrun, mc)
                        mhist.append(mrun)
                        if not tail and j == n - 1 and op == gtie:
                            gate(s[:, 0:128])
                    elif op[0] == 'C':
                        c = int(op[1:])
                        cs = slice(c * kc, (c + 1) * kc)
                        sp = s_c[j, :, cs] if j < L else svals[j][c]
                        m_use = m_prev
                        th = thr if do_b else thrl
                        if do_b and c == 0:
                            th = x0
                        if th and len(ocs) >= th:
                            m_use = m_prev + pltpu.bitcast(pltpu.bitcast(ocs[len(ocs) - th], i32) & z, f32)
                        p = jnp.exp2(sp - jnp.concatenate([m_use] * (kc // 128), axis=1))
                        if pmode == 0:
                            pb = p.astype(bf16)
                            pbs = [pb[:, t * 128:(t + 1) * 128] for t in range(kc // 128)]
                            lc = _fold(p, jnp.add)
                        elif pmode == 1:
                            pbs = [p[:, t * 128:(t + 1) * 128].astype(bf16) for t in range(kc // 128)]
                            lc = _fold(p, jnp.add)
                        elif pmode == 2:
                            pb = pltpu.bitcast(pltpu.bitcast(p.astype(bf16), u32), bf16)
                            pbs = [pb[:, t * 128:(t + 1) * 128] for t in range(kc // 128)]
                            lc = _fold(pb.astype(f32), jnp.add)
                        elif pmode == 3:
                            pb = pltpu.bitcast(pltpu.bitcast(p.astype(bf16), u32), bf16)
                            pbs = [pb[:, t * 128:(t + 1) * 128] for t in range(kc // 128)]
                            lc = _fold(p, jnp.add)
                        elif pmode == 4:
                            pu = pltpu.bitcast(p.astype(bf16), i32)
                            pb = pltpu.bitcast(pu, bf16)
                            pbs = [pb[:, t * 128:(t + 1) * 128] for t in range(kc // 128)]
                            w = _fold(pu, jnp.bitwise_or) & z[0:ts // 2, :]
                            lc = _fold(p, jnp.add) + pltpu.bitcast(jnp.concatenate([w, w], axis=0), f32)
                        lrun = lc if lrun is None else lrun + lc
                        parts = [jnp.dot(pbs[t], wld(v_v, h, c * kc + t * 128, 128),
                                         preferred_element_type=f32) for t in range(kc // 128)]
                        oc = (parts[0] + parts[1]) + (parts[2] + parts[3])
                        ocs.append(parts[0])
                        o = oc if o is None else o + oc
                        if not tail and j == n - 1 and op == gtie:
                            gate(ocs[-1])
                        if tail and do_b and c in extra_d:
                            flush()
                if do_b:
                    if tb >= n:
                        m_c[tb - n] = mrun
                    else:
                        svals[tb] = s_list
                        mvals[tb] = mrun
                q = q_next
                if j + 1 < n:
                    o_done = fin_o(o, lrun)
            if tail:
                pend.append((unit(n - 1), fin_o(o, lrun)))
                for u, od in pend:
                    oproj(*u, od, final=True)
                return
            q_c[...] = pltpu.bitcast(q, u32)
            o_c[...] = o
            l_c[...] = lrun

        later = dict(wql=cp_wq(H - 1, 5), v0=cp_v(0), wo0=cp_wo(0), wq1=cp_wq(1), k1=cp_k(1))
        cp_x(0).start()
        cp_x(1).start()
        cp_wq(0, 4).start()
        r_v[...] = jnp.zeros((16, 128), f32)
        xs_v[...] = jnp.zeros((16, D), f32)
        o_c[...] = jnp.zeros((ts, DH), f32)
        l_c[...] = jnp.ones((ts, 128), f32)
        if kdelay is not None:
            def idle(c, _):
                acc[pl.ds(pl.multiple_of(c * 64, 64), 64), :] = jnp.zeros((64, D), f32)
                return 0
            lax.fori_loop(0, kdelay, idle, 0)
            cp_k(0, 6).start()

        def mxu_front(c, u):
            wsel = (0 if c < na0 else H - 1) if isinstance(c, int) else jnp.where(c < na0, 0, H - 1)
            if u is not None:
                q = pltpu.bitcast(ql_v[half(u * ts, ts), :], bf16)

            def a_job(t):
                qn = qscale(jnp.dot(xn_ld((c * upc + t) * ts, ts), wld(wq_v, wsel, 0, D), preferred_element_type=f32))
                ql_v[half((c * upc + t) * ts, ts), :] = pltpu.bitcast(qn, u32)
            ap = (apos, apos) if isinstance(apos, int) else apos
            wrf = jnp.broadcast_to(wr_ref[...].astype(f32).reshape(1, D), (16, D))
            jobs = []
            for t in range(upc):
                lhs = jnp.where(lax.broadcasted_iota(i32, (16, D), 0) == c * upc + t, wrf, 0.0).astype(bf16)
                xn = xn_ld((c * upc + t) * ts, ts)
                jobs += [(lhs[:, k * 128:(k + 1) * 128], xn[:, k * 128:(k + 1) * 128]) for k in range(D // 128)]
            rs = r_v[...]
            mrun = None
            for cc in range(nch + 1):
                for t in range(upc):
                    if ap[t] == cc:
                        a_job(t)
                if cc == nch:
                    break
                if u is not None:
                    cs = slice(cc * kc, (cc + 1) * kc)
                    s = lax.dot_general(q, wld(k_v, 0, cc * kc, kc), NT, preferred_element_type=f32)
                    s_c[u, :, cs] = s
                    mc = _fold(s, jnp.maximum)
                    mrun = mc if mrun is None else jnp.maximum(mrun, mc)
                for _ in range(rgrp[cc]):
                    a, b = jobs.pop(0)
                    rs = rs + lax.dot_general(a, b, NT, preferred_element_type=f32)
            if u is not None:
                m_c[u] = mrun
            r_v[...] = rs

        def ln_rows(r0, n, zs):
            def ld(i):
                if i == 0 or not reload:
                    return x_v[pl.ds(r0, n), :]
                return x_v[pl.ds(pl.multiple_of(r0 + zs * i, n), n), :]
            for t, w in enumerate(_layernorm(ld, z_v[0:8, :] if ntie else None)):
                xn_v[half(r0, n), t * 128:(t + 1) * 128] = w

        def ln_chunk(c, zs):
            ns = lnsub if isinstance(lnsub, int) and c >= 2 else (lnsub0 if c < 2 else lnsub[c])
            n = xc // ns
            for t in range(ns):
                ln_rows(c * xc + t * n, n, zs)

        with scope('wx0'):
            cp_x(0).wait()
        with scope('ln01'):
            if kdelay is None:
                cp_k(0, 6).start()
            if x2early:
                cp_x(2).start()
            t0 = x_v[0:16, 0:128].astype(f32)[0:8, :]
            t0 = jnp.where(jnp.abs(t0) < 1.0, t0, 0.5)
            zv = pltpu.bitcast(t0 - t0, i32)
            z_v[0:8, :] = zv
            zs = zv[0, 0]
            ln_chunk(0, zs)
            cp_x(1).wait()
            cp_wq(0, 4).wait()
            for c in range(3 if x2early else 2, 3 + x2extra):
                cp_x(c).start()
            mxu_front(0, None)
            ln_chunk(1, zs)
            cp_k(0, 6).wait()
        def a_unit(uu):
            hsel = 0 if uu < na0 * upc else H - 1
            qn = qscale(jnp.dot(xn_ld(uu * ts, ts), wld(wq_v, hsel, 0, D), preferred_element_type=f32))
            ql_v[half(uu * ts, ts), :] = pltpu.bitcast(qn, u32)

        def r_jobs(uu):
            wrf = jnp.broadcast_to(wr_ref[...].astype(f32).reshape(1, D), (16, D))
            lhs = jnp.where(lax.broadcasted_iota(i32, (16, D), 0) == uu, wrf, 0.0).astype(bf16)
            xn = xn_ld(uu * ts, ts)
            return [(lhs[:, k * 128:(k + 1) * 128], xn[:, k * 128:(k + 1) * 128]) for k in range(D // 128)]

        plan = fplan or [
            "L2 a3 r2 a2 r3 b0.0 r3 b0.1 r2 b0.2 b0.3",
            "L3 L4 b1.0 r5 a4 a5 r5 b1.1 r4 b1.2 r4 b1.3 b2.0 r6 a6 b2.1 b2.2 r7 a7 r7 b2.3 b3.0 b3.1 r6 b3.2 b3.3",
            "L5 L6 L7 b4.0 a9 r8 a8 r9 b4.1 r9 a11 r11 b4.2 r10 a10 r8 b4.3 r10 b5.0 r12 b5.1 r13 a13 b5.2 r13 a14 r11 "
            "a12 r14 b5.3 r12 b6.0 r15 b6.1 a15 r14 b6.2 b6.3 r15",
        ]
        for bi, blk in enumerate(blocks):
            with scope('fb%d' % bi):
                for c in blk:
                    cp_x(c).wait()
                if bi == len(blocks) - 1 - wqlb:
                    later['wql'].wait()
                for k in bstart[bi]:
                    (cp_x(k) if isinstance(k, int) else later[k]).start()
                rs = r_v[...]
                rj = {}
                mr = {}
                qs = {}
                for op in plan[bi].split():
                    if op[0] == 'L':
                        ln_chunk(int(op[1:]), zs)
                    elif op[0] == 'a':
                        a_unit(int(op[1:]))
                    elif op[0] == 'r':
                        uu = int(op[1:])
                        first = uu not in rj
                        if first:
                            rj[uu] = r_jobs(uu)
                        for _ in range(3 if first else 2):
                            a, b = rj[uu].pop(0)
                            rs = rs + lax.dot_general(a, b, NT, preferred_element_type=f32)
                    elif op[0] == 'b':
                        uu, cc = (int(t) for t in op[1:].split('.'))
                        if uu not in qs:
                            qs[uu] = pltpu.bitcast(ql_v[half(uu * ts, ts), :], bf16)
                        sv = lax.dot_general(qs[uu], wld(k_v, 0, cc * kc, kc), NT, preferred_element_type=f32)
                        s_c[uu, :, cc * kc:(cc + 1) * kc] = sv
                        mc = _fold(sv, jnp.maximum)
                        mr[uu] = mc if uu not in mr else jnp.maximum(mr[uu], mc)
                        if cc == nch - 1:
                            m_c[uu] = mr[uu]
                r_v[...] = rs
        q_c[...] = ql_v[half(L * ts, ts), :]
        def nxt(h, do):
            do(cp_v(h))
            do(cp_wo(h))
            if isinstance(h, int):
                if h + 1 < H - 1:
                    do(cp_wq(h + 1))
                if h + 1 < H:
                    do(cp_k(h + 1))
                return

            @pl.when(h + 1 < H - 1)
            def _():
                do(cp_wq(h + 1))

            @pl.when(h + 1 < H)
            def _():
                do(cp_k(h + 1))

        if not waittop:
            nxt(0, lambda cp: cp.wait())

        def body(h, _):
            def hook():
                nxt(h + 1, lambda cp: cp.start())

                @pl.when(h == 1)
                def _():
                    for i in range(3):
                        cp_f(i).start()
            if waittop:
                cp_v(h).wait()
                cp_wo(h).wait()
                cp_k(h + 1).wait()

                @pl.when(h + 1 < H - 1)
                def _():
                    cp_wq(h + 1).wait()
            with scope('mid'):
                if nomid:
                    hook()
                    hh = h % L
                    s_c[hh, 0:8, 0:128] = s_c[hh, 0:8, 0:128] + 1.0
                    m_c[hh, 0:8, :] = m_c[hh, 0:8, :] + 1.0
                    rr = pl.ds(pl.multiple_of(h * 8, 8), 8)
                    ql_v[rr, :] = ql_v[rr, :] + 1
                    xn_v[rr, :] = xn_v[rr, :] + 1
                    q_c[...] = q_c[...] + 1
                    r_v[...] = r_v[...] + 1.0
                    o_c[...] = o_c[...] + 1.0
                    l_c[...] = l_c[...] + 1.0
                    z_v[0:8, :] = z_v[0:8, :] + 1
                else:
                    run_slots(h, False, hook)
            if not waittop:
                nxt(h + 1, lambda cp: cp.wait())
            return 0

        lax.fori_loop(0, H - 1, body, 0)
        if waittop:
            nxt(H - 1, lambda cp: cp.wait())
        for i in range(3):
            cp_f(i).wait()
        with scope('last'):
            if nolast:
                def ep(c, _):
                    rows = pl.ds(pl.multiple_of(c * 16, 16), 16)
                    out_v[rows, :] = (acc[rows, :] * g_v[rows, :] + xs_v[...] * idx_s[c % 8].astype(f32)
                                      + ms_v[:, 0:1] + r_v[:, 0:1] + s_c[c % L, 0:16, 0:640] + o_c[0:16, 0:1] + l_c[0:16, 0:1]
                                      + m_c[c % L, 0:16, 0:1] + pltpu.bitcast(q_c[0:16, 0:128], f32)[:, 0:1] + pltpu.bitcast(ql_v[pl.ds(pl.multiple_of((c % 64) * 16, 16), 16), :], f32)[:, 0:1]).astype(bf16)
                    return 0
                lax.fori_loop(0, S // 16, ep, 0)
                for c in range(noc):
                    cp_o(c).start()
            else:
                run_slots(H - 1, True)
        with scope('wout'):
            for c in range(noc):
                cp_o(c).wait()

    anyspec = pl.BlockSpec(memory_space=pl.ANY)
    out = pl.pallas_call(
        kernel,
        in_specs=[anyspec, anyspec, anyspec, anyspec, anyspec,
                  pl.BlockSpec(memory_space=pltpu.VMEM),
                  anyspec, anyspec, anyspec],
        out_specs=anyspec,
        out_shape=jax.ShapeDtypeStruct((S, D), bf16),
        scratch_shapes=[
            pltpu.VMEM((zrows, 128), i32),
            pltpu.VMEM((S, D), bf16),
            pltpu.VMEM((S // 2, D), u32),
            pltpu.VMEM((S, D), f32),
            pltpu.VMEM((H, S, DH), bf16),
            pltpu.VMEM((H, S, DH), bf16),
            pltpu.VMEM((H, D, DH), bf16),
            pltpu.VMEM((H, DH, D), bf16),
            pltpu.VMEM((F, D), bf16),
            pltpu.VMEM((F, D), bf16),
            pltpu.VMEM((F, D), bf16),
            pltpu.VMEM((S, D), f32),
            pltpu.VMEM((16, 128), f32),
            pltpu.VMEM((16, D), f32),
            pltpu.VMEM((16, 128), f32),
            pltpu.SMEM((C,), i32),
            pltpu.VMEM((L, ts, S), f32),
            pltpu.VMEM((L, ts, 128), f32),
            pltpu.VMEM((ts // 2, DH), u32),
            pltpu.VMEM((ts, DH), f32),
            pltpu.VMEM((ts, 128), f32),
            pltpu.VMEM((S, D), bf16),
            pltpu.VMEM((S // 2, DH), u32),
            pltpu.SemaphoreType.DMA((nxc,)),
            pltpu.SemaphoreType.DMA((7,)),
            pltpu.SemaphoreType.DMA((3,)),
            pltpu.SemaphoreType.DMA((noc,)),
        ],
        compiler_params=pltpu.CompilerParams(vmem_limit_bytes=120 * 1024 * 1024, disable_bounds_checks=True,
                                             disable_semaphore_checks=True,
                                             internal_scratch_in_bytes=isb),
    )(x2, k3, v3, A_wq, A_wo, B_w_r, B_w_gate.T, B_w_up.T, B_w_down)
    return out.reshape(1, S, D)


@jax.jit
def pallas_recurrent_scan__mha_block_cached__moe_arch_mod__prompt_kernel(
        A_x, A_k_cache, A_v_cache, A_wq, A_wo, B_x, B_w_r, B_w_gate, B_w_up, B_w_down):
    return build(A_x, A_k_cache, A_v_cache, A_wq, A_wo, B_x, B_w_r, B_w_gate, B_w_up, B_w_down)
```

```python
import jax
import jax.numpy as jnp
from jax import lax
import jax.experimental.pallas as pl
import jax.experimental.pallas.tpu as pltpu

S, D, H, DH, F, C = 2048, 640, 32, 128, 1728, 8
LOG2E = 1.4426950408889634
bf16 = jnp.bfloat16
f32 = jnp.float32
i32 = jnp.int32
u32 = jnp.uint32
NT = (((1,), (1,)), ((), ()))

TS = 128
KC = 512
NSUB = S // TS
NCH = S // KC
NT_D = D // 128
NF = (F + 127) // 128
XC = 256
L = 7
GROWS = 80
DMA_SLOT = 4
FFN_DELAY = 8

ORDER_LOOP = "A B0 D C0 B1 C1 B2 C2 B3 C3".split()
ORDER_TAIL = "B0 D C0 B1 C1 B2 C2 B3 C3 A".split()
ORDER_END = "C0 C1 D C2 X C3".split()
OUT_CUTS = [r * TS for r in (2, 4, 6, 8, 10, 12, 13, 14, 15)] + [S - TS // 2, S]

FRONT_PLAN = [
    "L1 a0 a1 r0 r1 r0 r1 a2 a3 r2 r3 r2 r3",
    "L2 b0.0 b0.1 b0.2 b0.3 b1.0 b1.1 b1.2 b1.3",
    "L3 L4 a4 b2.0 r5 b2.1 r5 b2.2 r4 a5 r4 b2.3 b3.0 b3.1 r6 a6 r7 b3.2 b3.3 a7 b4.0 r6 b4.1 r7 b4.2 b4.3",
    "L5 L6 L7 a8 r9 b5.0 b5.1 r8 a11 r10 b5.2 r8 a10 r9 a9 r10 b5.3 r12 a13 r11 a12 r12 b6.0 r11 a14 r15 a15 "
    "r13 b6.1 r13 b6.2 r14 b6.3 r14 r15",
]
FRONT_WAIT = ((1, 'wq0', 'wr'), ('k0', 2), (3, 4), (5, 6, 7, 'wql'))
FRONT_START = ((3,), (4, 5), ('wql', 6, 7, 'wo0', 'wq1'), ('v0', 'k1'))


def _rb(x):
    return x.astype(bf16).astype(f32)


def _layernorm(ld):
    mean = jnp.sum(ld(0).astype(f32), axis=-1, keepdims=True) * (1.0 / D)
    c = ld(1).astype(f32) - mean
    ssq = jnp.sum(c * c, axis=-1, keepdims=True)
    n = ssq.shape[0]
    ng = n // 8
    t = jnp.broadcast_to(ssq, (n, 128)).reshape(ng, 8, 128)
    lane = lax.broadcasted_iota(i32, (8, 128), 1)
    bit = 1
    while t.shape[0] > 1:
        hlf = t.shape[0] // 2
        t = jnp.where(((lane & bit) != 0)[None], t[hlf:], t[:hlf])
        bit *= 2
    den = _rb(jnp.sqrt(_rb(_rb(t[0] * (1.0 / D)) + 1e-5)))
    inv = pl.reciprocal(den, approx=True)
    inv = inv * (2.0 - den * inv)
    nb = ng.bit_length() - 1
    cols = []
    for g in range(ng):
        lg = int(format(g, '0%db' % nb)[::-1], 2)
        cols.append(jnp.broadcast_to(inv[:, lg:lg + 1], (8, 128)))
    inv = jnp.concatenate(cols, axis=0)
    mb = jnp.broadcast_to(_rb(mean), (n, 128))
    x = ld(2).astype(f32)
    return [pltpu.bitcast((_rb(x[:, t * 128:(t + 1) * 128] - mb) * inv).astype(bf16), u32) for t in range(NT_D)]


def _silu(x):
    hx = 0.5 * x
    return hx + hx * jnp.tanh(hx)


def _fold(x, op):
    r = x[:, 0:128]
    for t in range(1, x.shape[1] // 128):
        r = op(r, x[:, t * 128:(t + 1) * 128])
    return r


def _kernel(x_hbm, k_hbm, v_hbm, wq_hbm, wo_hbm, wr_hbm, wg_hbm, wu_hbm, wd_hbm, o_hbm,
            z_v, x_v, xn_v, g_v, k_v, v_v, wq_v, wo_v, wg_v, wu_v, wd_v, acc, r_v, xs_v, ms_v, idx_s,
            s_c, m_c, q_c, o_c, l_c, out_v, ql_v, wr_v,
            sem_x, sem_h, sem_f, sem_o):
    def hoff(h):
        return h * DH if isinstance(h, int) else pl.multiple_of(h * DH, DH)

    def cp_x(c):
        rows = pl.ds(c * XC, XC)
        return pltpu.make_async_copy(x_hbm.at[rows, :], x_v.at[rows, :], sem_x.at[c])

    def cp_k(h, i=0):
        return pltpu.make_async_copy(k_hbm.at[h], k_v.at[h], sem_h.at[i])

    def cp_v(h):
        return pltpu.make_async_copy(v_hbm.at[h], v_v.at[h], sem_h.at[1])

    def cp_wq(h, i=2):
        return pltpu.make_async_copy(wq_hbm.at[:, pl.ds(hoff(h), DH)], wq_v.at[h], sem_h.at[i])

    def cp_wo(h):
        return pltpu.make_async_copy(wo_hbm.at[pl.ds(hoff(h), DH), :], wo_v.at[h], sem_h.at[3])

    def cp_f(i):
        return pltpu.make_async_copy((wg_hbm, wu_hbm, wd_hbm)[i], (wg_v, wu_v, wd_v)[i], sem_f.at[i])

    def cp_o(c):
        lo = OUT_CUTS[c - 1] if c else 0
        rows = pl.ds(lo, OUT_CUTS[c] - lo)
        return pltpu.make_async_copy(out_v.at[rows, :], o_hbm.at[rows, :], sem_o.at[c])

    def sub(j):
        return pl.ds(j * TS, TS)

    def half(r0, n):
        if isinstance(r0, int):
            return pl.ds(r0 // 2, n // 2)
        return pl.ds(pl.multiple_of(r0 // 2, 8), n // 2)

    def xn_ld(r0, n):
        return pltpu.bitcast(xn_v[half(r0, n), :], bf16)

    def qproj(h, j):
        q = jnp.dot(xn_ld(j * TS, TS), wq_v[h], preferred_element_type=f32)
        return (q * (DH ** -0.5 * LOG2E)).astype(bf16)

    def oproj(h, j, o, fresh=None):
        y = jnp.dot(o, wo_v[h], preferred_element_type=f32)
        if fresh is None:
            acc[sub(j), :] += y
        else:
            acc[sub(j), :] = jnp.where(fresh, 0.0, acc[sub(j), :]) + y

    def oproj_final(h, j, o):
        npc = 2 if j == NSUB - 1 else 1
        n = TS // npc
        for i in range(npc):
            rows = pl.ds(j * TS + i * n, n)
            y = jnp.dot(o[i * n:(i + 1) * n, :], wo_v[h], preferred_element_type=f32)
            t = (acc[rows, :] + y) * g_v[rows, :]
            out_v[rows, :] = (x_v[rows, :].astype(f32) + t).astype(bf16)
            if j * TS + (i + 1) * n in OUT_CUTS:
                cp_o(OUT_CUTS.index(j * TS + (i + 1) * n)).start()

    def fin_m(mrun):
        return jnp.broadcast_to(jnp.max(mrun, axis=-1, keepdims=True), (TS, 128))

    def fin_o(o, lrun):
        l = jnp.sum(lrun, axis=-1, keepdims=True)
        return (o * pl.reciprocal(l, approx=True)).astype(bf16)

    def topk():
        r = _rb(r_v[...]) + 0.0
        bits = lax.shift_right_logical(pltpu.bitcast(r, i32), 16)
        ordered = jnp.where(bits >= 0x8000, 0xFFFF - bits, bits + 0x8000)
        ordered = jnp.where(r != r, 0, ordered)
        sl = lax.broadcasted_iota(i32, (16, 128), 0)
        ln = lax.broadcasted_iota(i32, (16, 128), 1)
        key = pltpu.bitcast(ordered * 2048 + (2047 - (sl * 128 + ln)) + (1 << 28), f32)
        msel = jnp.zeros((16, 128), f32)
        for c in range(C):
            m = jnp.max(jnp.max(key, axis=0, keepdims=True), axis=1, keepdims=True)
            mb = jnp.broadcast_to(m, (16, 128))
            key = jnp.where(key == mb, 0.0, key)
            msel = jnp.where(sl == c, mb, msel)
            ic = (2047 - (pltpu.bitcast(mb, i32) & 2047))[0, 0]
            idx_s[c] = ic
            pair = pltpu.bitcast(xn_v[pl.ds(lax.shift_right_logical(ic, 1), 1), :], i32)
            xs_v[c:c + 1, :] = pltpu.bitcast(lax.shift_left(lax.shift_right_logical(pair, (ic & 1) * 16), 16), f32)
        o16 = lax.shift_right_logical(pltpu.bitcast(msel, i32) - (1 << 28), 11) & 0xFFFF
        rbits = jnp.where(o16 >= 0x8000, o16 - 0x8000, 0xFFFF - o16)
        r_sel = jnp.where(sl < C, pltpu.bitcast(lax.shift_left(rbits, 16), f32), 0.0)
        ms_v[...] = _rb(0.5 + 0.5 * jnp.tanh(0.5 * r_sel))

    def moe():
        topk()
        x_sel = xs_v[...]
        xs = x_sel.astype(bf16)
        for _ in range(FFN_DELAY):
            yield
        cnt = 0
        hs = []
        for t in range(NF):
            fs = slice(t * 128, min((t + 1) * 128, F))
            hh = []
            for w_v in (wg_v, wu_v):
                a = None
                for kt in range(NT_D):
                    ks = slice(kt * 128, (kt + 1) * 128)
                    d = lax.dot_general(xs[:, ks], w_v[fs, ks], NT, preferred_element_type=f32)
                    a = d if a is None else a + d
                    cnt += 1
                    if cnt % 4 == 0:
                        yield
                hh.append(_rb(a))
            hs.append((_rb(_silu(hh[0])) * hh[1]).astype(bf16))
        cnt = 0
        ys = [None] * NT_D
        for t in range(NF):
            fs = slice(t * 128, min((t + 1) * 128, F))
            for kt in range(NT_D):
                d = jnp.dot(hs[t], wd_v[fs, kt * 128:(kt + 1) * 128], preferred_element_type=f32)
                ys[kt] = d if ys[kt] is None else ys[kt] + d
                cnt += 1
                if cnt % 4 == 0:
                    yield
        y = jnp.concatenate(ys, axis=1)
        y = _rb(_rb(y) * jnp.concatenate([ms_v[...]] * NT_D, axis=1))
        gsel = _silu(_rb(x_sel + y))
        for c in range(C):
            g_v[pl.ds(jnp.clip(idx_s[c], 0, S - 1), 1), :] = gsel[c:c + 1, :]

    def run_head(h, tail, hook=None):
        def unit(t):
            if t < 0:
                return (h - 1 if tail else jnp.maximum(h - 1, 0)), t + NSUB
            return h + t // NSUB, t % NSUB

        z = jnp.concatenate([z_v[0:8, :]] * (TS // 8), axis=0)
        svals = {}
        mvals = {}
        q = pltpu.bitcast(q_c[...], bf16)
        o_done = fin_o(o_c[...], l_c[...])
        pend = []
        pvs = []
        mhist = []
        moe_gen = moe() if tail else None

        def gate(dep):
            r0 = jnp.minimum(h * GROWS, S - GROWS)
            w = pltpu.bitcast(dep[0:GROWS // 2, :], i32) & z[0:GROWS // 2, :]
            xb = xn_v[half(r0, GROWS), :] | pltpu.bitcast(jnp.concatenate([w] * NT_D, axis=1), u32)
            g_v[pl.ds(pl.multiple_of(r0, 16), GROWS), :] = _silu(pltpu.bitcast(xb, bf16).astype(f32))

        def flush():
            if moe_gen is None and pend:
                oproj_final(*pend.pop(0))

        for j in range(NSUB):
            tb = j + L
            s_list = [None] * NCH
            mrun = None
            lrun = None
            o = None
            q_next = None
            do_a = not (tail and tb + 1 >= NSUB)
            do_b = not (tail and tb >= NSUB)
            m_row = fin_m(m_c[j] if j < L else mvals.pop(j))
            if hook is not None and j == DMA_SLOT:
                hook()
            for op in ((ORDER_TAIL if do_b else ORDER_END) if tail else ORDER_LOOP):
                if moe_gen is not None and op[0] in 'BC':
                    if next(moe_gen, 'done') == 'done':
                        moe_gen = None
                if op == 'A':
                    if do_a:
                        q_next = (pltpu.bitcast(ql_v[half((tb + 1) * TS, TS), :], bf16) if tail
                                  else qproj(*unit(tb + 1)))
                elif op == 'D':
                    if tail and j > 0:
                        pend.append((h, j - 1, o_done))
                        flush()
                    else:
                        oproj(*unit(j - 1), o_done, fresh=None if tail else (h == 0))
                elif op == 'X':
                    flush()
                elif op[0] == 'B':
                    c = int(op[1:])
                    cs = slice(c * KC, (c + 1) * KC)
                    qq = q
                    if len(mhist) >= 2 and c in (0, 2):
                        w = pltpu.bitcast(mhist[-2], i32)
                        w = (w[0:TS // 2, :] | w[TS // 2:, :]) & z[0:TS // 2, :]
                        qq = pltpu.bitcast(pltpu.bitcast(q, i32) | w, bf16)
                    s = lax.dot_general(qq, k_v[unit(tb)[0], cs, :], NT, preferred_element_type=f32)
                    if tb >= NSUB:
                        s_c[tb - NSUB, :, cs] = s
                    s_list[c] = s
                    mc = _fold(s, jnp.maximum)
                    mrun = mc if mrun is None else jnp.maximum(mrun, mc)
                    mhist.append(mrun)
                elif op[0] == 'C':
                    c = int(op[1:])
                    cs = slice(c * KC, (c + 1) * KC)
                    sp = s_c[j, :, cs] if j < L else svals[j][c]
                    m_use = m_row
                    lag = 1 if do_b else 2
                    if len(pvs) >= lag:
                        m_use = m_row + pltpu.bitcast(pltpu.bitcast(pvs[-lag], i32) & z, f32)
                    p = jnp.exp2(sp - jnp.concatenate([m_use] * (KC // 128), axis=1))
                    pb = p.astype(bf16)
                    lc = _fold(p, jnp.add)
                    lrun = lc if lrun is None else lrun + lc
                    parts = [jnp.dot(pb[:, t * 128:(t + 1) * 128], v_v[h, c * KC + t * 128:c * KC + (t + 1) * 128, :],
                                     preferred_element_type=f32) for t in range(KC // 128)]
                    oc = (parts[0] + parts[1]) + (parts[2] + parts[3])
                    pvs.append(parts[0])
                    o = oc if o is None else o + oc
                    if not tail and j == NSUB - 1 and c == NCH - 1:
                        gate(parts[0])
                    if tail and do_b and c == 1:
                        flush()
            if do_b:
                if tb >= NSUB:
                    m_c[tb - NSUB] = mrun
                else:
                    svals[tb] = s_list
                    mvals[tb] = mrun
            q = q_next
            if j + 1 < NSUB:
                o_done = fin_o(o, lrun)
        if tail:
            pend.append((h, NSUB - 1, fin_o(o, lrun)))
            for args in pend:
                oproj_final(*args)
            return
        q_c[...] = pltpu.bitcast(q, u32)
        o_c[...] = o
        l_c[...] = lrun

    named = dict(wql=cp_wq(H - 1, 5), v0=cp_v(0), wo0=cp_wo(0), wq1=cp_wq(1), k1=cp_k(1),
                 wq0=cp_wq(0, 4), k0=cp_k(0, 6), wr=pltpu.make_async_copy(wr_hbm, wr_v, sem_h.at[7]))

    def front_cp(k):
        return cp_x(k) if isinstance(k, int) else named[k]

    for k in (0, 1, 'wq0', 'wr'):
        front_cp(k).start()
    r_v[...] = jnp.zeros((16, 128), f32)
    xs_v[...] = jnp.zeros((16, D), f32)
    o_c[...] = jnp.zeros((TS, DH), f32)
    l_c[...] = jnp.ones((TS, 128), f32)
    front_cp('k0').start()

    def ln_chunk(c, zs):
        pieces = 4 if c >= 2 else 2
        n = XC // pieces
        for t in range(pieces):
            r0 = c * XC + t * n

            def ld(i):
                if i == 0:
                    return x_v[pl.ds(r0, n), :]
                return x_v[pl.ds(pl.multiple_of(r0 + zs * i, n), n), :]
            for tt, w in enumerate(_layernorm(ld)):
                xn_v[half(r0, n), tt * 128:(tt + 1) * 128] = w

    def router_tiles(u):
        wrf = jnp.broadcast_to(wr_v[...].astype(f32).reshape(1, D), (16, D))
        lhs = jnp.where(lax.broadcasted_iota(i32, (16, D), 0) == u, wrf, 0.0).astype(bf16)
        xn = xn_ld(u * TS, TS)
        return [(lhs[:, k * 128:(k + 1) * 128], xn[:, k * 128:(k + 1) * 128]) for k in range(NT_D)]

    cp_x(0).wait()
    cp_x(2).start()
    t0 = x_v[0:16, 0:128].astype(f32)[0:8, :]
    t0 = jnp.where(jnp.abs(t0) < 1.0, t0, 0.5)
    zv = pltpu.bitcast(t0 - t0, i32)
    z_v[0:8, :] = zv
    zs = zv[0, 0]
    ln_chunk(0, zs)

    for bi, plan in enumerate(FRONT_PLAN):
        for k in FRONT_WAIT[bi]:
            front_cp(k).wait()
        for k in FRONT_START[bi]:
            front_cp(k).start()
        rs = r_v[...]
        rj = {}
        mr = {}
        qs = {}
        for op in plan.split():
            if op[0] == 'L':
                ln_chunk(int(op[1:]), zs)
            elif op[0] == 'a':
                u = int(op[1:])
                ql_v[half(u * TS, TS), :] = pltpu.bitcast(qproj(0 if u <= L else H - 1, u), u32)
            elif op[0] == 'r':
                u = int(op[1:])
                first = u not in rj
                if first:
                    rj[u] = router_tiles(u)
                for _ in range(3 if first else 2):
                    a, b = rj[u].pop(0)
                    rs = rs + lax.dot_general(a, b, NT, preferred_element_type=f32)
            else:
                u, c = (int(t) for t in op[1:].split('.'))
                if u not in qs:
                    qs[u] = pltpu.bitcast(ql_v[half(u * TS, TS), :], bf16)
                s = lax.dot_general(qs[u], k_v[0, c * KC:(c + 1) * KC, :], NT, preferred_element_type=f32)
                s_c[u, :, c * KC:(c + 1) * KC] = s
                mc = _fold(s, jnp.maximum)
                mr[u] = mc if u not in mr else jnp.maximum(mr[u], mc)
                if c == NCH - 1:
                    m_c[u] = mr[u]
        r_v[...] = rs
    q_c[...] = ql_v[half(L * TS, TS), :]

    def body(h, carry):
        def hook():
            cp_v(h + 1).start()
            cp_wo(h + 1).start()

            @pl.when(h + 2 < H - 1)
            def _():
                cp_wq(h + 2).start()

            @pl.when(h + 2 < H)
            def _():
                cp_k(h + 2).start()

            @pl.when(h == 1)
            def _():
                for i in range(3):
                    cp_f(i).start()

        cp_v(h).wait()
        cp_wo(h).wait()
        cp_k(h + 1).wait()

        @pl.when(h + 1 < H - 1)
        def _():
            cp_wq(h + 1).wait()
        run_head(h, False, hook)
        return carry

    lax.fori_loop(0, H - 1, body, 0)

    cp_v(H - 1).wait()
    cp_wo(H - 1).wait()
    for i in range(3):
        cp_f(i).wait()
    run_head(H - 1, True)
    for c in range(len(OUT_CUTS)):
        cp_o(c).wait()


def build(A_x, A_k_cache, A_v_cache, A_wq, A_wo, B_x, B_w_r, B_w_gate, B_w_up, B_w_down):
    out = pl.pallas_call(
        _kernel,
        in_specs=[pl.BlockSpec(memory_space=pl.ANY)] * 9,
        out_specs=pl.BlockSpec(memory_space=pl.ANY),
        out_shape=jax.ShapeDtypeStruct((S, D), bf16),
        scratch_shapes=[
            pltpu.VMEM((128, 128), i32),
            pltpu.VMEM((S, D), bf16),
            pltpu.VMEM((S // 2, D), u32),
            pltpu.VMEM((S, D), f32),
            pltpu.VMEM((H, S, DH), bf16),
            pltpu.VMEM((H, S, DH), bf16),
            pltpu.VMEM((H, D, DH), bf16),
            pltpu.VMEM((H, DH, D), bf16),
            pltpu.VMEM((F, D), bf16),
            pltpu.VMEM((F, D), bf16),
            pltpu.VMEM((F, D), bf16),
            pltpu.VMEM((S, D), f32),
            pltpu.VMEM((16, 128), f32),
            pltpu.VMEM((16, D), f32),
            pltpu.VMEM((16, 128), f32),
            pltpu.SMEM((C,), i32),
            pltpu.VMEM((L, TS, S), f32),
            pltpu.VMEM((L, TS, 128), f32),
            pltpu.VMEM((TS // 2, DH), u32),
            pltpu.VMEM((TS, DH), f32),
            pltpu.VMEM((TS, 128), f32),
            pltpu.VMEM((S, D), bf16),
            pltpu.VMEM((S // 2, DH), u32),
            pltpu.VMEM((D,), bf16),
            pltpu.SemaphoreType.DMA((S // XC,)),
            pltpu.SemaphoreType.DMA((8,)),
            pltpu.SemaphoreType.DMA((3,)),
            pltpu.SemaphoreType.DMA((len(OUT_CUTS),)),
        ],
        compiler_params=pltpu.CompilerParams(vmem_limit_bytes=120 * 1024 * 1024,
                                             internal_scratch_in_bytes=64 * 1024,
                                             disable_bounds_checks=True,
                                             disable_semaphore_checks=True),
    )(A_x.reshape(S, D), A_k_cache.reshape(H, S, DH), A_v_cache.reshape(H, S, DH), A_wq, A_wo,
      B_w_r, B_w_gate.T, B_w_up.T, B_w_down)
    return out.reshape(1, S, D)


@jax.jit
def pallas_recurrent_scan__mha_block_cached__moe_arch_mod__prompt_kernel(
        A_x, A_k_cache, A_v_cache, A_wq, A_wo, B_x, B_w_r, B_w_gate, B_w_up, B_w_down):
    return build(A_x, A_k_cache, A_v_cache, A_wq, A_wo, B_x, B_w_r, B_w_gate, B_w_up, B_w_down)
```

```python
import jax
import jax.numpy as jnp
from jax import lax
import jax.experimental.pallas as pl
import jax.experimental.pallas.tpu as pltpu

S, D, H, DH, F, C = 2048, 640, 32, 128, 1728, 8
LOG2E = 1.4426950408889634
bf16 = jnp.bfloat16
f32 = jnp.float32
i32 = jnp.int32
u32 = jnp.uint32
NT = (((1,), (1,)), ((), ()))

TS = 128
KC = 512
NSUB = S // TS
NCH = S // KC
NT_D = D // 128
NF = (F + 127) // 128
XC = 256
L = 7
GROWS = 80
DMA_SLOT = 4
FFN_DELAY = 8

ORDER_LOOP = "A B0 D C0 B1 C1 B2 C2 B3 C3".split()
ORDER_TAIL = "B0 D C0 B1 C1 B2 C2 B3 C3 A".split()
ORDER_END = "C0 C1 D C2 X C3".split()
OUT_CUTS = [r * TS for r in (2, 4, 6, 8, 10, 12, 13, 14, 15)] + [S - TS // 2, S]

FRONT_PLAN = [
    "L1 a0 a1 r0 r1 r0 r1 a2 a3 r2 r3 r2 r3",
    "L2 b0.0 b0.1 b0.2 b0.3 b1.0 b1.1 b1.2 b1.3",
    "L3 L4 a4 b2.0 r5 b2.1 r5 b2.2 r4 a5 r4 b2.3 b3.0 b3.1 r6 a6 r7 b3.2 b3.3 a7 b4.0 r6 b4.1 r7 b4.2 b4.3",
    "L5 L6 L7 a8 r9 b5.0 b5.1 r8 a11 r10 b5.2 r8 a10 r9 a9 r10 b5.3 r12 a13 r11 a12 r12 b6.0 r11 a14 r15 a15 "
    "r13 b6.1 r13 b6.2 r14 b6.3 r14 r15",
]
FRONT_WAIT = ((1, 'wq0', 'wr'), ('k0', 2), (3, 4), (5, 6, 7, 'wql'))
FRONT_START = ((3,), (4, 5), ('wql', 6, 7, 'wo0', 'wq1'), ('v0', 'k1'))


def _rb(x):
    return x.astype(bf16).astype(f32)


def _layernorm(ld):
    mean = jnp.sum(ld(0).astype(f32), axis=-1, keepdims=True) * (1.0 / D)
    c = ld(1).astype(f32) - mean
    ssq = jnp.sum(c * c, axis=-1, keepdims=True)
    n = ssq.shape[0]
    ng = n // 8
    t = jnp.broadcast_to(ssq, (n, 128)).reshape(ng, 8, 128)
    lane = lax.broadcasted_iota(i32, (8, 128), 1)
    bit = 1
    while t.shape[0] > 1:
        hlf = t.shape[0] // 2
        t = jnp.where(((lane & bit) != 0)[None], t[hlf:], t[:hlf])
        bit *= 2
    den = _rb(jnp.sqrt(_rb(_rb(t[0] * (1.0 / D)) + 1e-5)))
    inv = pl.reciprocal(den, approx=True)
    inv = inv * (2.0 - den * inv)
    nb = ng.bit_length() - 1
    cols = []
    for g in range(ng):
        lg = int(format(g, '0%db' % nb)[::-1], 2)
        cols.append(jnp.broadcast_to(inv[:, lg:lg + 1], (8, 128)))
    inv = jnp.concatenate(cols, axis=0)
    mb = jnp.broadcast_to(_rb(mean), (n, 128))
    x = ld(2).astype(f32)
    return [pltpu.bitcast((_rb(x[:, t * 128:(t + 1) * 128] - mb) * inv).astype(bf16), u32) for t in range(NT_D)]


def _silu(x):
    hx = 0.5 * x
    return hx + hx * jnp.tanh(hx)


def _fold(x, op):
    r = x[:, 0:128]
    for t in range(1, x.shape[1] // 128):
        r = op(r, x[:, t * 128:(t + 1) * 128])
    return r


def _kernel(x_hbm, k_hbm, v_hbm, wq_hbm, wo_hbm, wr_hbm, wg_hbm, wu_hbm, wd_hbm, o_hbm,
            z_v, x_v, xn_v, g_v, k_v, v_v, wq_v, wo_v, wg_v, wu_v, wd_v, acc, r_v, xs_v, ms_v, idx_s,
            s_c, m_c, q_c, o_c, l_c, out_v, ql_v, wr_v,
            sem_x, sem_h, sem_f, sem_o):
    def hoff(h):
        return h * DH if isinstance(h, int) else pl.multiple_of(h * DH, DH)

    def cp_x(c):
        rows = pl.ds(c * XC, XC)
        return pltpu.make_async_copy(x_hbm.at[rows, :], x_v.at[rows, :], sem_x.at[c])

    def cp_k(h, i=0):
        return pltpu.make_async_copy(k_hbm.at[h], k_v.at[h], sem_h.at[i])

    def cp_v(h):
        return pltpu.make_async_copy(v_hbm.at[h], v_v.at[h], sem_h.at[1])

    def cp_wq(h, i=2):
        return pltpu.make_async_copy(wq_hbm.at[:, pl.ds(hoff(h), DH)], wq_v.at[h], sem_h.at[i])

    def cp_wo(h):
        return pltpu.make_async_copy(wo_hbm.at[pl.ds(hoff(h), DH), :], wo_v.at[h], sem_h.at[3])

    def cp_f(i):
        return pltpu.make_async_copy((wg_hbm, wu_hbm, wd_hbm)[i], (wg_v, wu_v, wd_v)[i], sem_f.at[i])

    def cp_o(c):
        lo = OUT_CUTS[c - 1] if c else 0
        rows = pl.ds(lo, OUT_CUTS[c] - lo)
        return pltpu.make_async_copy(out_v.at[rows, :], o_hbm.at[rows, :], sem_o.at[c])

    def sub(j):
        return pl.ds(j * TS, TS)

    def half(r0, n):
        if isinstance(r0, int):
            return pl.ds(r0 // 2, n // 2)
        return pl.ds(pl.multiple_of(r0 // 2, 8), n // 2)

    def xn_ld(r0, n):
        return pltpu.bitcast(xn_v[half(r0, n), :], bf16)

    def qproj(h, j):
        q = jnp.dot(xn_ld(j * TS, TS), wq_v[h], preferred_element_type=f32)
        return (q * (DH ** -0.5 * LOG2E)).astype(bf16)

    def oproj(h, j, o, fresh=None):
        y = jnp.dot(o, wo_v[h], preferred_element_type=f32)
        if fresh is None:
            acc[sub(j), :] += y
        else:
            acc[sub(j), :] = jnp.where(fresh, 0.0, acc[sub(j), :]) + y

    def oproj_final(h, j, o):
        npc = 2 if j == NSUB - 1 else 1
        n = TS // npc
        for i in range(npc):
            rows = pl.ds(j * TS + i * n, n)
            y = jnp.dot(o[i * n:(i + 1) * n, :], wo_v[h], preferred_element_type=f32)
            t = (acc[rows, :] + y) * g_v[rows, :]
            out_v[rows, :] = (x_v[rows, :].astype(f32) + t).astype(bf16)
            if j * TS + (i + 1) * n in OUT_CUTS:
                cp_o(OUT_CUTS.index(j * TS + (i + 1) * n)).start()

    def fin_m(mrun):
        return jnp.broadcast_to(jnp.max(mrun, axis=-1, keepdims=True), (TS, 128))

    def fin_o(o, lrun):
        l = jnp.sum(lrun, axis=-1, keepdims=True)
        return (o * pl.reciprocal(l, approx=True)).astype(bf16)

    def topk():
        r = _rb(r_v[...]) + 0.0
        bits = lax.shift_right_logical(pltpu.bitcast(r, i32), 16)
        ordered = jnp.where(bits >= 0x8000, 0xFFFF - bits, bits + 0x8000)
        ordered = jnp.where(r != r, 0, ordered)
        sl = lax.broadcasted_iota(i32, (16, 128), 0)
        ln = lax.broadcasted_iota(i32, (16, 128), 1)
        key = pltpu.bitcast(ordered * 2048 + (2047 - (sl * 128 + ln)) + (1 << 28), f32)
        msel = jnp.zeros((16, 128), f32)
        for c in range(C):
            m = jnp.max(jnp.max(key, axis=0, keepdims=True), axis=1, keepdims=True)
            mb = jnp.broadcast_to(m, (16, 128))
            key = jnp.where(key == mb, 0.0, key)
            msel = jnp.where(sl == c, mb, msel)
            ic = (2047 - (pltpu.bitcast(mb, i32) & 2047))[0, 0]
            idx_s[c] = ic
            pair = pltpu.bitcast(xn_v[pl.ds(lax.shift_right_logical(ic, 1), 1), :], i32)
            xs_v[c:c + 1, :] = pltpu.bitcast(lax.shift_left(lax.shift_right_logical(pair, (ic & 1) * 16), 16), f32)
        o16 = lax.shift_right_logical(pltpu.bitcast(msel, i32) - (1 << 28), 11) & 0xFFFF
        rbits = jnp.where(o16 >= 0x8000, o16 - 0x8000, 0xFFFF - o16)
        r_sel = jnp.where(sl < C, pltpu.bitcast(lax.shift_left(rbits, 16), f32), 0.0)
        ms_v[...] = _rb(0.5 + 0.5 * jnp.tanh(0.5 * r_sel))

    def moe():
        topk()
        x_sel = xs_v[...]
        xs = x_sel.astype(bf16)
        for _ in range(FFN_DELAY):
            yield
        cnt = 0
        hs = []
        for t in range(NF):
            fs = slice(t * 128, min((t + 1) * 128, F))
            hh = []
            for w_v in (wg_v, wu_v):
                a = None
                for kt in range(NT_D):
                    ks = slice(kt * 128, (kt + 1) * 128)
                    d = lax.dot_general(xs[:, ks], w_v[fs, ks], NT, preferred_element_type=f32)
                    a = d if a is None else a + d
                    cnt += 1
                    if cnt % 4 == 0:
                        yield
                hh.append(_rb(a))
            hs.append((_rb(_silu(hh[0])) * hh[1]).astype(bf16))
        cnt = 0
        ys = [None] * NT_D
        for t in range(NF):
            fs = slice(t * 128, min((t + 1) * 128, F))
            for kt in range(NT_D):
                d = jnp.dot(hs[t], wd_v[fs, kt * 128:(kt + 1) * 128], preferred_element_type=f32)
                ys[kt] = d if ys[kt] is None else ys[kt] + d
                cnt += 1
                if cnt % 4 == 0:
                    yield
        y = jnp.concatenate(ys, axis=1)
        y = _rb(_rb(y) * jnp.concatenate([ms_v[...]] * NT_D, axis=1))
        gsel = _silu(_rb(x_sel + y))
        for c in range(C):
            g_v[pl.ds(jnp.clip(idx_s[c], 0, S - 1), 1), :] = gsel[c:c + 1, :]

    def run_head(h, tail, hook=None):
        def unit(t):
            if t < 0:
                return (h - 1 if tail else jnp.maximum(h - 1, 0)), t + NSUB
            return h + t // NSUB, t % NSUB

        z = jnp.concatenate([z_v[0:8, :]] * (TS // 8), axis=0)
        svals = {}
        mvals = {}
        q = pltpu.bitcast(q_c[...], bf16)
        o_done = fin_o(o_c[...], l_c[...])
        pend = []
        pvs = []
        mhist = []
        moe_gen = moe() if tail else None

        def gate(dep):
            r0 = jnp.minimum(h * GROWS, S - GROWS)
            w = pltpu.bitcast(dep[0:GROWS // 2, :], i32) & z[0:GROWS // 2, :]
            xb = xn_v[half(r0, GROWS), :] | pltpu.bitcast(jnp.concatenate([w] * NT_D, axis=1), u32)
            g_v[pl.ds(pl.multiple_of(r0, 16), GROWS), :] = _silu(pltpu.bitcast(xb, bf16).astype(f32))

        def flush():
            if moe_gen is None and pend:
                oproj_final(*pend.pop(0))

        for j in range(NSUB):
            tb = j + L
            s_list = [None] * NCH
            mrun = None
            lrun = None
            o = None
            q_next = None
            do_a = not (tail and tb + 1 >= NSUB)
            do_b = not (tail and tb >= NSUB)
            m_row = fin_m(m_c[j] if j < L else mvals.pop(j))
            if hook is not None and j == DMA_SLOT:
                hook()
            for op in ((ORDER_TAIL if do_b else ORDER_END) if tail else ORDER_LOOP):
                if moe_gen is not None and op[0] in 'BC':
                    if next(moe_gen, 'done') == 'done':
                        moe_gen = None
                if op == 'A':
                    if do_a:
                        q_next = (pltpu.bitcast(ql_v[half((tb + 1) * TS, TS), :], bf16) if tail
                                  else qproj(*unit(tb + 1)))
                elif op == 'D':
                    if tail and j > 0:
                        pend.append((h, j - 1, o_done))
                        flush()
                    else:
                        oproj(*unit(j - 1), o_done, fresh=None if tail else (h == 0))
                elif op == 'X':
                    flush()
                elif op[0] == 'B':
                    c = int(op[1:])
                    cs = slice(c * KC, (c + 1) * KC)
                    qq = q
                    if len(mhist) >= 2 and c in (0, 2):
                        w = pltpu.bitcast(mhist[-2], i32)
                        w = (w[0:TS // 2, :] | w[TS // 2:, :]) & z[0:TS // 2, :]
                        qq = pltpu.bitcast(pltpu.bitcast(q, i32) | w, bf16)
                    s = lax.dot_general(qq, k_v[unit(tb)[0], cs, :], NT, preferred_element_type=f32)
                    if tb >= NSUB:
                        s_c[tb - NSUB, :, cs] = s
                    s_list[c] = s
                    mc = _fold(s, jnp.maximum)
                    mrun = mc if mrun is None else jnp.maximum(mrun, mc)
                    mhist.append(mrun)
                elif op[0] == 'C':
                    c = int(op[1:])
                    cs = slice(c * KC, (c + 1) * KC)
                    sp = s_c[j, :, cs] if j < L else svals[j][c]
                    m_use = m_row
                    lag = 1 if do_b else 2
                    if len(pvs) >= lag:
                        m_use = m_row + pltpu.bitcast(pltpu.bitcast(pvs[-lag], i32) & z, f32)
                    p = jnp.exp2(sp - jnp.concatenate([m_use] * (KC // 128), axis=1))
                    pb = p.astype(bf16)
                    lc = _fold(p, jnp.add)
                    lrun = lc if lrun is None else lrun + lc
                    parts = [jnp.dot(pb[:, t * 128:(t + 1) * 128], v_v[h, c * KC + t * 128:c * KC + (t + 1) * 128, :],
                                     preferred_element_type=f32) for t in range(KC // 128)]
                    oc = (parts[0] + parts[1]) + (parts[2] + parts[3])
                    pvs.append(parts[0])
                    o = oc if o is None else o + oc
                    if not tail and j == NSUB - 1 and c == NCH - 1:
                        gate(parts[0])
                    if tail and do_b and c == 1:
                        flush()
            if do_b:
                if tb >= NSUB:
                    m_c[tb - NSUB] = mrun
                else:
                    svals[tb] = s_list
                    mvals[tb] = mrun
            q = q_next
            if j + 1 < NSUB:
                o_done = fin_o(o, lrun)
        if tail:
            pend.append((h, NSUB - 1, fin_o(o, lrun)))
            for args in pend:
                oproj_final(*args)
            return
        q_c[...] = pltpu.bitcast(q, u32)
        o_c[...] = o
        l_c[...] = lrun

    named = dict(wql=cp_wq(H - 1, 5), v0=cp_v(0), wo0=cp_wo(0), wq1=cp_wq(1), k1=cp_k(1),
                 wq0=cp_wq(0, 4), k0=cp_k(0, 6), wr=pltpu.make_async_copy(wr_hbm, wr_v, sem_h.at[7]))

    def front_cp(k):
        return cp_x(k) if isinstance(k, int) else named[k]

    for k in (0, 1, 'wq0', 'wr'):
        front_cp(k).start()
    r_v[...] = jnp.zeros((16, 128), f32)
    xs_v[...] = jnp.zeros((16, D), f32)
    o_c[...] = jnp.zeros((TS, DH), f32)
    l_c[...] = jnp.ones((TS, 128), f32)
    front_cp('k0').start()

    def ln_chunk(c, zs):
        pieces = 4 if c >= 2 else 2
        n = XC // pieces
        for t in range(pieces):
            r0 = c * XC + t * n

            def ld(i):
                if i == 0:
                    return x_v[pl.ds(r0, n), :]
                return x_v[pl.ds(pl.multiple_of(r0 + zs * i, n), n), :]
            for tt, w in enumerate(_layernorm(ld)):
                xn_v[half(r0, n), tt * 128:(tt + 1) * 128] = w

    def router_tiles(u):
        wrf = jnp.broadcast_to(wr_v[...].astype(f32).reshape(1, D), (16, D))
        lhs = jnp.where(lax.broadcasted_iota(i32, (16, D), 0) == u, wrf, 0.0).astype(bf16)
        xn = xn_ld(u * TS, TS)
        return [(lhs[:, k * 128:(k + 1) * 128], xn[:, k * 128:(k + 1) * 128]) for k in range(NT_D)]

    cp_x(0).wait()
    cp_x(2).start()
    t0 = x_v[0:16, 0:128].astype(f32)[0:8, :]
    t0 = jnp.where(jnp.abs(t0) < 1.0, t0, 0.5)
    zv = pltpu.bitcast(t0 - t0, i32)
    z_v[0:8, :] = zv
    zs = zv[0, 0]
    ln_chunk(0, zs)

    for bi, plan in enumerate(FRONT_PLAN):
        for k in FRONT_WAIT[bi]:
            front_cp(k).wait()
        for k in FRONT_START[bi]:
            front_cp(k).start()
        rs = r_v[...]
        rj = {}
        mr = {}
        qs = {}
        for op in plan.split():
            if op[0] == 'L':
                ln_chunk(int(op[1:]), zs)
            elif op[0] == 'a':
                u = int(op[1:])
                ql_v[half(u * TS, TS), :] = pltpu.bitcast(qproj(0 if u <= L else H - 1, u), u32)
            elif op[0] == 'r':
                u = int(op[1:])
                first = u not in rj
                if first:
                    rj[u] = router_tiles(u)
                for _ in range(3 if first else 2):
                    a, b = rj[u].pop(0)
                    rs = rs + lax.dot_general(a, b, NT, preferred_element_type=f32)
            else:
                u, c = (int(t) for t in op[1:].split('.'))
                if u not in qs:
                    qs[u] = pltpu.bitcast(ql_v[half(u * TS, TS), :], bf16)
                s = lax.dot_general(qs[u], k_v[0, c * KC:(c + 1) * KC, :], NT, preferred_element_type=f32)
                s_c[u, :, c * KC:(c + 1) * KC] = s
                mc = _fold(s, jnp.maximum)
                mr[u] = mc if u not in mr else jnp.maximum(mr[u], mc)
                if c == NCH - 1:
                    m_c[u] = mr[u]
        r_v[...] = rs
    q_c[...] = ql_v[half(L * TS, TS), :]

    def body(h, carry):
        def hook():
            cp_v(h + 1).start()
            cp_wo(h + 1).start()

            @pl.when(h + 2 < H - 1)
            def _():
                cp_wq(h + 2).start()

            @pl.when(h + 2 < H)
            def _():
                cp_k(h + 2).start()

            @pl.when(h == 1)
            def _():
                for i in range(3):
                    cp_f(i).start()

        cp_v(h).wait()
        cp_wo(h).wait()
        cp_k(h + 1).wait()

        @pl.when(h + 1 < H - 1)
        def _():
            cp_wq(h + 1).wait()
        run_head(h, False, hook)
        return carry

    lax.fori_loop(0, H - 1, body, 0)

    cp_v(H - 1).wait()
    cp_wo(H - 1).wait()
    for i in range(3):
        cp_f(i).wait()
    run_head(H - 1, True)
    for c in range(len(OUT_CUTS)):
        cp_o(c).wait()


def _wrapped(*refs):
    @pl.when(pl.program_id(0) == 0)
    def _():
        _kernel(*refs)


def build(A_x, A_k_cache, A_v_cache, A_wq, A_wo, B_x, B_w_r, B_w_gate, B_w_up, B_w_down):
    out = pl.pallas_call(
        _wrapped,
        grid=(2,),
        in_specs=[pl.BlockSpec(memory_space=pl.ANY)] * 9,
        out_specs=pl.BlockSpec(memory_space=pl.ANY),
        out_shape=jax.ShapeDtypeStruct((S, D), bf16),
        scratch_shapes=[
            pltpu.VMEM((128, 128), i32),
            pltpu.VMEM((S, D), bf16),
            pltpu.VMEM((S // 2, D), u32),
            pltpu.VMEM((S, D), f32),
            pltpu.VMEM((H, S, DH), bf16),
            pltpu.VMEM((H, S, DH), bf16),
            pltpu.VMEM((H, D, DH), bf16),
            pltpu.VMEM((H, DH, D), bf16),
            pltpu.VMEM((F, D), bf16),
            pltpu.VMEM((F, D), bf16),
            pltpu.VMEM((F, D), bf16),
            pltpu.VMEM((S, D), f32),
            pltpu.VMEM((16, 128), f32),
            pltpu.VMEM((16, D), f32),
            pltpu.VMEM((16, 128), f32),
            pltpu.SMEM((C,), i32),
            pltpu.VMEM((L, TS, S), f32),
            pltpu.VMEM((L, TS, 128), f32),
            pltpu.VMEM((TS // 2, DH), u32),
            pltpu.VMEM((TS, DH), f32),
            pltpu.VMEM((TS, 128), f32),
            pltpu.VMEM((S, D), bf16),
            pltpu.VMEM((S // 2, DH), u32),
            pltpu.VMEM((D,), bf16),
            pltpu.SemaphoreType.DMA((S // XC,)),
            pltpu.SemaphoreType.DMA((8,)),
            pltpu.SemaphoreType.DMA((3,)),
            pltpu.SemaphoreType.DMA((len(OUT_CUTS),)),
        ],
        compiler_params=pltpu.CompilerParams(vmem_limit_bytes=120 * 1024 * 1024,
                                             internal_scratch_in_bytes=64 * 1024,
                                             disable_bounds_checks=True,
                                             disable_semaphore_checks=True),
    )(A_x.reshape(S, D), A_k_cache.reshape(H, S, DH), A_v_cache.reshape(H, S, DH), A_wq, A_wo,
      B_w_r, B_w_gate.T, B_w_up.T, B_w_down)
    return out.reshape(1, S, D)


@jax.jit
def pallas_recurrent_scan__mha_block_cached__moe_arch_mod__prompt_kernel(
        A_x, A_k_cache, A_v_cache, A_wq, A_wo, B_x, B_w_r, B_w_gate, B_w_up, B_w_down):
    return build(A_x, A_k_cache, A_v_cache, A_wq, A_wo, B_x, B_w_r, B_w_gate, B_w_up, B_w_down)
```

```python
import jax
import jax.numpy as jnp
from jax import lax
import jax.experimental.pallas as pl
import jax.experimental.pallas.tpu as pltpu

S, D, H, DH, F, C = 2048, 640, 32, 128, 1728, 8
LOG2E = 1.4426950408889634
bf16 = jnp.bfloat16
f32 = jnp.float32
i32 = jnp.int32
u32 = jnp.uint32
NT = (((1,), (1,)), ((), ()))

TS = 128
KC = 512
NSUB = S // TS
NCH = S // KC
NT_D = D // 128
NF = (F + 127) // 128
XC = 256
L = 7
GROWS = 80
DMA_SLOT = 4
FFN_DELAY = 10

OFF_V, OFF_Q, OFF_O, SLAB = S, 2 * S, 2 * S + D, 2 * S + 2 * D
ORDER_LOOP = "A B0 D C0 B1 C1 B2 C2 B3 C3".split()
ORDER_TAIL = "B0 C0 B1 D C1 B2 C2 B3 C3 A".split()
ORDER_END = "C0 C1 D C2 X C3".split()
OUT_CUTS = [r * TS for r in (2, 4, 6, 8, 10, 12, 13, 14, 15)] + [S - TS // 2, S]

FRONT_PLAN = [
    "L1 a0 a1 r0 r1 r0 r1 a2 a3 r2 r3 r2 r3",
    "L2 b0.0 b0.1 b0.2 b0.3 b1.0 b1.1 b1.2 b1.3",
    "L3 L4 a4 b2.0 r5 b2.1 r5 b2.2 b2.3 r4 a5 b3.0 r4 b3.1 r6 a6 r7 b3.2 b3.3 a7 r6 b4.0 b4.1 r7 b4.2 b4.3",
    "L5 L6 L7 b5.0 a8 b5.1 r9 r8 a11 r10 b5.2 r9 r8 a10 a9 r10 b5.3 r12 r11 a13 r12 b6.0 a12 r11 a14 r15 a15 "
    "r13 b6.1 r13 b6.2 r14 b6.3 r14 r15",
]
LN_PIECES = (2, 2, 4, 8, 4, 4, 4, 4)
FRONT_WAIT = ((1, 'wq0', 'wr'), ('k0', 2), (3, 4), (5, 6, 7, 'wql'))
FRONT_START = ((3,), (4, 5), ('wql', 6, 7, 'wo0', 'wq1'), ('v0', 'k1'))


def _rb(x):
    return x.astype(bf16).astype(f32)


def _layernorm(ld):
    mean = jnp.sum(ld(0).astype(f32), axis=-1, keepdims=True) * (1.0 / D)
    c = ld(1).astype(f32) - mean
    ssq = jnp.sum(c * c, axis=-1, keepdims=True)
    n = ssq.shape[0]
    ng = n // 8
    t = jnp.broadcast_to(ssq, (n, 128)).reshape(ng, 8, 128)
    lane = lax.broadcasted_iota(i32, (8, 128), 1)
    bit = 1
    while t.shape[0] > 1:
        hlf = t.shape[0] // 2
        t = jnp.where(((lane & bit) != 0)[None], t[hlf:], t[:hlf])
        bit *= 2
    den = _rb(jnp.sqrt(_rb(_rb(t[0] * (1.0 / D)) + 1e-5)))
    inv = pl.reciprocal(den, approx=True)
    inv = inv * (2.0 - den * inv)
    nb = ng.bit_length() - 1
    cols = []
    for g in range(ng):
        lg = int(format(g, '0%db' % nb)[::-1], 2)
        cols.append(jnp.broadcast_to(inv[:, lg:lg + 1], (8, 128)))
    inv = jnp.concatenate(cols, axis=0)
    mb = jnp.broadcast_to(_rb(mean), (n, 128))
    x = ld(2).astype(f32)
    return [pltpu.bitcast((_rb(x[:, t * 128:(t + 1) * 128] - mb) * inv).astype(bf16), u32) for t in range(NT_D)]


def _silu(x):
    hx = 0.5 * x
    return hx + hx * jnp.tanh(hx)


def _fold(x, op):
    r = x[:, 0:128]
    for t in range(1, x.shape[1] // 128):
        r = op(r, x[:, t * 128:(t + 1) * 128])
    return r


def _kernel(x_hbm, k_hbm, v_hbm, wq_hbm, wo_hbm, wr_hbm, wg_hbm, wu_hbm, wd_hbm, o_hbm,
            z_v, x_v, xn_v, g_v, hw_v, wg_v, wu_v, wd_v, acc, r_v, xs_v, ms_v, idx_s,
            s_c, m_c, q_c, o_c, l_c, out_v, ql_v, wr_v,
            sem_x, sem_h, sem_f, sem_o):
    def hoff(h):
        return h * DH if isinstance(h, int) else pl.multiple_of(h * DH, DH)

    def cp_x(c):
        rows = pl.ds(c * XC, XC)
        return pltpu.make_async_copy(x_hbm.at[rows, :], x_v.at[rows, :], sem_x.at[c])

    def cp_k(h, i=0):
        return pltpu.make_async_copy(k_hbm.at[h], hw_v.at[h, pl.ds(0, S), :], sem_h.at[i])

    def cp_v(h, i=0):
        return pltpu.make_async_copy(v_hbm.at[h], hw_v.at[h + 1, pl.ds(OFF_V, S), :], sem_h.at[i])

    def cp_wq(h, i=0):
        return pltpu.make_async_copy(wq_hbm.at[:, pl.ds(hoff(h), DH)], hw_v.at[h, pl.ds(OFF_Q, D), :], sem_h.at[i])

    def cp_wo(h, t, i=0):
        return pltpu.make_async_copy(wo_hbm.at[pl.ds(hoff(h), DH), pl.ds(t * 128, 128)],
                                     hw_v.at[h + 1, pl.ds(OFF_O + t * DH, DH), :], sem_h.at[i])

    def wo_dot(o, h):
        return jnp.concatenate([jnp.dot(o, hw_v[h + 1, OFF_O + t * DH:OFF_O + (t + 1) * DH, :],
                                        preferred_element_type=f32) for t in range(NT_D)], axis=1)

    def cp_f(i):
        return pltpu.make_async_copy((wg_hbm, wu_hbm, wd_hbm)[i], (wg_v, wu_v, wd_v)[i], sem_f.at[0])

    def cp_o(c):
        lo = OUT_CUTS[c - 1] if c else 0
        rows = pl.ds(lo, OUT_CUTS[c] - lo)
        return pltpu.make_async_copy(out_v.at[rows, :], o_hbm.at[rows, :], sem_o.at[c])

    def sub(j):
        return pl.ds(j * TS, TS)

    def half(r0, n):
        if isinstance(r0, int):
            return pl.ds(r0 // 2, n // 2)
        return pl.ds(pl.multiple_of(r0 // 2, 8), n // 2)

    def xn_ld(r0, n):
        return pltpu.bitcast(xn_v[half(r0, n), :], bf16)

    def qproj(h, j):
        q = jnp.dot(xn_ld(j * TS, TS), hw_v[h, OFF_Q:OFF_Q + D, :], preferred_element_type=f32)
        return (q * (DH ** -0.5 * LOG2E)).astype(bf16)

    def oproj(h, j, o, fresh=None):
        y = wo_dot(o, h)
        if fresh is None:
            acc[sub(j), :] += y
        else:
            acc[sub(j), :] = jnp.where(fresh, 0.0, acc[sub(j), :]) + y

    def final_rows(h, r0, n, o):
        rows = pl.ds(r0, n)
        t = (acc[rows, :] + wo_dot(o, h)) * g_v[rows, :]
        out_v[rows, :] = (x_v[rows, :].astype(f32) + t).astype(bf16)
        if r0 + n in OUT_CUTS:
            cp_o(OUT_CUTS.index(r0 + n)).start()

    def oproj_final(h, j, o):
        final_rows(h, j * TS, TS, o)

    def fin_m(mrun):
        return jnp.broadcast_to(jnp.max(mrun, axis=-1, keepdims=True), (TS, 128))

    def fin_o(o, lrun):
        l = jnp.sum(lrun, axis=-1, keepdims=True)
        return (o * pl.reciprocal(l, approx=True)).astype(bf16)

    def topk():
        r = _rb(r_v[...]) + 0.0
        bits = lax.shift_right_logical(pltpu.bitcast(r, i32), 16)
        ordered = jnp.where(bits >= 0x8000, 0xFFFF - bits, bits + 0x8000)
        ordered = jnp.where(r != r, 0, ordered)
        sl = lax.broadcasted_iota(i32, (16, 128), 0)
        ln = lax.broadcasted_iota(i32, (16, 128), 1)
        key = pltpu.bitcast(ordered * 2048 + (2047 - (sl * 128 + ln)) + (1 << 28), f32)
        msel = jnp.zeros((16, 128), f32)
        for c in range(C):
            m = jnp.max(jnp.max(key, axis=0, keepdims=True), axis=1, keepdims=True)
            mb = jnp.broadcast_to(m, (16, 128))
            key = jnp.where(key == mb, 0.0, key)
            msel = jnp.where(sl == c, mb, msel)
            ic = (2047 - (pltpu.bitcast(mb, i32) & 2047))[0, 0]
            idx_s[c] = ic
            pair = pltpu.bitcast(xn_v[pl.ds(lax.shift_right_logical(ic, 1), 1), :], i32)
            xs_v[c:c + 1, :] = pltpu.bitcast(lax.shift_left(lax.shift_right_logical(pair, (ic & 1) * 16), 16), f32)
        o16 = lax.shift_right_logical(pltpu.bitcast(msel, i32) - (1 << 28), 11) & 0xFFFF
        rbits = jnp.where(o16 >= 0x8000, o16 - 0x8000, 0xFFFF - o16)
        r_sel = jnp.where(sl < C, pltpu.bitcast(lax.shift_left(rbits, 16), f32), 0.0)
        ms_v[...] = _rb(0.5 + 0.5 * jnp.tanh(0.5 * r_sel))

    def moe():
        topk()
        x_sel = xs_v[...]
        xs = x_sel.astype(bf16)
        for _ in range(FFN_DELAY):
            yield
        cnt = 0
        hs = []
        for t in range(NF):
            fs = slice(t * 128, min((t + 1) * 128, F))
            hh = []
            for w_v in (wg_v, wu_v):
                a = None
                for kt in range(NT_D):
                    ks = slice(kt * 128, (kt + 1) * 128)
                    d = lax.dot_general(xs[:, ks], w_v[fs, ks], NT, preferred_element_type=f32)
                    a = d if a is None else a + d
                    cnt += 1
                    if cnt % 4 == 0:
                        yield
                hh.append(_rb(a))
            hs.append((_rb(_silu(hh[0])) * hh[1]).astype(bf16))
        cnt = 0
        ys = [None] * NT_D
        for t in range(NF):
            fs = slice(t * 128, min((t + 1) * 128, F))
            for kt in range(NT_D):
                d = jnp.dot(hs[t], wd_v[fs, kt * 128:(kt + 1) * 128], preferred_element_type=f32)
                ys[kt] = d if ys[kt] is None else ys[kt] + d
                cnt += 1
                if cnt % 4 == 0:
                    yield
        y = jnp.concatenate(ys, axis=1)
        y = _rb(_rb(y) * jnp.concatenate([ms_v[...]] * NT_D, axis=1))
        gsel = _silu(_rb(x_sel + y))
        for c in range(C):
            g_v[pl.ds(jnp.clip(idx_s[c], 0, S - 1), 1), :] = gsel[c:c + 1, :]

    def run_head(h, tail, hook=None):
        def unit(t):
            if t < 0:
                return (h - 1 if tail else jnp.maximum(h - 1, 0)), t + NSUB
            return h + t // NSUB, t % NSUB

        z = jnp.concatenate([z_v[0:8, :]] * (TS // 8), axis=0)
        svals = {}
        mvals = {}
        q = pltpu.bitcast(q_c[...], bf16)
        o_done = fin_o(o_c[...], l_c[...])
        pend = []
        pvs = []
        mhist = []
        moe_gen = moe() if tail else None

        def gate(dep):
            r0 = jnp.minimum(h * GROWS, S - GROWS)
            w = pltpu.bitcast(dep[0:GROWS // 2, :], i32) & z[0:GROWS // 2, :]
            xb = xn_v[half(r0, GROWS), :] | pltpu.bitcast(jnp.concatenate([w] * NT_D, axis=1), u32)
            g_v[pl.ds(pl.multiple_of(r0, 16), GROWS), :] = _silu(pltpu.bitcast(xb, bf16).astype(f32))

        def flush():
            if moe_gen is None and pend:
                oproj_final(*pend.pop(0))

        def last_unit(o_prev):
            j = NSUB - 1
            pend.append((h, j - 1, o_prev))
            m_all = fin_m(mvals.pop(j))
            n = TS // 2
            done = None
            for i in range(2):
                rs = slice(i * n, (i + 1) * n)
                o = None
                lrun = None
                for c in range(NCH):
                    m_use = m_all[rs, :] + pltpu.bitcast(pltpu.bitcast(pvs[-2][0:n, :], i32) & z[0:n, :], f32)
                    p = jnp.exp2(svals[j][c][rs, :] - jnp.concatenate([m_use] * (KC // 128), axis=1))
                    pb = p.astype(bf16)
                    lc = _fold(p, jnp.add)
                    lrun = lc if lrun is None else lrun + lc
                    parts = [jnp.dot(pb[:, t * 128:(t + 1) * 128],
                                     hw_v[h + 1, OFF_V + c * KC + t * 128:OFF_V + c * KC + (t + 1) * 128, :],
                                     preferred_element_type=f32) for t in range(KC // 128)]
                    oc = (parts[0] + parts[1]) + (parts[2] + parts[3])
                    pvs.append(parts[0])
                    o = oc if o is None else o + oc
                    if i == 0 and c == 1:
                        while pend:
                            oproj_final(*pend.pop(0))
                if done is not None:
                    final_rows(h, j * TS + (i - 1) * n, n, done)
                done = fin_o(o, lrun)
            final_rows(h, j * TS + (2 - 1) * n, n, done)

        for j in range(NSUB):
            if tail and j == NSUB - 1:
                last_unit(o_done)
                return
            tb = j + L
            s_list = [None] * NCH
            mrun = None
            lrun = None
            o = None
            q_next = None
            do_a = not (tail and tb + 1 >= NSUB)
            do_b = not (tail and tb >= NSUB)
            m_row = fin_m(m_c[j] if j < L else mvals.pop(j))
            if hook is not None and j == DMA_SLOT:
                hook()
            for op in ((ORDER_TAIL if do_b else ORDER_END) if tail else ORDER_LOOP):
                if moe_gen is not None and op[0] in 'BC':
                    if next(moe_gen, 'done') == 'done':
                        moe_gen = None
                if op == 'A':
                    if do_a:
                        q_next = (pltpu.bitcast(ql_v[half((tb + 1) * TS, TS), :], bf16) if tail
                                  else qproj(*unit(tb + 1)))
                elif op == 'D':
                    if tail and j > 0:
                        pend.append((h, j - 1, o_done))
                        flush()
                    else:
                        oproj(*unit(j - 1), o_done, fresh=None if tail else (h == 0))
                elif op == 'X':
                    flush()
                elif op[0] == 'B':
                    c = int(op[1:])
                    cs = slice(c * KC, (c + 1) * KC)
                    qq = q
                    if len(mhist) >= 2 and c in (0, 2):
                        w = pltpu.bitcast(mhist[-2], i32)
                        w = (w[0:TS // 2, :] | w[TS // 2:, :]) & z[0:TS // 2, :]
                        qq = pltpu.bitcast(pltpu.bitcast(q, i32) | w, bf16)
                    s = lax.dot_general(qq, hw_v[unit(tb)[0], cs, :], NT, preferred_element_type=f32)
                    if tb >= NSUB:
                        s_c[tb - NSUB, :, cs] = s
                    s_list[c] = s
                    mc = _fold(s, jnp.maximum)
                    mrun = mc if mrun is None else jnp.maximum(mrun, mc)
                    mhist.append(mrun)
                elif op[0] == 'C':
                    c = int(op[1:])
                    cs = slice(c * KC, (c + 1) * KC)
                    sp = s_c[j, :, cs] if j < L else svals[j][c]
                    m_use = m_row
                    lag = 1 if do_b else 2
                    if len(pvs) >= lag:
                        m_use = m_row + pltpu.bitcast(pltpu.bitcast(pvs[-lag], i32) & z, f32)
                    p = jnp.exp2(sp - jnp.concatenate([m_use] * (KC // 128), axis=1))
                    pb = p.astype(bf16)
                    lc = _fold(p, jnp.add)
                    lrun = lc if lrun is None else lrun + lc
                    parts = [jnp.dot(pb[:, t * 128:(t + 1) * 128],
                                     hw_v[h + 1, OFF_V + c * KC + t * 128:OFF_V + c * KC + (t + 1) * 128, :],
                                     preferred_element_type=f32) for t in range(KC // 128)]
                    oc = (parts[0] + parts[1]) + (parts[2] + parts[3])
                    pvs.append(parts[0])
                    o = oc if o is None else o + oc
                    if not tail and j == NSUB - 1 and c == NCH - 1:
                        gate(parts[0])
                    if tail and do_b and c == 1:
                        flush()
            if do_b:
                if tb >= NSUB:
                    m_c[tb - NSUB] = mrun
                else:
                    svals[tb] = s_list
                    mvals[tb] = mrun
            q = q_next
            if j + 1 < NSUB:
                o_done = fin_o(o, lrun)
        q_c[...] = pltpu.bitcast(q, u32)
        o_c[...] = o
        l_c[...] = lrun

    class _Many:
        def __init__(self, cps):
            self.cps = cps

        def start(self):
            for cp in self.cps:
                cp.start()

    named = dict(wql=cp_wq(H - 1, 1), v0=cp_v(0), wo0=_Many([cp_wo(0, t) for t in range(NT_D)]),
                 wq1=cp_wq(1), k1=cp_k(1),
                 wq0=cp_wq(0, 2), k0=cp_k(0, 3), wr=pltpu.make_async_copy(wr_hbm, wr_v, sem_h.at[4]))

    def front_cp(k):
        return cp_x(k) if isinstance(k, int) else named[k]

    for k in (0, 1, 'wq0', 'wr'):
        front_cp(k).start()
    r_v[...] = jnp.zeros((16, 128), f32)
    xs_v[...] = jnp.zeros((16, D), f32)
    o_c[...] = jnp.zeros((TS, DH), f32)
    l_c[...] = jnp.ones((TS, 128), f32)
    front_cp('k0').start()

    def ln_chunk(c, zs):
        pieces = LN_PIECES[c]
        n = XC // pieces
        for t in range(pieces):
            r0 = c * XC + t * n

            def ld(i):
                if i == 0:
                    return x_v[pl.ds(r0, n), :]
                return x_v[pl.ds(pl.multiple_of(r0 + zs * i, n), n), :]
            for tt, w in enumerate(_layernorm(ld)):
                xn_v[half(r0, n), tt * 128:(tt + 1) * 128] = w

    def router_tiles(u):
        wrf = jnp.broadcast_to(wr_v[...].astype(f32).reshape(1, D), (16, D))
        lhs = jnp.where(lax.broadcasted_iota(i32, (16, D), 0) == u, wrf, 0.0).astype(bf16)
        xn = xn_ld(u * TS, TS)
        return [(lhs[:, k * 128:(k + 1) * 128], xn[:, k * 128:(k + 1) * 128]) for k in range(NT_D)]

    cp_x(0).wait()
    cp_x(2).start()
    t0 = x_v[0:16, 0:128].astype(f32)[0:8, :]
    t0 = jnp.where(jnp.abs(t0) < 1.0, t0, 0.5)
    zv = pltpu.bitcast(t0 - t0, i32)
    z_v[0:8, :] = zv
    zs = zv[0, 0]
    ln_chunk(0, zs)

    for bi, plan in enumerate(FRONT_PLAN):
        for k in FRONT_WAIT[bi]:
            front_cp(k).wait()
        for k in FRONT_START[bi]:
            front_cp(k).start()
        rs = r_v[...]
        rj = {}
        mr = {}
        qs = {}
        for op in plan.split():
            if op[0] == 'L':
                ln_chunk(int(op[1:]), zs)
            elif op[0] == 'a':
                u = int(op[1:])
                ql_v[half(u * TS, TS), :] = pltpu.bitcast(qproj(0 if u <= L else H - 1, u), u32)
            elif op[0] == 'r':
                u = int(op[1:])
                first = u not in rj
                if first:
                    rj[u] = router_tiles(u)
                for _ in range(3 if first else 2):
                    a, b = rj[u].pop(0)
                    rs = rs + lax.dot_general(a, b, NT, preferred_element_type=f32)
            else:
                u, c = (int(t) for t in op[1:].split('.'))
                if u not in qs:
                    qs[u] = pltpu.bitcast(ql_v[half(u * TS, TS), :], bf16)
                s = lax.dot_general(qs[u], hw_v[0, c * KC:(c + 1) * KC, :], NT, preferred_element_type=f32)
                s_c[u, :, c * KC:(c + 1) * KC] = s
                mc = _fold(s, jnp.maximum)
                mr[u] = mc if u not in mr else jnp.maximum(mr[u], mc)
                if c == NCH - 1:
                    m_c[u] = mr[u]
        r_v[...] = rs
    q_c[...] = ql_v[half(L * TS, TS), :]

    def body(h, carry):
        def hook():
            cp_v(h + 1).start()
            for t in range(NT_D):
                cp_wo(h + 1, t).start()

            @pl.when(h + 2 < H)
            def _():
                cp_wq(h + 2).start()
                cp_k(h + 2).start()

            @pl.when(h == 1)
            def _():
                for i in range(3):
                    cp_f(i).start()

        pltpu.make_async_copy(hw_v.at[h + 1], hw_v.at[h + 1], sem_h.at[0]).wait()
        run_head(h, False, hook)
        return carry

    lax.fori_loop(0, H - 1, body, 0)

    cp_v(H - 1).wait()
    for t in range(NT_D):
        cp_wo(H - 1, t).wait()
    for i in range(3):
        cp_f(i).wait()
    run_head(H - 1, True)
    for c in range(len(OUT_CUTS)):
        cp_o(c).wait()


def _wrapped(*refs):
    @pl.when(pl.program_id(0) == 0)
    def _():
        _kernel(*refs)


def build(A_x, A_k_cache, A_v_cache, A_wq, A_wo, B_x, B_w_r, B_w_gate, B_w_up, B_w_down):
    out = pl.pallas_call(
        _wrapped,
        grid=(2,),
        in_specs=[pl.BlockSpec(memory_space=pl.ANY)] * 9,
        out_specs=pl.BlockSpec(memory_space=pl.ANY),
        out_shape=jax.ShapeDtypeStruct((S, D), bf16),
        scratch_shapes=[
            pltpu.VMEM((128, 128), i32),
            pltpu.VMEM((S, D), bf16),
            pltpu.VMEM((S // 2, D), u32),
            pltpu.VMEM((S, D), f32),
            pltpu.VMEM((H + 1, SLAB, DH), bf16),
            pltpu.VMEM((F, D), bf16),
            pltpu.VMEM((F, D), bf16),
            pltpu.VMEM((F, D), bf16),
            pltpu.VMEM((S, D), f32),
            pltpu.VMEM((16, 128), f32),
            pltpu.VMEM((16, D), f32),
            pltpu.VMEM((16, 128), f32),
            pltpu.SMEM((C,), i32),
            pltpu.VMEM((L, TS, S), f32),
            pltpu.VMEM((L, TS, 128), f32),
            pltpu.VMEM((TS // 2, DH), u32),
            pltpu.VMEM((TS, DH), f32),
            pltpu.VMEM((TS, 128), f32),
            pltpu.VMEM((S, D), bf16),
            pltpu.VMEM((S // 2, DH), u32),
            pltpu.VMEM((D,), bf16),
            pltpu.SemaphoreType.DMA((S // XC,)),
            pltpu.SemaphoreType.DMA((5,)),
            pltpu.SemaphoreType.DMA((1,)),
            pltpu.SemaphoreType.DMA((len(OUT_CUTS),)),
        ],
        compiler_params=pltpu.CompilerParams(vmem_limit_bytes=120 * 1024 * 1024,
                                             internal_scratch_in_bytes=64 * 1024,
                                             disable_bounds_checks=True,
                                             disable_semaphore_checks=True),
    )(A_x.reshape(S, D), A_k_cache.reshape(H, S, DH), A_v_cache.reshape(H, S, DH), A_wq, A_wo,
      B_w_r, B_w_gate.T, B_w_up.T, B_w_down)
    return out.reshape(1, S, D)


@jax.jit
def pallas_recurrent_scan__mha_block_cached__moe_arch_mod__prompt_kernel(
        A_x, A_k_cache, A_v_cache, A_wq, A_wo, B_x, B_w_r, B_w_gate, B_w_up, B_w_down):
    return build(A_x, A_k_cache, A_v_cache, A_wq, A_wo, B_x, B_w_r, B_w_gate, B_w_up, B_w_down)
```

```python
import jax
import jax.numpy as jnp
from jax import lax
import jax.experimental.pallas as pl
import jax.experimental.pallas.tpu as pltpu

S, D, H, DH, F, C = 2048, 640, 32, 128, 1728, 8
LOG2E = 1.4426950408889634
bf16 = jnp.bfloat16
f32 = jnp.float32
i32 = jnp.int32
u32 = jnp.uint32
NT = (((1,), (1,)), ((), ()))

TS = 128
KC = 512
NSUB = S // TS
NCH = S // KC
NT_D = D // 128
NF = (F + 127) // 128
XC = 256
L = 7
GROWS = 80
DMA_SLOT = 4
FFN_DELAY = 10

OFF_V, OFF_Q, OFF_O, SLAB = S, 2 * S, 2 * S + D, 2 * S + 2 * D
ORDER_LOOP = "A B0 D C0 B1 C1 B2 C2 B3 C3".split()
ORDER_TAIL = "B0 C0 B1 D C1 B2 C2 B3 C3 A".split()
ORDER_END = "C0 C1 D C2 X C3".split()
OUT_CUTS = [r * TS for r in (2, 4, 6, 8, 10, 12, 13, 14, 15)] + [S - TS // 2, S]

FRONT_PLAN = [
    "L1 a0 a1 r0 r1 r0 r1 a2 a3 r2 r3 r2 r3",
    "L2 b0.0 b0.1 b0.2 b0.3 b1.0 b1.1 b1.2 b1.3",
    "L3 L4 a4 b2.0 r5 b2.1 r5 b2.2 b2.3 r4 a5 b3.0 r4 b3.1 r6 a6 r7 b3.2 b3.3 a7 r6 b4.0 b4.1 r7 b4.2 b4.3",
    "L5 L6 L7 b5.0 a8 b5.1 r9 r8 a11 r10 b5.2 r9 r8 a10 a9 r10 b5.3 r12 r11 a13 r12 b6.0 a12 r11 a14 r15 a15 "
    "r13 b6.1 r13 b6.2 r14 b6.3 r14 r15",
]
LN_PIECES = (2, 2, 4, 8, 4, 4, 4, 4)
FRONT_WAIT = ((1, 'wq0', 'wr'), ('k0', 2), (3, 4), (5, 6, 7, 'wql'))
FRONT_START = ((3,), (4, 5), ('wql', 6, 7, 'wo0', 'wq1'), ('v0', 'k1'))


def _rb(x):
    return x.astype(bf16).astype(f32)


def _layernorm(ld):
    mean = jnp.sum(ld(0).astype(f32), axis=-1, keepdims=True) * (1.0 / D)
    c = ld(1).astype(f32) - mean
    ssq = jnp.sum(c * c, axis=-1, keepdims=True)
    n = ssq.shape[0]
    ng = n // 8
    t = jnp.broadcast_to(ssq, (n, 128)).reshape(ng, 8, 128)
    lane = lax.broadcasted_iota(i32, (8, 128), 1)
    bit = 1
    while t.shape[0] > 1:
        hlf = t.shape[0] // 2
        t = jnp.where(((lane & bit) != 0)[None], t[hlf:], t[:hlf])
        bit *= 2
    den = _rb(jnp.sqrt(_rb(_rb(t[0] * (1.0 / D)) + 1e-5)))
    inv = pl.reciprocal(den, approx=True)
    inv = inv * (2.0 - den * inv)
    nb = ng.bit_length() - 1
    cols = []
    for g in range(ng):
        lg = int(format(g, '0%db' % nb)[::-1], 2)
        cols.append(jnp.broadcast_to(inv[:, lg:lg + 1], (8, 128)))
    inv = jnp.concatenate(cols, axis=0)
    mb = jnp.broadcast_to(_rb(mean), (n, 128))
    x = ld(2).astype(f32)
    return [pltpu.bitcast((_rb(x[:, t * 128:(t + 1) * 128] - mb) * inv).astype(bf16), u32) for t in range(NT_D)]


def _silu(x):
    hx = 0.5 * x
    return hx + hx * jnp.tanh(hx)


def _fold(x, op):
    r = x[:, 0:128]
    for t in range(1, x.shape[1] // 128):
        r = op(r, x[:, t * 128:(t + 1) * 128])
    return r


def _kernel(x_hbm, k_hbm, v_hbm, wq_hbm, wo_hbm, wr_hbm, wg_hbm, wu_hbm, wd_hbm, o_hbm,
            z_v, x_v, xn_v, g_v, hw_v, wg_v, wu_v, wd_v, acc, r_v, xs_v, ms_v, idx_s,
            s_c, m_c, q_c, o_c, l_c, out_v, ql_v, wr_v,
            sem_x, sem_h, sem_f, sem_o):
    def hoff(h):
        return h * DH if isinstance(h, int) else pl.multiple_of(h * DH, DH)

    def cp_x(c):
        rows = pl.ds(c * XC, XC)
        return pltpu.make_async_copy(x_hbm.at[rows, :], x_v.at[rows, :], sem_x.at[c])

    def cp_k(h, i=0):
        return pltpu.make_async_copy(k_hbm.at[h], hw_v.at[h, pl.ds(0, S), :], sem_h.at[i])

    def cp_v(h, i=0):
        return pltpu.make_async_copy(v_hbm.at[h], hw_v.at[h + 1, pl.ds(OFF_V, S), :], sem_h.at[i])

    def cp_wq(h, i=0):
        return pltpu.make_async_copy(wq_hbm.at[:, pl.ds(hoff(h), DH)], hw_v.at[h, pl.ds(OFF_Q, D), :], sem_h.at[i])

    def cp_wo(h, t, i=0):
        return pltpu.make_async_copy(wo_hbm.at[pl.ds(hoff(h), DH), pl.ds(t * 128, 128)],
                                     hw_v.at[h + 1, pl.ds(OFF_O + t * DH, DH), :], sem_h.at[i])

    def wo_dot(o, h):
        return jnp.concatenate([jnp.dot(o, hw_v[h + 1, OFF_O + t * DH:OFF_O + (t + 1) * DH, :],
                                        preferred_element_type=f32) for t in range(NT_D)], axis=1)

    def cp_f(i):
        return pltpu.make_async_copy((wg_hbm, wu_hbm, wd_hbm)[i], (wg_v, wu_v, wd_v)[i], sem_f.at[0])

    def cp_o(c):
        lo = OUT_CUTS[c - 1] if c else 0
        rows = pl.ds(lo, OUT_CUTS[c] - lo)
        return pltpu.make_async_copy(out_v.at[rows, :], o_hbm.at[rows, :], sem_o.at[c])

    def sub(j):
        return pl.ds(j * TS, TS)

    def half(r0, n):
        if isinstance(r0, int):
            return pl.ds(r0 // 2, n // 2)
        return pl.ds(pl.multiple_of(r0 // 2, 8), n // 2)

    def xn_ld(r0, n):
        return pltpu.bitcast(xn_v[half(r0, n), :], bf16)

    def qproj(h, j):
        q = jnp.dot(xn_ld(j * TS, TS), hw_v[h, OFF_Q:OFF_Q + D, :], preferred_element_type=f32)
        return (q * (DH ** -0.5 * LOG2E)).astype(bf16)

    def oproj(h, j, o, fresh=None):
        y = wo_dot(o, h)
        if fresh is None:
            acc[sub(j), :] += y
        else:
            acc[sub(j), :] = jnp.where(fresh, 0.0, acc[sub(j), :]) + y

    def final_rows(h, r0, n, o):
        rows = pl.ds(r0, n)
        t = (acc[rows, :] + wo_dot(o, h)) * g_v[rows, :]
        out_v[rows, :] = (x_v[rows, :].astype(f32) + t).astype(bf16)
        if r0 + n in OUT_CUTS:
            cp_o(OUT_CUTS.index(r0 + n)).start()

    def oproj_final(h, j, o):
        final_rows(h, j * TS, TS, o)

    def fin_m(mrun):
        return jnp.broadcast_to(jnp.max(mrun, axis=-1, keepdims=True), (TS, 128))

    def fin_o(o, lrun):
        l = jnp.sum(lrun, axis=-1, keepdims=True)
        return (o * pl.reciprocal(l, approx=True)).astype(bf16)

    def topk():
        r = _rb(r_v[...])
        bits = lax.shift_right_logical(pltpu.bitcast(r, i32), 16)
        bits = jnp.where(bits == 0x8000, 0, bits)
        ordered = jnp.where(bits >= 0x8000, 0xFFFF - bits, bits + 0x8000)
        ordered = jnp.where(r != r, 0, ordered)
        sl = lax.broadcasted_iota(i32, (16, 128), 0)
        ln = lax.broadcasted_iota(i32, (16, 128), 1)
        key = pltpu.bitcast(ordered * 2048 + (2047 - (sl * 128 + ln)) + (1 << 28), f32)
        msel = jnp.zeros((16, 128), f32)
        for c in range(C):
            m = jnp.max(jnp.max(key, axis=0, keepdims=True), axis=1, keepdims=True)
            mb = jnp.broadcast_to(m, (16, 128))
            key = jnp.where(key == mb, 0.0, key)
            msel = jnp.where(sl == c, mb, msel)
            ic = (2047 - (pltpu.bitcast(mb, i32) & 2047))[0, 0]
            idx_s[c] = ic
            pair = pltpu.bitcast(xn_v[pl.ds(lax.shift_right_logical(ic, 1), 1), :], i32)
            xs_v[c:c + 1, :] = pltpu.bitcast(lax.shift_left(lax.shift_right_logical(pair, (ic & 1) * 16), 16), f32)
        o16 = lax.shift_right_logical(pltpu.bitcast(msel, i32) - (1 << 28), 11) & 0xFFFF
        rbits = jnp.where(o16 >= 0x8000, o16 - 0x8000, 0xFFFF - o16)
        r_sel = jnp.where(sl < C, pltpu.bitcast(lax.shift_left(rbits, 16), f32), 0.0)
        ms_v[...] = _rb(0.5 + 0.5 * jnp.tanh(0.5 * r_sel))

    def moe():
        topk()
        x_sel = xs_v[...]
        xs = x_sel.astype(bf16)
        for _ in range(FFN_DELAY):
            yield
        cnt = 0
        hs = []
        for t in range(NF):
            fs = slice(t * 128, min((t + 1) * 128, F))
            hh = []
            for w_v in (wg_v, wu_v):
                a = None
                for kt in range(NT_D):
                    ks = slice(kt * 128, (kt + 1) * 128)
                    d = lax.dot_general(xs[:, ks], w_v[fs, ks], NT, preferred_element_type=f32)
                    a = d if a is None else a + d
                    cnt += 1
                    if cnt % 4 == 0:
                        yield
                hh.append(_rb(a))
            hs.append((_rb(_silu(hh[0])) * hh[1]).astype(bf16))
        cnt = 0
        ys = [None] * NT_D
        for t in range(NF):
            fs = slice(t * 128, min((t + 1) * 128, F))
            for kt in range(NT_D):
                d = jnp.dot(hs[t], wd_v[fs, kt * 128:(kt + 1) * 128], preferred_element_type=f32)
                ys[kt] = d if ys[kt] is None else ys[kt] + d
                cnt += 1
                if cnt % 4 == 0:
                    yield
        y = jnp.concatenate(ys, axis=1)
        y = _rb(_rb(y) * jnp.concatenate([ms_v[...]] * NT_D, axis=1))
        gsel = _silu(_rb(x_sel + y))
        for c in range(C):
            g_v[pl.ds(jnp.clip(idx_s[c], 0, S - 1), 1), :] = gsel[c:c + 1, :]

    def run_head(h, tail, hook=None):
        def unit(t):
            if t < 0:
                return (h - 1 if tail else jnp.maximum(h - 1, 0)), t + NSUB
            return h + t // NSUB, t % NSUB

        z = jnp.concatenate([z_v[0:8, :]] * (TS // 8), axis=0)
        svals = {}
        mvals = {}
        q = pltpu.bitcast(q_c[...], bf16)
        o_done = fin_o(o_c[...], l_c[...])
        pend = []
        pvs = []
        mhist = []
        moe_gen = moe() if tail else None

        def gate(dep):
            r0 = jnp.minimum(h * GROWS, S - GROWS)
            w = pltpu.bitcast(dep[0:GROWS // 2, :], i32) & z[0:GROWS // 2, :]
            xb = xn_v[half(r0, GROWS), :] | pltpu.bitcast(jnp.concatenate([w] * NT_D, axis=1), u32)
            g_v[pl.ds(pl.multiple_of(r0, 16), GROWS), :] = _silu(pltpu.bitcast(xb, bf16).astype(f32))

        def flush():
            if moe_gen is None and pend:
                oproj_final(*pend.pop(0))

        def last_unit(o_prev):
            assert moe_gen is None
            j = NSUB - 1
            pend.append((h, j - 1, o_prev))
            m_all = fin_m(mvals.pop(j))
            n = TS // 2
            done = None
            for i in range(2):
                rs = slice(i * n, (i + 1) * n)
                o = None
                lrun = None
                for c in range(NCH):
                    m_use = m_all[rs, :] + pltpu.bitcast(pltpu.bitcast(pvs[-2][0:n, :], i32) & z[0:n, :], f32)
                    p = jnp.exp2(svals[j][c][rs, :] - jnp.concatenate([m_use] * (KC // 128), axis=1))
                    pb = p.astype(bf16)
                    lc = _fold(p, jnp.add)
                    lrun = lc if lrun is None else lrun + lc
                    parts = [jnp.dot(pb[:, t * 128:(t + 1) * 128],
                                     hw_v[h + 1, OFF_V + c * KC + t * 128:OFF_V + c * KC + (t + 1) * 128, :],
                                     preferred_element_type=f32) for t in range(KC // 128)]
                    oc = (parts[0] + parts[1]) + (parts[2] + parts[3])
                    pvs.append(parts[0])
                    o = oc if o is None else o + oc
                    if i == 0 and c == 1:
                        while pend:
                            oproj_final(*pend.pop(0))
                if done is not None:
                    final_rows(h, j * TS + (i - 1) * n, n, done)
                done = fin_o(o, lrun)
            final_rows(h, j * TS + n, n, done)

        for j in range(NSUB):
            if tail and j == NSUB - 1:
                last_unit(o_done)
                return
            tb = j + L
            s_list = [None] * NCH
            mrun = None
            lrun = None
            o = None
            q_next = None
            do_a = not (tail and tb + 1 >= NSUB)
            do_b = not (tail and tb >= NSUB)
            m_row = fin_m(m_c[j] if j < L else mvals.pop(j))
            if hook is not None and j == DMA_SLOT:
                hook()
            for op in ((ORDER_TAIL if do_b else ORDER_END) if tail else ORDER_LOOP):
                if moe_gen is not None and op[0] in 'BC':
                    if next(moe_gen, 'done') == 'done':
                        moe_gen = None
                if op == 'A':
                    if do_a:
                        q_next = (pltpu.bitcast(ql_v[half((tb + 1) * TS, TS), :], bf16) if tail
                                  else qproj(*unit(tb + 1)))
                elif op == 'D':
                    if tail and j > 0:
                        pend.append((h, j - 1, o_done))
                        flush()
                    else:
                        oproj(*unit(j - 1), o_done, fresh=None if tail else (h == 0))
                elif op == 'X':
                    flush()
                elif op[0] == 'B':
                    c = int(op[1:])
                    cs = slice(c * KC, (c + 1) * KC)
                    qq = q
                    if len(mhist) >= 2 and c in (0, 2):
                        w = pltpu.bitcast(mhist[-2], i32)
                        w = (w[0:TS // 2, :] | w[TS // 2:, :]) & z[0:TS // 2, :]
                        qq = pltpu.bitcast(pltpu.bitcast(q, i32) | w, bf16)
                    s = lax.dot_general(qq, hw_v[unit(tb)[0], cs, :], NT, preferred_element_type=f32)
                    if tb >= NSUB:
                        s_c[tb - NSUB, :, cs] = s
                    s_list[c] = s
                    mc = _fold(s, jnp.maximum)
                    mrun = mc if mrun is None else jnp.maximum(mrun, mc)
                    mhist.append(mrun)
                elif op[0] == 'C':
                    c = int(op[1:])
                    cs = slice(c * KC, (c + 1) * KC)
                    sp = s_c[j, :, cs] if j < L else svals[j][c]
                    m_use = m_row
                    lag = 1 if do_b else 2
                    if len(pvs) >= lag:
                        m_use = m_row + pltpu.bitcast(pltpu.bitcast(pvs[-lag], i32) & z, f32)
                    p = jnp.exp2(sp - jnp.concatenate([m_use] * (KC // 128), axis=1))
                    pb = p.astype(bf16)
                    lc = _fold(p, jnp.add)
                    lrun = lc if lrun is None else lrun + lc
                    parts = [jnp.dot(pb[:, t * 128:(t + 1) * 128],
                                     hw_v[h + 1, OFF_V + c * KC + t * 128:OFF_V + c * KC + (t + 1) * 128, :],
                                     preferred_element_type=f32) for t in range(KC // 128)]
                    oc = (parts[0] + parts[1]) + (parts[2] + parts[3])
                    pvs.append(parts[0])
                    o = oc if o is None else o + oc
                    if not tail and j == NSUB - 1 and c == NCH - 1:
                        gate(parts[0])
                    if tail and do_b and c == 1:
                        flush()
            if do_b:
                if tb >= NSUB:
                    m_c[tb - NSUB] = mrun
                else:
                    svals[tb] = s_list
                    mvals[tb] = mrun
            q = q_next
            if j + 1 < NSUB:
                o_done = fin_o(o, lrun)
        q_c[...] = pltpu.bitcast(q, u32)
        o_c[...] = o
        l_c[...] = lrun

    class _Many:
        def __init__(self, cps):
            self.cps = cps

        def start(self):
            for cp in self.cps:
                cp.start()

    named = dict(wql=cp_wq(H - 1, 1), v0=cp_v(0), wo0=_Many([cp_wo(0, t) for t in range(NT_D)]),
                 wq1=cp_wq(1), k1=cp_k(1),
                 wq0=cp_wq(0, 2), k0=cp_k(0, 3), wr=pltpu.make_async_copy(wr_hbm, wr_v, sem_h.at[4]))

    def front_cp(k):
        return cp_x(k) if isinstance(k, int) else named[k]

    for k in (0, 1, 'wq0', 'wr'):
        front_cp(k).start()
    r_v[...] = jnp.zeros((16, 128), f32)
    xs_v[...] = jnp.zeros((16, D), f32)
    o_c[...] = jnp.zeros((TS, DH), f32)
    l_c[...] = jnp.ones((TS, 128), f32)
    front_cp('k0').start()

    def ln_chunk(c, zs):
        pieces = LN_PIECES[c]
        n = XC // pieces
        for t in range(pieces):
            r0 = c * XC + t * n

            def ld(i):
                if i == 0:
                    return x_v[pl.ds(r0, n), :]
                return x_v[pl.ds(pl.multiple_of(r0 + zs * i, n), n), :]
            for tt, w in enumerate(_layernorm(ld)):
                xn_v[half(r0, n), tt * 128:(tt + 1) * 128] = w

    def router_tiles(u):
        wrf = jnp.broadcast_to(wr_v[...].astype(f32).reshape(1, D), (16, D))
        lhs = jnp.where(lax.broadcasted_iota(i32, (16, D), 0) == u, wrf, 0.0).astype(bf16)
        xn = xn_ld(u * TS, TS)
        return [(lhs[:, k * 128:(k + 1) * 128], xn[:, k * 128:(k + 1) * 128]) for k in range(NT_D)]

    cp_x(0).wait()
    cp_x(2).start()
    t0 = x_v[0:16, 0:128].astype(f32)[0:8, :]
    t0 = jnp.where(jnp.abs(t0) < 1.0, t0, 0.5)
    zv = pltpu.bitcast(t0 - t0, i32)
    z_v[0:8, :] = zv
    zs = zv[0, 0]
    ln_chunk(0, zs)

    for bi, plan in enumerate(FRONT_PLAN):
        for k in FRONT_WAIT[bi]:
            front_cp(k).wait()
        for k in FRONT_START[bi]:
            front_cp(k).start()
        rs = r_v[...]
        rj = {}
        mr = {}
        qs = {}
        for op in plan.split():
            if op[0] == 'L':
                ln_chunk(int(op[1:]), zs)
            elif op[0] == 'a':
                u = int(op[1:])
                ql_v[half(u * TS, TS), :] = pltpu.bitcast(qproj(0 if u <= L else H - 1, u), u32)
            elif op[0] == 'r':
                u = int(op[1:])
                first = u not in rj
                if first:
                    rj[u] = router_tiles(u)
                for _ in range(3 if first else 2):
                    a, b = rj[u].pop(0)
                    rs = rs + lax.dot_general(a, b, NT, preferred_element_type=f32)
            else:
                u, c = (int(t) for t in op[1:].split('.'))
                if u not in qs:
                    qs[u] = pltpu.bitcast(ql_v[half(u * TS, TS), :], bf16)
                s = lax.dot_general(qs[u], hw_v[0, c * KC:(c + 1) * KC, :], NT, preferred_element_type=f32)
                s_c[u, :, c * KC:(c + 1) * KC] = s
                mc = _fold(s, jnp.maximum)
                mr[u] = mc if u not in mr else jnp.maximum(mr[u], mc)
                if c == NCH - 1:
                    m_c[u] = mr[u]
        r_v[...] = rs
    q_c[...] = ql_v[half(L * TS, TS), :]

    def body(h, carry):
        def hook():
            cp_v(h + 1).start()
            for t in range(NT_D):
                cp_wo(h + 1, t).start()

            @pl.when(h + 2 < H)
            def _():
                cp_wq(h + 2).start()
                cp_k(h + 2).start()

            @pl.when(h == 1)
            def _():
                for i in range(3):
                    cp_f(i).start()

        pltpu.make_async_copy(hw_v.at[h + 1], hw_v.at[h + 1], sem_h.at[0]).wait()
        run_head(h, False, hook)
        return carry

    lax.fori_loop(0, H - 1, body, 0)

    cp_v(H - 1).wait()
    for t in range(NT_D):
        cp_wo(H - 1, t).wait()
    for i in range(3):
        cp_f(i).wait()
    run_head(H - 1, True)
    for c in range(len(OUT_CUTS)):
        cp_o(c).wait()


def _wrapped(*refs):
    @pl.when(pl.program_id(0) == 0)
    def _():
        _kernel(*refs)


def build(A_x, A_k_cache, A_v_cache, A_wq, A_wo, B_x, B_w_r, B_w_gate, B_w_up, B_w_down):
    out = pl.pallas_call(
        _wrapped,
        grid=(2,),
        in_specs=[pl.BlockSpec(memory_space=pl.ANY)] * 9,
        out_specs=pl.BlockSpec(memory_space=pl.ANY),
        out_shape=jax.ShapeDtypeStruct((S, D), bf16),
        scratch_shapes=[
            pltpu.VMEM((128, 128), i32),
            pltpu.VMEM((S, D), bf16),
            pltpu.VMEM((S // 2, D), u32),
            pltpu.VMEM((S, D), f32),
            pltpu.VMEM((H + 1, SLAB, DH), bf16),
            pltpu.VMEM((F, D), bf16),
            pltpu.VMEM((F, D), bf16),
            pltpu.VMEM((F, D), bf16),
            pltpu.VMEM((S, D), f32),
            pltpu.VMEM((16, 128), f32),
            pltpu.VMEM((16, D), f32),
            pltpu.VMEM((16, 128), f32),
            pltpu.SMEM((C,), i32),
            pltpu.VMEM((L, TS, S), f32),
            pltpu.VMEM((L, TS, 128), f32),
            pltpu.VMEM((TS // 2, DH), u32),
            pltpu.VMEM((TS, DH), f32),
            pltpu.VMEM((TS, 128), f32),
            pltpu.VMEM((S, D), bf16),
            pltpu.VMEM((S // 2, DH), u32),
            pltpu.VMEM((D,), bf16),
            pltpu.SemaphoreType.DMA((S // XC,)),
            pltpu.SemaphoreType.DMA((5,)),
            pltpu.SemaphoreType.DMA((1,)),
            pltpu.SemaphoreType.DMA((len(OUT_CUTS),)),
        ],
        compiler_params=pltpu.CompilerParams(vmem_limit_bytes=120 * 1024 * 1024,
                                             internal_scratch_in_bytes=64 * 1024,
                                             disable_bounds_checks=True,
                                             disable_semaphore_checks=True),
    )(A_x.reshape(S, D), A_k_cache.reshape(H, S, DH), A_v_cache.reshape(H, S, DH), A_wq, A_wo,
      B_w_r, B_w_gate.T, B_w_up.T, B_w_down)
    return out.reshape(1, S, D)


@jax.jit
def pallas_recurrent_scan__mha_block_cached__moe_arch_mod__prompt_kernel(
        A_x, A_k_cache, A_v_cache, A_wq, A_wo, B_x, B_w_r, B_w_gate, B_w_up, B_w_down):
    return build(A_x, A_k_cache, A_v_cache, A_wq, A_wo, B_x, B_w_r, B_w_gate, B_w_up, B_w_down)
```
